```python
import jax
import jax.numpy as jnp

def _softmax(x, axis=-1):
    return jax.nn.softmax(x, axis=axis)
def _gelu(x):
    return jax.nn.gelu(x, approximate=True)
def _silu(x):
    return jax.nn.silu(x)
def _sigmoid(x):
    return jax.nn.sigmoid(x)
def _layernorm(x, axis=-1, eps=1e-5):
    m = jnp.mean(x, axis=axis, keepdims=True)
    v = jnp.var(x, axis=axis, keepdims=True)
    return (x - m) / jnp.sqrt(v + eps)
def _scatter_add(tgt, idx, src, axis=0):
    return tgt.at[idx].add(src)
def _segment_sum(src, seg, n):
    return jax.ops.segment_sum(src, seg, n)
class _Rng:
    def __init__(self, key):
        self._k = key
    def _next(self):
        self._k, sub = jax.random.split(self._k)
        return sub
    def normal(self, shape):
        return jax.random.normal(self._next(), shape, dtype=jnp.bfloat16)
    def randint(self, lo, hi, shape):
        return jax.random.randint(self._next(), shape, lo, hi, dtype=jnp.int32)
    def uniform(self, shape, lo=0.0, hi=1.0):
        return jax.random.uniform(self._next(), shape, jnp.bfloat16, lo, hi)
    def permutation(self, n):
        return jax.random.permutation(self._next(), n)


kernel_name = 'concat_heads__ssm_conv_h3__linear_attn_block__prompt'

def setup_inputs():
    _rng = _Rng(jax.random.key(int.from_bytes(__import__("os").urandom(4), "little")))
    _w = (lambda a: (lambda t: t.astype(jnp.bfloat16) if jnp.issubdtype(t.dtype, jnp.floating) else t)(jnp.asarray(a)))
    def _A_setup():
        B, S, D = 1, 2048, 1024
        ks = 4
        return {
            "q": _w((lambda *s: _rng.normal(s) * 0.05)(B, S, D)),
            "k": _w((lambda *s: _rng.normal(s) * 0.05)(B, S, D)),
            "v": _w((lambda *s: _rng.normal(s) * 0.05)(B, S, D)),
            "shift_k": _w((lambda *s: _rng.normal(s) * 0.05)(D, ks) * 0.5),
            "ssm_k": _w((lambda *s: _rng.normal(s) * 0.05)(D, S) * (1.0 / S ** 0.5)),
            "ssm_D": _w((lambda *s: _rng.normal(s) * 0.05)(D)),
        }
    _A_in = _A_setup()

    def _B_setup():
        B, S, D = 1, 2048, 1024
        return {
            "x": _w((lambda *s: _rng.normal(s) * 0.05)(B, S, D)),
            "wqkv": _w((lambda *s: _rng.normal(s) * 0.05)(D, 3 * D)),
            "wo": _w((lambda *s: _rng.normal(s) * 0.05)(D, D)),
        }
    _B_in = _B_setup()

    return {
        "A_q": _A_in["q"],
        "A_k": _A_in["k"],
        "A_v": _A_in["v"],
        "A_shift_k": _A_in["shift_k"],
        "A_ssm_k": _A_in["ssm_k"],
        "A_ssm_D": _A_in["ssm_D"],
        "B_x": _B_in["x"],
        "B_wqkv": _B_in["wqkv"],
        "B_wo": _B_in["wo"],
    }

def reference(A_q, A_k, A_v, A_shift_k, A_ssm_k, A_ssm_D, B_x, B_wqkv, B_wo):
    def _A_ref(q, k, v, shift_k, ssm_k, ssm_D):
        B, S, D = q.shape
        ks = shift_k.shape[-1]
        k_pad = jnp.pad(k, ((0, 0), (ks - 1, 0), (0, 0)))
        k_shift = jnp.zeros_like(k)
        for t in range(ks):
            k_shift = k_shift + k_pad[:, t:t + S, :] * shift_k[:, ks - 1 - t][None, None, :]
        kv = k_shift * v
        L = 2 * S
        kv_pad = jnp.pad(kv, ((0, 0), (0, S), (0, 0)))
        kf_pad = jnp.pad(ssm_k, ((0, 0), (0, S)))
        kv_f = (lambda x, axes=(-2,-1): jnp.fft.rfft2(x.astype(jnp.float32), axes=axes))(kv_pad[:, None, :, :], axes=(1, 2))
        kf_f = (lambda x, axes=(-2,-1): jnp.fft.rfft2(x.astype(jnp.float32), axes=axes))(kf_pad[:, None, :], axes=(1, 2))
        kf_f = (lambda x, *d: x.transpose(*d))(kf_f, 1, 2, 0)
        y_f = kv_f * kf_f[None, :, :, :]
        y = (lambda x, s, axes=(-2,-1): jnp.fft.irfft2(x, s=s, axes=axes).astype(jnp.bfloat16))(y_f, (1, L), axes=(1, 2))[:, 0, :S, :]
        y = y + kv * ssm_D[None, None, :]
        return q * y

    def _B_ref(x, wqkv, wo):
        B, S, D = x.shape
        H = 32; Dh = D // H
        qkv = (lambda x, *d: x.transpose(*d))((x @ wqkv).reshape(B, S, 3, H, Dh), 2, 0, 3, 1, 4)
        q, k, v = qkv[0], qkv[1], qkv[2]
        phi = lambda t: jnp.where(t > 0, t + 1, jnp.exp(t)) + 1e-6
        pq, pk = phi(q), phi(k)
        kv = jnp.einsum("bhsd,bhse->bhde", pk, v)
        z = jnp.einsum("bhsd->bhd", pk)
        num = jnp.einsum("bhqd,bhde->bhqe", pq, kv)
        den = jnp.einsum("bhqd,bhd->bhq", pq, z)[..., None] + 1e-6
        o = num / den
        return (lambda x, *d: x.transpose(*d))(o, 0, 2, 1, 3).reshape(B, S, D) @ wo

    a = _A_ref(A_q, A_k, A_v, A_shift_k, A_ssm_k, A_ssm_D)
    b = _B_ref(B_x, B_wqkv, B_wo)
    return jnp.concatenate([a, b], axis=-1)
```

```python
import functools
import numpy as np
import jax
import jax.numpy as jnp
from jax import lax
from jax.experimental import pallas as pl
from jax.experimental.pallas import tpu as pltpu

f32, bf16, u32 = jnp.float32, jnp.bfloat16, jnp.uint32

S, D = 2048, 1024
G = 128
NG = D // G
B = 128
NB = S // B
HEAD = 32

PARAMS = {'RP': 8, 'KSPLIT': 2, 'CH': 128, 'RT': 256, 'FWD_START': 12, 'FILL_END': 11.5, 'KVPARTS': 4, 'ORDER': 'asc', 'TI': 1, 'PACE': 1, 'PSTEP': 2, 'NTA': 3, 'FILL_END_F': 0.9, 'SKIP': ''}


def _pack_rows(a):
    b = np.asarray(a, dtype=bf16).view(np.uint16).astype(np.uint32)
    return b[0::2] | (b[1::2] << 16)


def _dft_mats(RP):
    ks = np.concatenate([np.arange(0, 128, 2), np.arange(1, 128, 2)])
    th = np.pi * (2 * ks + 1) / 256.0
    ang = th[:, None] * np.arange(128)[None, :]
    C, Sn = np.cos(ang), -np.sin(ang)
    rows = []
    for r in range(128 // RP):
        rows.append(C[r * RP:(r + 1) * RP])
        rows.append(Sn[r * RP:(r + 1) * RP])
    F = np.concatenate(rows, axis=0)
    Finv = F.T * (2.0 / 256.0)
    return _pack_rows(F), _pack_rows(Finv)


def _phi(t):
    return jnp.where(t > 0, t + 1.0, jnp.exp(t)) + 1e-6


def _dot(a, b):
    return jnp.dot(a, b, preferred_element_type=f32)


def _bc(x):
    return pltpu.bitcast(x, bf16)


def _ld(ref, *idx):
    *lead, (r0, n) = idx
    return _bc(ref.bitcast(u32)[(*lead, pl.ds(r0 // 2, n // 2), slice(None))])


def make_kernel(P):
    RP, KSPLIT, CH, RT = P['RP'], P['KSPLIT'], P['CH'], P['RT']
    NR = 128 // RP
    NCH = S // CH
    NT = S // RT
    NTA = P['NTA']
    NSTEPS = NG + 1 + (NT - NTA)

    def kernel(q_hbm, k_hbm, v_hbm, sk_hbm, h_hbm, d_hbm, f_hbm, fi_hbm, x_hbm, w_hbm, wo_hbm, o_hbm,
               qs, ks, vs, sks, hs, ds_, fs, fis, xs, ws, wos,
               kpad, u_s, U_s, H_s, G_s, Z_s, oa_s, pk_s, v_s, pq_s, kv_s, z_s, M_s, zb_s, ob_s,
               sem_c, sem_x, sem_w, sem_a, sem_q, sem_wo, sem_oa, sem_ob):
        step = pl.program_id(0)
        q32, k32, v32, h32 = (r.bitcast(u32) for r in (q_hbm, k_hbm, v_hbm, h_hbm))
        x32, w32, wo32 = (r.bitcast(u32) for r in (x_hbm, w_hbm, wo_hbm))

        def col(g):
            return pl.ds(pl.multiple_of(g * G, G), G)

        def cp_consts():
            return [pltpu.make_async_copy(a, b, sem_c.at[n]) for n, (a, b) in
                    enumerate(((f_hbm, fs), (fi_hbm, fis), (sk_hbm, sks), (d_hbm, ds_)))]

        def cp_x(c):
            rows = pl.ds(c * (CH // 2), CH // 2)
            return pltpu.make_async_copy(x32.at[rows], xs.at[rows], sem_x.at[c])

        def cp_w(g, p):
            return pltpu.make_async_copy(w32.at[:, pl.ds(pl.multiple_of(p * D + g * G, G), G)], ws.at[g, p], sem_w.at[g, p])

        def cp_a(g):
            return [pltpu.make_async_copy(k32.at[:, col(g)], ks.at[g], sem_a.at[g]),
                    pltpu.make_async_copy(v32.at[:, col(g)], vs.at[g], sem_a.at[g]),
                    pltpu.make_async_copy(h32.at[pl.ds(pl.multiple_of(g * (G // 2), G // 2), G // 2)], hs.at[g], sem_a.at[g])]

        def cp_q(g):
            return pltpu.make_async_copy(q32.at[:, col(g)], qs.at[g], sem_q.at[g])

        def cp_wo():
            return pltpu.make_async_copy(wo32, wos, sem_wo.at[0])

        def cp_oa(g):
            return pltpu.make_async_copy(oa_s.at[g], o_hbm.at[:, col(g)], sem_oa.at[g])

        def cp_ob(t):
            rows = pl.ds(pl.multiple_of(t * RT, RT), RT)
            return pltpu.make_async_copy(ob_s.at[t], o_hbm.at[rows, pl.ds(D, D)], sem_ob.at[t])

        def a_pre(g, sk, j):
            r0 = j * B
            if j == 0:
                kpad[0:8, :] = jnp.zeros((8, G), f32)
            kpad[pl.ds(8 + r0, B), :] = _bc(ks[g, pl.ds(r0 // 2, B // 2), :]).astype(f32)
            ksh = kpad[pl.ds(8 + r0, B), :] * sk[0:1, :]
            for t in range(1, 4):
                ksh = ksh + kpad[pl.ds(8 + r0 - t, B), :] * sk[t:t + 1, :]
            u = (ksh * _bc(vs[g, pl.ds(r0 // 2, B // 2), :]).astype(f32)).astype(bf16)
            u_s[pl.ds(r0, B), :] = u
            return u

        def a_fwd(g, sk, j0):
            F = _bc(fs[...])
            u2 = jnp.concatenate([a_pre(g, sk, j0), a_pre(g, sk, j0 + 1)], axis=1)
            U2 = _dot(F, u2)
            h2 = jnp.concatenate([_bc(hs[g, :, pl.ds((j0 + d) * B, B)]) for d in range(2)], axis=0)
            H2 = lax.dot_general(F, h2, (((1,), (1,)), ((), ())), preferred_element_type=f32)
            for d in range(2):
                j = j0 + d
                U_s[j] = U2[:, d * G:(d + 1) * G]
                H = H2[:, d * G:(d + 1) * G]
                if j == 0:
                    G_s[0] = H
                else:
                    for r in range(NR):
                        a, b = 2 * r * RP, (2 * r + 1) * RP
                        hre, him = H[a:a + RP], H[b:b + RP]
                        if d == 0:
                            pre, pim = H_s[pl.ds(a, RP), :], H_s[pl.ds(b, RP), :]
                        else:
                            pre, pim = H2[a:a + RP, 0:G], H2[b:b + RP, 0:G]
                        if r < NR // 2:
                            G_s[j, pl.ds(a, RP), :] = hre - pim
                            G_s[j, pl.ds(b, RP), :] = him + pre
                        else:
                            G_s[j, pl.ds(a, RP), :] = hre + pim
                            G_s[j, pl.ds(b, RP), :] = him - pre
            if j0 + 2 < NB:
                H_s[...] = H2[:, G:2 * G]

        def load_sk(g):
            return sks[:, col(g)].astype(f32)

        def load_d(g):
            dall = ds_[...].astype(f32)
            return jnp.sum(jnp.where(lax.broadcasted_iota(jnp.int32, (8, G), 0) == g, dall, 0.0), axis=0, keepdims=True)

        def a_piece(i0, r, dep=None):
            a, b = 2 * r * RP, (2 * r + 1) * RP
            cache = {}
            def ld(ref, nm, j, off):
                if (nm, j, off) not in cache:
                    cache[(nm, j, off)] = ref[j, pl.ds(off, RP), :]
                return cache[(nm, j, off)]
            for i in range(i0, i0 + P['TI']):
                zre = zim = dep
                for j in range(i + 1):
                    gre, gim = ld(G_s, 'g', i - j, a), ld(G_s, 'g', i - j, b)
                    ure, uim = ld(U_s, 'u', j, a), ld(U_s, 'u', j, b)
                    tre = gre * ure - gim * uim
                    tim = gre * uim + gim * ure
                    zre = tre if zre is None else zre + tre
                    zim = tim if zim is None else zim + tim
                z = jnp.concatenate([zre, zim], axis=0)
                Z_s[i, pl.ds(2 * r * RP, 2 * RP), :] = z.astype(bf16)

        def a_inv(g, dvec, i0):
            z2 = jnp.concatenate([_ld(Z_s, i0 + d, (0, 256)) for d in range(2)], axis=1)
            y2 = _dot(_bc(fis[...]), z2)
            for d in range(2):
                r0 = (i0 + d) * B
                uu = _ld(u_s, (r0, B)).astype(f32)
                y = y2[:, d * G:(d + 1) * G] + uu * dvec
                qq = _bc(qs[g, pl.ds(r0 // 2, B // 2), :]).astype(f32)
                oa_s[g, pl.ds(r0, B), :] = (qq * y).astype(bf16)

        def emit(mm, state, ga, t_fill_end):
            pieces = []
            TI = P['TI']
            if ga is not None:
                dvec = load_d(ga)
                pairs = list(range(0, NB, 2))
                if P['ORDER'] == 'desc':
                    pairs = pairs[::-1]
                elif P['ORDER'] == 'mix':
                    lo, hi = pairs[:len(pairs) // 2], pairs[len(pairs) // 2:][::-1]
                    pairs = [b for pair in zip(hi, lo) for b in pair]
                for i0 in pairs:
                    pp = [(i, r) for r in range(NR) for i in range(i0, i0 + 2, TI)]
                    pieces += [(i, r, i0 if n == len(pp) - 1 else None) for n, (i, r) in enumerate(pp)]
            pcost = lambda i: sum(ii + 1 for ii in range(i, i + TI))
            tot_p = sum(pcost(p[0]) for p in pieces)
            T = 0
            done_cost = 0
            pi = 0
            pend_inv = []
            q_waited = False
            for (cost, fn, tag) in mm:
                if tag == 'fwd':
                    assert pi == len(pieces) and not pend_inv, "fwd for next tile would overwrite live U/G/u"
                fn()
                T += cost
                for i0 in pend_inv:
                    if not q_waited:
                        cp_q(ga).wait()
                        q_waited = True
                    a_inv(ga, dvec, i0)
                    T += 128
                pend_inv = []
                target = tot_p * min(1.0, T / t_fill_end)
                kk = 0
                while pi < len(pieces) and done_cost < target:
                    i, r, fin = pieces[pi]
                    dep = None
                    if P['PACE'] and 'pace' in state:
                        pace = state['pace']
                        idx = min(pace.shape[0] // RP - 1, kk * P['PSTEP'] * 8 // RP)
                        pv = pltpu.bitcast(pace[idx * RP:(idx + 1) * RP, :], u32)
                        dep = pltpu.bitcast(lax.shift_right_logical(lax.shift_right_logical(pv, u32(16)), u32(16)), f32)
                        kk += 1
                    a_piece(i, r, dep)
                    done_cost += pcost(i)
                    pi += 1
                    if fin is not None:
                        pend_inv.append(fin)
            assert pi == len(pieces) and not pend_inv
            if ga is not None:
                cp_oa(ga).start()

        def group_step(g, ga, first):
            KS = D // KSPLIT
            state = {}

            def proj_part(name, p, c, ks_):
                if first:
                    if ks_ == 0 and name == 'k':
                        cp_x(c).wait()
                    if ks_ == 0 and c == 0:
                        cp_w(g, p).wait()
                x = _bc(xs[pl.ds(c * CH // 2, CH // 2), pl.ds(ks_ * KS, KS)])
                w = _bc(ws[g, p, pl.ds(ks_ * KS // 2, KS // 2), :])
                part = _dot(x, w)
                state[name] = part if ks_ == 0 else state[name] + part
                state['pace'] = part

            def fin_k(c):
                pk = _phi(state.pop('k'))
                pk_s[pl.ds(c * CH, CH), :] = pk.astype(bf16)
                zp = jnp.sum(pk.reshape(CH // 8, 8, G), axis=0)
                state['z'] = zp if c == 0 else state['z'] + zp

            def fin_v(c):
                v_s[pl.ds(c * CH, CH), :] = state.pop('v').astype(bf16)

            def fin_q(c):
                pq_s[g, pl.ds(c * CH, CH), :] = _phi(state.pop('q')).astype(bf16)

            def kv_part(n):
                rows = S // P['KVPARTS']
                a = _ld(pk_s, (n * rows, rows))
                b = _ld(v_s, (n * rows, rows))
                part = lax.dot_general(a, b, (((0,), (0,)), ((), ())), preferred_element_type=f32)
                state['kv'] = part if n == 0 else state['kv'] + part
                if n == P['KVPARTS'] - 1:
                    kv_s[g] = state.pop('kv')
                    z_s[g] = state.pop('z')

            def fwd_task(j):
                if j == 0:
                    for c in cp_a(g):
                        c.wait()
                    state['sk'] = load_sk(g)
                a_fwd(g, state['sk'], j)

            mm = []
            pc = CH * 8 // KSPLIT // 4
            nfw = NCH - int(P['FWD_START'] * NCH / 16)
            fwd_sched = {}
            c0 = NCH - nfw
            for j in range(0, NB, 2):
                fwd_sched.setdefault(c0 + j * nfw // NB, []).append(j)
            t_fill_end = None
            for c in range(NCH):
                if c == int(P['FILL_END'] * NCH / 16):
                    frac = P['FILL_END'] * NCH / 16 - c
                    t_fill_end = sum(m[0] for m in mm) + frac * 3 * KSPLIT * pc
                fw = list(fwd_sched.get(c, []))
                for name, p, fin in (('k', 1, fin_k), ('v', 2, fin_v)):
                    for ks_ in range(KSPLIT):
                        def t(name=name, p=p, c=c, ks_=ks_, fin=fin):
                            proj_part(name, p, c, ks_)
                            if ks_ == KSPLIT - 1:
                                fin(c)
                        mm.append((pc, t, None))
                    if fw:
                        ntake = (len(fw) + 1) // 2 if name == 'k' else len(fw)
                        for j in fw[:ntake]:
                            mm.append((256, functools.partial(fwd_task, j), 'fwd'))
                        fw = fw[ntake:]
                if c >= 1:
                    for ks_ in range(KSPLIT):
                        def t(c=c - 1, ks_=ks_):
                            proj_part('q', 0, c, ks_)
                            if ks_ == KSPLIT - 1:
                                fin_q(c)
                        mm.append((pc, t, None))
                per = NCH // P['KVPARTS']
                if (c + 1) % per == 0:
                    mm.append((512 // P['KVPARTS'], functools.partial(kv_part, c // per), None))
            for ks_ in range(KSPLIT):
                def t(c=NCH - 1, ks_=ks_):
                    proj_part('q', 0, c, ks_)
                    if ks_ == KSPLIT - 1:
                        fin_q(c)
                mm.append((pc, t, None))
            emit(mm, state, ga, t_fill_end)

        def out_tasks(t, state):
            t0 = t * (RT // 2)
            rows = pl.ds(t0 if isinstance(t, int) else pl.multiple_of(t0, RT // 2), RT // 2)
            pq32 = pq_s.bitcast(u32)
            key = ('pqn', t if isinstance(t, int) else 0)

            def norm(gs):
                for g in gs:
                    pq = _bc(pq32[g, rows, :])
                    den = _dot(pq, _ld(zb_s, g, (0, G))) + 1e-6
                    state.setdefault(key, []).append((pq.astype(f32) * pl.reciprocal(den, approx=True)).astype(bf16))
                    state['pace'] = den

            def proj(j):
                lhs = jnp.concatenate(state[key], axis=1)
                res = _dot(lhs, _ld(M_s, j, (0, D)))
                ob_s[t, :, pl.ds(j * G, G)] = res.astype(bf16)
                state['pace'] = res
                if j == NG - 1:
                    cp_ob(t).start()

            tasks = [(RT, functools.partial(norm, range(0, 4)), None), (RT, functools.partial(norm, range(4, 8)), None)]
            tasks += [(2 * RT, functools.partial(proj, j), None) for j in range(NG)]
            return tasks

        def m_tasks():
            r = lax.broadcasted_iota(jnp.int32, (G, G), 0) // HEAD
            c = lax.broadcasted_iota(jnp.int32, (G, G), 1) // HEAD
            bd = r == c

            def mt(g):
                z = jnp.sum(z_s[g], axis=0, keepdims=True)
                zc = jnp.broadcast_to(z, (G, G)).T
                zb_s[g] = jnp.where(bd, zc, 0.0).astype(bf16)
                kvb = jnp.where(bd, kv_s[g], 0.0).astype(bf16)
                wo = _bc(wos[pl.ds(g * G // 2, G // 2), :])
                Mg = _dot(kvb, wo).astype(bf16)
                for j in range(NG):
                    M_s[j, pl.ds(g * G, G), :] = Mg[:, j * G:(j + 1) * G]
            return [(256, functools.partial(mt, g), None) for g in range(NG)]

        @pl.when(step == 0)
        def _():
            for c in cp_consts():
                c.start()
            cp_w(0, 1).start()
            cp_x(0).start()
            cp_w(0, 2).start()
            cp_x(1).start()
            cp_w(0, 0).start()
            for c in range(2, NCH):
                cp_x(c).start()
            for c in cp_a(0):
                c.start()
            for g in range(1, NG):
                for p in (1, 2, 0):
                    cp_w(g, p).start()
                cp_q(g - 1).start()
                for c in cp_a(g):
                    c.start()
            cp_wo().start()
            cp_q(NG - 1).start()
            for c in cp_consts():
                c.wait()
            group_step(0, None, True)

        @pl.when(jnp.logical_and(step > 0, step < NG))
        def _():
            for p in (1, 2, 0):
                cp_w(step, p).wait()
            group_step(step, step - 1, False)

        @pl.when(step == NG)
        def _():
            cp_wo().wait()
            state = {}
            mm = m_tasks()
            for t in range(NTA):
                mm += out_tasks(t, state)
            emit(mm, state, NG - 1, sum(m[0] for m in mm) * P['FILL_END_F'])

        @pl.when(step > NG)
        def _():
            state = {}
            for (_, fn, _) in out_tasks(step - (NG + 1) + NTA, state):
                fn()

        @pl.when(step == NSTEPS - 1)
        def _():
            for g in range(NG):
                cp_oa(g).wait()
            for t in range(NT):
                cp_ob(t).wait()

    scratch = [
        pltpu.VMEM((NG, S // 2, G), u32), pltpu.VMEM((NG, S // 2, G), u32), pltpu.VMEM((NG, S // 2, G), u32),
        pltpu.VMEM((4, D), bf16), pltpu.VMEM((NG, G // 2, S), u32), pltpu.VMEM((8, 128), bf16),
        pltpu.VMEM((128, 128), u32), pltpu.VMEM((64, 256), u32),
        pltpu.VMEM((S // 2, D), u32), pltpu.VMEM((NG, 3, D // 2, G), u32), pltpu.VMEM((D // 2, D), u32),
        pltpu.VMEM((S + 8, G), f32), pltpu.VMEM((S, G), bf16),
        pltpu.VMEM((NB, 256, G), f32), pltpu.VMEM((256, G), f32), pltpu.VMEM((NB, 256, G), f32),
        pltpu.VMEM((NB, 256, G), bf16), pltpu.VMEM((NG, S, G), bf16),
        pltpu.VMEM((S, G), bf16), pltpu.VMEM((S, G), bf16), pltpu.VMEM((NG, S, G), bf16),
        pltpu.VMEM((NG, G, G), f32), pltpu.VMEM((NG, 8, G), f32),
        pltpu.VMEM((NG, D, G), bf16), pltpu.VMEM((NG, G, G), bf16), pltpu.VMEM((NT, RT, D), bf16),
        pltpu.SemaphoreType.DMA((4,)), pltpu.SemaphoreType.DMA((NCH,)), pltpu.SemaphoreType.DMA((NG, 3)),
        pltpu.SemaphoreType.DMA((NG,)), pltpu.SemaphoreType.DMA((NG,)), pltpu.SemaphoreType.DMA((1,)),
        pltpu.SemaphoreType.DMA((NG,)), pltpu.SemaphoreType.DMA((NT,)),
    ]
    return kernel, scratch, NSTEPS


_KERNEL, _SCRATCH, _NSTEPS = make_kernel(PARAMS)
_FP, _FIP = _dft_mats(PARAMS['RP'])


@jax.jit
def pallas_concat_heads__ssm_conv_h3__linear_attn_block__prompt_kernel(A_q, A_k, A_v, A_shift_k, A_ssm_k, A_ssm_D, B_x, B_wqkv, B_wo):
    out = pl.pallas_call(
        _KERNEL, grid=(_NSTEPS,),
        in_specs=[pl.BlockSpec(memory_space=pl.ANY)] * 11,
        out_specs=pl.BlockSpec(memory_space=pl.ANY),
        out_shape=jax.ShapeDtypeStruct((S, 2 * D), bf16),
        scratch_shapes=_SCRATCH,
        compiler_params=pltpu.CompilerParams(vmem_limit_bytes=110 * 1024 * 1024, dimension_semantics=("arbitrary",)),
    )(A_q.reshape(S, D), A_k.reshape(S, D), A_v.reshape(S, D), A_shift_k.T, A_ssm_k, A_ssm_D.reshape(8, 128),
      jnp.asarray(_FP), jnp.asarray(_FIP), B_x.reshape(S, D), B_wqkv, B_wo)
    return out.reshape(1, S, 2 * D)
```

```python
import functools
import numpy as np
import jax
import jax.numpy as jnp
from jax import lax
from jax.experimental import pallas as pl
from jax.experimental.pallas import tpu as pltpu

f32, bf16, u32 = jnp.float32, jnp.bfloat16, jnp.uint32

S, D = 2048, 1024
G = 128
NG = D // G
B = 128
NB = S // B
HEAD = 32

PARAMS = {'RP': 8, 'KSPLIT': 2, 'CH': 128, 'RT': 256, 'FWD_START': 14.0, 'FWD_START0': 16, 'ORDER_F': 'desc', 'PSTEP_F': 4, 'FILL_END': 13.8, 'KVPARTS': 4, 'ORDER': 'asc', 'TI': 4, 'PACE': 1, 'PSTEP': 4, 'NTA': 3, 'NTB': 1, 'FILL_END_F': 0.9, 'SKIP': '', 'XG': '1-2-4-7-11-16'}


def _pack_rows(a):
    b = np.asarray(a, dtype=bf16).view(np.uint16).astype(np.uint32)
    return b[0::2] | (b[1::2] << 16)


def _dft_mats(RP):
    ks = np.concatenate([np.arange(0, 128, 2), np.arange(1, 128, 2)])
    th = np.pi * (2 * ks + 1) / 256.0
    ang = th[:, None] * np.arange(128)[None, :]
    C, Sn = np.cos(ang), -np.sin(ang)
    rows = []
    for r in range(128 // RP):
        rows.append(C[r * RP:(r + 1) * RP])
        rows.append(Sn[r * RP:(r + 1) * RP])
    F = np.concatenate(rows, axis=0)
    Finv = F.T * (2.0 / 256.0)
    return _pack_rows(F), _pack_rows(Finv)


def _phi(t):
    return jnp.where(t > 0, t + 1.0, jnp.exp(t)) + 1e-6


def _dot(a, b):
    return jnp.dot(a, b, preferred_element_type=f32)


def _bc(x):
    return pltpu.bitcast(x, bf16)


def _ld(ref, *idx):
    *lead, (r0, n) = idx
    return _bc(ref.bitcast(u32)[(*lead, pl.ds(r0 // 2, n // 2), slice(None))])


def make_kernel(P):
    RP, KSPLIT, CH, RT = P['RP'], P['KSPLIT'], P['CH'], P['RT']
    NR = 128 // RP
    NCH = S // CH
    NT = S // RT
    NTA = P['NTA']
    NTB = P['NTB']
    assert (NT - NTA) % NTB == 0
    NSTEPS = NG + 1 + (NT - NTA) // NTB
    X_GROUPS = []
    bnds = [int(v) for v in P['XG'].split('-')]
    for lo, hi in zip(bnds[:-1], bnds[1:]):
        X_GROUPS.append((list(range(lo, hi)), ('v', lo - 1)))

    def kernel(q_hbm, k_hbm, v_hbm, sk_hbm, h_hbm, d_hbm, f_hbm, fi_hbm, x_hbm, w_hbm, wo_hbm, o_hbm,
               qs, ks, vs, sks, hs, ds_, fs, fis, xs, ws, wos, wcur,
               kpad, u_s, U_s, H_s, G_s, Z_s, oa_s, pk_s, v_s, pq_s, kv_s, z_s, M_s, zb_s, ob_s,
               sem_c, sem_x, sem_w, sem_a, sem_q, sem_wo, sem_oa, sem_ob):
        step = pl.program_id(0)
        q32, k32, v32, h32 = (r.bitcast(u32) for r in (q_hbm, k_hbm, v_hbm, h_hbm))
        x32, w32, wo32 = (r.bitcast(u32) for r in (x_hbm, w_hbm, wo_hbm))

        def col(g):
            return pl.ds(pl.multiple_of(g * G, G), G)

        def cp_consts():
            return [pltpu.make_async_copy(a, b, sem_c.at[n]) for n, (a, b) in
                    enumerate(((f_hbm, fs), (fi_hbm, fis), (sk_hbm, sks), (d_hbm, ds_)))]

        def cp_x(c):
            rows = pl.ds(c * (CH // 2), CH // 2)
            return pltpu.make_async_copy(x32.at[rows], xs.at[rows], sem_x.at[c])

        def cp_w(g, p):
            gs = min(g, NG - 1) if isinstance(g, int) else jnp.minimum(g, NG - 1)
            cols = pl.ds(p * D + gs * G if isinstance(gs, int) else pl.multiple_of(p * D + gs * G, G), G)
            return pltpu.make_async_copy(w32.at[:, cols], ws.at[g, p], sem_w.at[3 * g + p])

        def cp_a(g):
            return [pltpu.make_async_copy(k32.at[:, col(g)], ks.at[g], sem_a.at[g]),
                    pltpu.make_async_copy(v32.at[:, col(g)], vs.at[g], sem_a.at[g]),
                    pltpu.make_async_copy(h32.at[pl.ds(pl.multiple_of(g * (G // 2), G // 2), G // 2)], hs.at[g], sem_a.at[g])]

        def cp_q(g):
            return pltpu.make_async_copy(q32.at[:, col(g)], qs.at[g], sem_q.at[g])

        def cp_wo():
            return pltpu.make_async_copy(wo32, wos, sem_wo.at[0])

        def cp_oa(g):
            return pltpu.make_async_copy(oa_s.at[g], o_hbm.at[:, col(g)], sem_oa.at[g])

        def cp_ob(t, j):
            rows = pl.ds(t * RT if isinstance(t, int) else pl.multiple_of(t * RT, RT), RT)
            return pltpu.make_async_copy(ob_s.at[t, j], o_hbm.at[rows, pl.ds(D + j * G, G)], sem_ob.at[t])

        def a_pre(g, sk, j):
            r0 = j * B
            if j == 0:
                kpad[0:8, :] = jnp.zeros((8, G), f32)
            kpad[pl.ds(8 + r0, B), :] = _bc(ks[g, pl.ds(r0 // 2, B // 2), :]).astype(f32)
            ksh = kpad[pl.ds(8 + r0, B), :] * sk[0:1, :]
            for t in range(1, 4):
                ksh = ksh + kpad[pl.ds(8 + r0 - t, B), :] * sk[t:t + 1, :]
            u = (ksh * _bc(vs[g, pl.ds(r0 // 2, B // 2), :]).astype(f32)).astype(bf16)
            u_s[pl.ds(r0, B), :] = u
            return u

        def a_fwd(g, sk, j0):
            F = _bc(fs[...])
            u2 = jnp.concatenate([a_pre(g, sk, j0), a_pre(g, sk, j0 + 1)], axis=1)
            U2 = _dot(F, u2)
            h2 = jnp.concatenate([_bc(hs[g, :, pl.ds((j0 + d) * B, B)]) for d in range(2)], axis=0)
            H2 = lax.dot_general(F, h2, (((1,), (1,)), ((), ())), preferred_element_type=f32)
            for d in range(2):
                j = j0 + d
                U_s[j] = U2[:, d * G:(d + 1) * G]
                H = H2[:, d * G:(d + 1) * G]
                if j == 0:
                    G_s[0] = H
                else:
                    for r in range(NR):
                        a, b = 2 * r * RP, (2 * r + 1) * RP
                        hre, him = H[a:a + RP], H[b:b + RP]
                        if d == 0:
                            pre, pim = H_s[pl.ds(a, RP), :], H_s[pl.ds(b, RP), :]
                        else:
                            pre, pim = H2[a:a + RP, 0:G], H2[b:b + RP, 0:G]
                        if r < NR // 2:
                            G_s[j, pl.ds(a, RP), :] = hre - pim
                            G_s[j, pl.ds(b, RP), :] = him + pre
                        else:
                            G_s[j, pl.ds(a, RP), :] = hre + pim
                            G_s[j, pl.ds(b, RP), :] = him - pre
            if j0 + 2 < NB:
                H_s[...] = H2[:, G:2 * G]

        def load_sk(g):
            return sks[:, col(g)].astype(f32)

        def load_d(g):
            dall = ds_[...].astype(f32)
            return jnp.sum(jnp.where(lax.broadcasted_iota(jnp.int32, (8, G), 0) == g, dall, 0.0), axis=0, keepdims=True)

        def a_piece(i0, r, dep=None):
            a, b = 2 * r * RP, (2 * r + 1) * RP
            T = P['TI']
            acc = [(dep, dep)] * T
            gw = {}
            for j in range(i0 + T):
                ure, uim = U_s[j, pl.ds(a, RP), :], U_s[j, pl.ds(b, RP), :]
                for t in range(T):
                    m = i0 + t - j
                    if m < 0:
                        continue
                    if m not in gw:
                        gw[m] = (G_s[m, pl.ds(a, RP), :], G_s[m, pl.ds(b, RP), :])
                    gre, gim = gw[m]
                    tre = gre * ure - gim * uim
                    tim = gre * uim + gim * ure
                    zre, zim = acc[t]
                    acc[t] = (tre if zre is None else zre + tre, tim if zim is None else zim + tim)
            for t in range(T):
                z = jnp.concatenate(acc[t], axis=0)
                Z_s[i0 + t, pl.ds(2 * r * RP, 2 * RP), :] = z.astype(bf16)

        def a_inv(g, dvec, i0):
            z2 = jnp.concatenate([_ld(Z_s, i0 + d, (0, 256)) for d in range(2)], axis=1)
            y2 = _dot(_bc(fis[...]), z2)
            for d in range(2):
                r0 = (i0 + d) * B
                uu = _ld(u_s, (r0, B)).astype(f32)
                y = y2[:, d * G:(d + 1) * G] + uu * dvec
                qq = _bc(qs[g, pl.ds(r0 // 2, B // 2), :]).astype(f32)
                oa_s[g, pl.ds(r0, B), :] = (qq * y).astype(bf16)

        def emit(mm, state, ga, t_fill_end, order, pstep):
            pieces = []
            TI = P['TI']
            if ga is not None:
                dvec = load_d(ga)
                GS = max(2, TI)
                pairs = list(range(0, NB, GS))
                if order == 'desc':
                    pairs = pairs[::-1]
                elif order == 'mix':
                    lo, hi = pairs[:len(pairs) // 2], pairs[len(pairs) // 2:][::-1]
                    pairs = [b for pair in zip(hi, lo) for b in pair]
                for i0 in pairs:
                    pp = [(i, r) for r in range(NR) for i in range(i0, i0 + GS, TI)]
                    pieces += [(i, r, list(range(i0, i0 + GS, 2)) if n == len(pp) - 1 else None) for n, (i, r) in enumerate(pp)]
            pcost = lambda i: sum(ii + 1 for ii in range(i, i + TI))
            tot_p = sum(pcost(p[0]) for p in pieces)
            T = 0
            done_cost = 0
            pi = 0
            pend_inv = []
            for (cost, fn, tag) in mm:
                if tag == 'fwd':
                    assert pi == len(pieces) and not pend_inv, "fwd for next tile would overwrite live U/G/u"
                fn()
                T += cost
                for i0 in pend_inv:
                    a_inv(ga, dvec, i0)
                    T += 128
                pend_inv = []
                target = tot_p * min(1.0, T / t_fill_end)
                kk = 0
                while pi < len(pieces) and done_cost < target:
                    i, r, fin = pieces[pi]
                    dep = None
                    if P['PACE'] and 'pace' in state:
                        pace = state['pace']
                        idx = min(pace.shape[0] // RP - 1, kk * pstep * 8 // RP)
                        pv = pltpu.bitcast(pace[idx * RP:(idx + 1) * RP, :], u32)
                        dep = pltpu.bitcast(lax.shift_right_logical(lax.shift_right_logical(pv, u32(16)), u32(16)), f32)
                        kk += 1
                    a_piece(i, r, dep)
                    done_cost += pcost(i)
                    pi += 1
                    if fin is not None:
                        pend_inv.extend(fin)
            assert pi == len(pieces) and not pend_inv
            if ga is not None:
                cp_oa(ga).start()

        def group_step(g, ga, first):
            KS = D // KSPLIT
            state = {}

            hooks = {}

            def proj_part(name, p, c, ks_):
                x = _bc(xs[pl.ds(c * CH // 2, CH // 2), pl.ds(ks_ * KS, KS)])
                if first:
                    w = _bc(ws[g, p, pl.ds(ks_ * KS // 2, KS // 2), :])
                else:
                    w = _bc(wcur[p, pl.ds(ks_ * KS // 2, KS // 2), :])
                part = _dot(x, w)
                state[name] = part if ks_ == 0 else state[name] + part
                state['pace'] = part
                if ks_ == KSPLIT - 1:
                    for h in hooks.get((name, c), []):
                        h()

            def fin_k(c):
                pk = _phi(state.pop('k'))
                pk_s[pl.ds(c * CH, CH), :] = pk.astype(bf16)
                zp = jnp.sum(pk.reshape(CH // 8, 8, G), axis=0)
                state['z'] = zp if c == 0 else state['z'] + zp

            def fin_v(c):
                v_s[pl.ds(c * CH, CH), :] = state.pop('v').astype(bf16)
                if c == NCH - 1:
                    next_w(1)
                    next_w(2)

            def next_w(p):
                if not first:
                    wcur[p] = ws[g + 1, p]

            def fin_q(c):
                pq_s[g, pl.ds(c * CH, CH), :] = _phi(state.pop('q')).astype(bf16)
                if c == NCH - 1:
                    next_w(0)

            def kv_part(n):
                if 'kv' in P['SKIP']:
                    if n == P['KVPARTS'] - 1:
                        kv_s[g] = jnp.zeros((G, G), f32) + state['pace'][0:G, :]
                        z_s[g] = state.pop('z')
                    return
                rows = S // P['KVPARTS']
                a = _ld(pk_s, (n * rows, rows))
                b = _ld(v_s, (n * rows, rows))
                part = lax.dot_general(a, b, (((0,), (0,)), ((), ())), preferred_element_type=f32)
                state['kv'] = part if n == 0 else state['kv'] + part
                if n == P['KVPARTS'] - 1:
                    kv_s[g] = state.pop('kv')
                    z_s[g] = state.pop('z')

            def fwd_task(j):
                if 'fwd' in P['SKIP']:
                    return
                if j == 0:
                    state['sk'] = load_sk(g)
                a_fwd(g, state['sk'], j)

            def wait_all(cps, nm="w"):
                if True:
                    for c in cps:
                        c.wait()

            fwd_start = P['FWD_START0'] if first else P['FWD_START']
            c_fw0 = int(fwd_start * NCH / 16)
            def wait_late():
                cps = cp_a(g)
                if not first:
                    cps = cps + [cp_w(g + 1, p) for p in (1, 2, 0)]
                wait_all(cps, 'a')

            if c_fw0 < NCH:
                hooks.setdefault(('k', c_fw0), []).append(wait_late)
            else:
                hooks.setdefault(('q', NCH - 1), []).append(wait_late)
            if first:
                hooks.setdefault(('k', 0), []).append(lambda: wait_all([cp_w(g, 2)], 'wv'))
                hooks.setdefault(('v', 0), []).append(lambda: wait_all([cp_w(g, 0)], 'wq'))
                for grp, at in X_GROUPS:
                    hooks.setdefault(at, []).append(functools.partial(lambda grp: wait_all([cp_x(c) for c in grp], 'x%d' % grp[0]), grp))

            mm = []
            pc = CH * 8 // KSPLIT // 4
            nfw = NCH - c_fw0
            fwd_sched = {}
            for j in range(0, NB, 2):
                fwd_sched.setdefault(c_fw0 + j * nfw // NB, []).append(j)
            t_fill_end = None
            for c in range(NCH):
                if c == int(P['FILL_END'] * NCH / 16):
                    frac = P['FILL_END'] * NCH / 16 - c
                    t_fill_end = sum(m[0] for m in mm) + frac * 3 * KSPLIT * pc
                fw = list(fwd_sched.get(c, []))
                for name, p, fin in (('k', 1, fin_k), ('v', 2, fin_v)):
                    for ks_ in range(KSPLIT):
                        def t(name=name, p=p, c=c, ks_=ks_, fin=fin):
                            proj_part(name, p, c, ks_)
                            if ks_ == KSPLIT - 1:
                                fin(c)
                        mm.append((pc, t, None))
                    if fw:
                        ntake = (len(fw) + 1) // 2 if name == 'k' else len(fw)
                        for j in fw[:ntake]:
                            mm.append((256, functools.partial(fwd_task, j), 'fwd'))
                        fw = fw[ntake:]
                if c >= 1:
                    for ks_ in range(KSPLIT):
                        def t(c=c - 1, ks_=ks_):
                            proj_part('q', 0, c, ks_)
                            if ks_ == KSPLIT - 1:
                                fin_q(c)
                        mm.append((pc, t, None))
                per = NCH // P['KVPARTS']
                if (c + 1) % per == 0:
                    mm.append((512 // P['KVPARTS'], functools.partial(kv_part, c // per), None))
            for ks_ in range(KSPLIT):
                def t(c=NCH - 1, ks_=ks_):
                    proj_part('q', 0, c, ks_)
                    if ks_ == KSPLIT - 1:
                        fin_q(c)
                mm.append((pc, t, None))
            for j in fwd_sched.get(NCH, []):
                mm.append((256, functools.partial(fwd_task, j), 'fwd'))
            emit(mm, state, ga, t_fill_end, P['ORDER'], P['PSTEP'])
            if first:
                wait_all([cp_w(1, p) for p in (1, 2, 0)], 'w1')
                for p in range(3):
                    wcur[p] = ws[1, p]

        def out_tasks(t, state, uid):
            t0 = t * (RT // 2)
            rows = pl.ds(t0 if isinstance(t, int) else pl.multiple_of(t0, RT // 2), RT // 2)
            pq32 = pq_s.bitcast(u32)
            key = ('pqn', uid)

            def norm(gs):
                for g in gs:
                    pq = _bc(pq32[g, rows, :])
                    den = _dot(pq, _ld(zb_s, g, (0, G))) + 1e-6
                    state.setdefault(key, []).append((pq.astype(f32) * pl.reciprocal(den, approx=True)).astype(bf16))
                    state['pace'] = den

            def proj(j):
                lhs = jnp.concatenate(state[key], axis=1)
                res = _dot(lhs, _ld(M_s, j, (0, D)))
                ob_s[t, j] = res.astype(bf16)
                state['pace'] = res
                cp_ob(t, j).start()

            tasks = [(RT, functools.partial(norm, range(0, 4)), None), (RT, functools.partial(norm, range(4, 8)), None)]
            tasks += [(2 * RT, functools.partial(proj, j), None) for j in range(NG)]
            return tasks

        def m_tasks():
            r = lax.broadcasted_iota(jnp.int32, (G, G), 0) // HEAD
            c = lax.broadcasted_iota(jnp.int32, (G, G), 1) // HEAD
            bd = r == c

            def mt(g):
                z = jnp.sum(z_s[g], axis=0, keepdims=True)
                zc = jnp.broadcast_to(z, (G, G)).T
                zb_s[g] = jnp.where(bd, zc, 0.0).astype(bf16)
                kvb = jnp.where(bd, kv_s[g], 0.0).astype(bf16)
                wo = _bc(wos[pl.ds(g * G // 2, G // 2), :])
                Mg = _dot(kvb, wo).astype(bf16)
                for j in range(NG):
                    M_s[j, pl.ds(g * G, G), :] = Mg[:, j * G:(j + 1) * G]
            return [(256, functools.partial(mt, g), None) for g in range(NG)]

        @pl.when(step == 0)
        def _():
            for c in cp_consts():
                c.start()
            cp_w(0, 1).start()
            cp_x(0).start()
            cp_w(0, 2).start()
            cp_w(0, 0).start()
            for c in range(1, NCH):
                cp_x(c).start()
            for c in cp_a(0):
                c.start()
            for g in range(1, NG + 1):
                for p in (1, 2, 0):
                    cp_w(g, p).start()
                cp_q(g - 1).start()
                if g < NG:
                    for c in cp_a(g):
                        c.start()
            cp_wo().start()
            if True:
                for c in cp_consts():
                    c.wait()
                cp_w(0, 1).wait()
                cp_x(0).wait()
            group_step(0, None, True)

        @pl.when(jnp.logical_and(step > 0, step < NG))
        def _():
            cp_q(step - 1).wait()
            group_step(step, step - 1, False)

        @pl.when(step == NG)
        def _():
            cp_wo().wait()
            cp_q(NG - 1).wait()
            state = {}
            mm = m_tasks()
            for t in range(NTA):
                mm += out_tasks(t, state, t)
            emit(mm, state, NG - 1, sum(m[0] for m in mm) * P['FILL_END_F'], P['ORDER_F'], P['PSTEP_F'])

        @pl.when(step > NG)
        def _():
            state = {}
            for d in range(NTB):
                t = (step - (NG + 1)) * NTB + NTA + d if NSTEPS > NG + 2 else NTA + d
                for (_, fn, _) in out_tasks(t, state, d):
                    fn()

        @pl.when(step == NSTEPS - 1)
        def _():
            for g in range(NG):
                cp_oa(g).wait()
            for t in range(NT):
                for j in range(NG):
                    cp_ob(t, j).wait()

    scratch = [
        pltpu.VMEM((NG, S // 2, G), u32), pltpu.VMEM((NG, S // 2, G), u32), pltpu.VMEM((NG, S // 2, G), u32),
        pltpu.VMEM((4, D), bf16), pltpu.VMEM((NG, G // 2, S), u32), pltpu.VMEM((8, 128), bf16),
        pltpu.VMEM((128, 128), u32), pltpu.VMEM((64, 256), u32),
        pltpu.VMEM((S // 2, D), u32), pltpu.VMEM((NG + 1, 3, D // 2, G), u32), pltpu.VMEM((D // 2, D), u32),
        pltpu.VMEM((3, D // 2, G), u32),
        pltpu.VMEM((S + 8, G), f32), pltpu.VMEM((S, G), bf16),
        pltpu.VMEM((NB, 256, G), f32), pltpu.VMEM((256, G), f32), pltpu.VMEM((NB, 256, G), f32),
        pltpu.VMEM((NB, 256, G), bf16), pltpu.VMEM((NG, S, G), bf16),
        pltpu.VMEM((S, G), bf16), pltpu.VMEM((S, G), bf16), pltpu.VMEM((NG, S, G), bf16),
        pltpu.VMEM((NG, G, G), f32), pltpu.VMEM((NG, 8, G), f32),
        pltpu.VMEM((NG, D, G), bf16), pltpu.VMEM((NG, G, G), bf16), pltpu.VMEM((NT, NG, RT, G), bf16),
        pltpu.SemaphoreType.DMA((4,)), pltpu.SemaphoreType.DMA((NCH,)), pltpu.SemaphoreType.DMA((3 * (NG + 1),)),
        pltpu.SemaphoreType.DMA((NG,)), pltpu.SemaphoreType.DMA((NG,)), pltpu.SemaphoreType.DMA((1,)),
        pltpu.SemaphoreType.DMA((NG,)), pltpu.SemaphoreType.DMA((NT,)),
    ]
    return kernel, scratch, NSTEPS


_KERNEL, _SCRATCH, _NSTEPS = make_kernel(PARAMS)
_FP, _FIP = _dft_mats(PARAMS['RP'])


@jax.jit
def pallas_concat_heads__ssm_conv_h3__linear_attn_block__prompt_kernel(A_q, A_k, A_v, A_shift_k, A_ssm_k, A_ssm_D, B_x, B_wqkv, B_wo):
    out = pl.pallas_call(
        _KERNEL, grid=(_NSTEPS,),
        in_specs=[pl.BlockSpec(memory_space=pl.ANY)] * 11,
        out_specs=pl.BlockSpec(memory_space=pl.ANY),
        out_shape=jax.ShapeDtypeStruct((S, 2 * D), bf16),
        scratch_shapes=_SCRATCH,
        compiler_params=pltpu.CompilerParams(vmem_limit_bytes=110 * 1024 * 1024, dimension_semantics=("arbitrary",)),
    )(A_q.reshape(S, D), A_k.reshape(S, D), A_v.reshape(S, D), A_shift_k.T, A_ssm_k, A_ssm_D.reshape(8, 128),
      jnp.asarray(_FP), jnp.asarray(_FIP), B_x.reshape(S, D), B_wqkv, B_wo)
    return out.reshape(1, S, 2 * D)
```

```python
import functools
import numpy as np
import jax
import jax.numpy as jnp
from jax import lax
from jax.experimental import pallas as pl
from jax.experimental.pallas import tpu as pltpu

f32, bf16, u32 = jnp.float32, jnp.bfloat16, jnp.uint32

S, D = 2048, 1024
G = 128
NG = D // G
B = 128
NB = S // B
HEAD = 32

PARAMS = {'RP': 8, 'KSPLIT': 2, 'CH': 128, 'RT': 256, 'FWD_START': 14.0, 'FWD_START0': 14, 'ORDER_F': 'desc', 'PSTEP_F': 4, 'FILL_END': 13.9, 'KVPARTS': 4, 'ORDER': 'asc', 'TI': 4, 'PACE': 1, 'PSTEP': 4, 'NTA': 3, 'NPOS': 2, 'NM0': 4, 'W0FIRST': 1, 'FWD_LAST': 0, 'ZPAIR': 1, 'FILL_END_F': 0.9, 'SKIP': '', 'XG': '1-3-5-8-12-16'}


def _pack_rows(a):
    b = np.asarray(a, dtype=bf16).view(np.uint16).astype(np.uint32)
    return b[0::2] | (b[1::2] << 16)


def _dft_mats(RP):
    ks = np.concatenate([np.arange(0, 128, 2), np.arange(1, 128, 2)])
    sg = np.where(ks % 2 == 0, 1.0, -1.0)[:, None]
    th = (np.pi * (2 * ks + 1) / 256.0)[:, None]
    t = np.arange(128)[None, :]

    def inter(re, im):
        rows = []
        for r in range(128 // RP):
            rows.append(re[r * RP:(r + 1) * RP])
            rows.append(im[r * RP:(r + 1) * RP])
        return np.concatenate(rows, axis=0)

    hre, him = np.cos(th * t), -np.sin(th * t)
    ure, uim = np.cos(th * (t + 0.5)), -np.sin(th * (t + 0.5))
    FU = inter(ure - sg * uim, uim + sg * ure)
    FH = inter(hre, him)
    phi = th * (np.arange(64)[None, :] + 0.5)
    C1 = ((np.cos(phi) + sg * np.sin(phi)) / 256.0).T
    C2 = ((sg * np.cos(phi) - np.sin(phi)) / 256.0).T
    fwd = np.concatenate([_pack_rows(FU), _pack_rows(FH)], axis=0)
    inv = np.concatenate([_pack_rows(C1), _pack_rows(C2)], axis=0)
    return fwd, inv


def _phi(t):
    return jnp.where(t > 0, t + 1.0, jnp.exp(t)) + 1e-6


def _dot(a, b):
    return jnp.dot(a, b, preferred_element_type=f32)


def _bc(x):
    return pltpu.bitcast(x, bf16)


def _ld(ref, *idx):
    *lead, (r0, n) = idx
    return _bc(ref.bitcast(u32)[(*lead, pl.ds(r0 // 2, n // 2), slice(None))])


def make_kernel(P):
    RP, KSPLIT, CH, RT = P['RP'], P['KSPLIT'], P['CH'], P['RT']
    NR = 128 // RP
    NCH = S // CH
    NT = S // RT
    NTA = P['NTA']
    NSTEPS = NG + 1 + (NT - NTA)
    X_GROUPS = []
    bnds = [int(v) for v in P['XG'].split('-')]
    for lo, hi in zip(bnds[:-1], bnds[1:]):
        X_GROUPS.append((list(range(lo, hi)), ('v', lo - 1)))

    def kernel(q_hbm, k_hbm, v_hbm, sk_hbm, h_hbm, d_hbm, f_hbm, fi_hbm, x_hbm, w_hbm, wo_hbm, o_hbm,
               qs, ks, vs, sks, hs, ds_, fs, fis, xs, ws, wos, wcur,
               u_s, U_s, H_s, G_s, Z_s, oa_s, pk_s, v_s, pq_s, kv_s, z_s, M_s, zb_s, ob_s, pqn_s,
               sem_c, sem_x, sem_w, sem_a, sem_q, sem_wo, sem_oa, sem_ob):
        step = pl.program_id(0)
        q32, k32, v32, h32 = (r.bitcast(u32) for r in (q_hbm, k_hbm, v_hbm, h_hbm))
        x32, w32, wo32 = (r.bitcast(u32) for r in (x_hbm, w_hbm, wo_hbm))

        def col(g):
            return pl.ds(pl.multiple_of(g * G, G), G)

        def cp_consts():
            return [pltpu.make_async_copy(a, b, sem_c.at[n]) for n, (a, b) in
                    enumerate(((f_hbm, fs), (fi_hbm, fis), (sk_hbm, sks), (d_hbm, ds_)))]

        def cp_x(c):
            rows = pl.ds(c * (CH // 2), CH // 2)
            return pltpu.make_async_copy(x32.at[rows], xs.at[rows], sem_x.at[c])

        def cp_w(g, p):
            gs = min(g, NG - 1) if isinstance(g, int) else jnp.minimum(g, NG - 1)
            cols = pl.ds(p * D + gs * G if isinstance(gs, int) else pl.multiple_of(p * D + gs * G, G), G)
            return pltpu.make_async_copy(w32.at[:, cols], ws.at[g, p], sem_w.at[3 * g + p])

        def cp_a(g):
            return [pltpu.make_async_copy(k32.at[:, col(g)], ks.at[g, pl.ds(8, S // 2)], sem_a.at[g]),
                    pltpu.make_async_copy(v32.at[:, col(g)], vs.at[g], sem_a.at[g]),
                    pltpu.make_async_copy(h32.at[pl.ds(pl.multiple_of(g * (G // 2), G // 2), G // 2)], hs.at[g], sem_a.at[g])]

        def cp_q(g):
            return pltpu.make_async_copy(q32.at[:, col(g)], qs.at[g], sem_q.at[g])

        def cp_wo():
            return pltpu.make_async_copy(wo32, wos, sem_wo.at[0])

        def cp_oa(g):
            return pltpu.make_async_copy(oa_s.at[g], o_hbm.at[:, col(g)], sem_oa.at[g])

        def cp_ob(t, j):
            rows = pl.ds(t * RT if isinstance(t, int) else pl.multiple_of(t * RT, RT), RT)
            return pltpu.make_async_copy(ob_s.at[t, j], o_hbm.at[rows, pl.ds(D + j * G, G)], sem_ob.at[t])

        def a_pre(g, sk, j):
            w0 = 8 + j * (B // 2)
            n = B // 2
            lo = lambda x: pltpu.bitcast(lax.shift_left(x, u32(16)), f32)
            hi = lambda x: pltpu.bitcast(x & u32(0xFFFF0000), f32)
            k0, k1, k2 = (ks[g, pl.ds(w0 - d, n), :] for d in range(3))
            e0, o0, e1, o1, o2 = lo(k0), hi(k0), lo(k1), hi(k1), hi(k2)
            s0, s1, s2, s3 = (sk[t:t + 1, :] for t in range(4))
            ye = e0 * s0 + o1 * s1 + e1 * s2 + o2 * s3
            yo = o0 * s0 + e0 * s1 + o1 * s2 + e1 * s3
            vv = vs[g, pl.ds(j * n, n), :]
            u = pltpu.bitcast(pltpu.pack_elementwise([ye * lo(vv), yo * hi(vv)], packed_dtype=bf16), u32)
            u_s[pl.ds(j * n, n), :] = u
            return _bc(u)

        def a_fwd(g, sk, j0):
            u2 = jnp.concatenate([a_pre(g, sk, j0), a_pre(g, sk, j0 + 1)], axis=1)
            U2 = _dot(_bc(fs[0:128, :]), u2)
            h2 = jnp.concatenate([_bc(hs[g, :, pl.ds((j0 + d) * B, B)]) for d in range(2)], axis=0)
            H2 = lax.dot_general(_bc(fs[128:256, :]), h2, (((1,), (1,)), ((), ())), preferred_element_type=f32)
            for d in range(2):
                j = j0 + d
                U_s[j] = U2[:, d * G:(d + 1) * G]
                H = H2[:, d * G:(d + 1) * G]
                if j == 0:
                    G_s[0] = H
                else:
                    for r in range(NR):
                        a, b = 2 * r * RP, (2 * r + 1) * RP
                        hre, him = H[a:a + RP], H[b:b + RP]
                        if d == 0:
                            pre, pim = H_s[pl.ds(a, RP), :], H_s[pl.ds(b, RP), :]
                        else:
                            pre, pim = H2[a:a + RP, 0:G], H2[b:b + RP, 0:G]
                        if r < NR // 2:
                            G_s[j, pl.ds(a, RP), :] = hre - pim
                            G_s[j, pl.ds(b, RP), :] = him + pre
                        else:
                            G_s[j, pl.ds(a, RP), :] = hre + pim
                            G_s[j, pl.ds(b, RP), :] = him - pre
            if j0 + 2 < NB:
                H_s[...] = H2[:, G:2 * G]

        def load_sk(g):
            return sks[:, col(g)].astype(f32)

        def load_d(g):
            dall = ds_[...].astype(f32)
            return jnp.sum(jnp.where(lax.broadcasted_iota(jnp.int32, (8, G), 0) == g, dall, 0.0), axis=0, keepdims=True)

        held = {}

        def a_piece(i0, r, dep=None):
            a, b = 2 * r * RP, (2 * r + 1) * RP
            T = P['TI']
            acc = [(dep, dep)] * T
            gw = {}
            for j in range(i0 + T):
                ure, uim = U_s[j, pl.ds(a, RP), :], U_s[j, pl.ds(b, RP), :]
                for t in range(T):
                    m = i0 + t - j
                    if m < 0:
                        continue
                    if m not in gw:
                        gw[m] = (G_s[m, pl.ds(a, RP), :], G_s[m, pl.ds(b, RP), :])
                    gre, gim = gw[m]
                    tre = gre * ure - gim * uim
                    tim = gre * uim + gim * ure
                    zre, zim = acc[t]
                    acc[t] = (tre if zre is None else zre + tre, tim if zim is None else zim + tim)
            if P['ZPAIR'] and RP == 8:
                if r % 2 == 0:
                    held[(i0, r)] = acc
                else:
                    prev = held.pop((i0, r - 1))
                    for t in range(T):
                        for c in range(2):
                            z = jnp.concatenate([prev[t][c], acc[t][c]], axis=0)
                            Z_s[i0 + t, c, pl.ds((r - 1) * RP, 2 * RP), :] = z.astype(bf16)
            else:
                for t in range(T):
                    Z_s[i0 + t, 0, pl.ds(r * RP, RP), :] = acc[t][0].astype(bf16)
                    Z_s[i0 + t, 1, pl.ds(r * RP, RP), :] = acc[t][1].astype(bf16)

        def a_inv(g, dvec, i0):
            e2 = _dot(_bc(fis[0:32, :]), jnp.concatenate([_ld(Z_s, i0 + d, 0, (0, 128)) for d in range(2)], axis=1))
            o2 = _dot(_bc(fis[32:64, :]), jnp.concatenate([_ld(Z_s, i0 + d, 1, (0, 128)) for d in range(2)], axis=1))
            rev = 7 - lax.broadcasted_iota(jnp.int32, (8, G), 0)
            for d in range(2):
                r0 = (i0 + d) * B
                e, o = e2[:, d * G:(d + 1) * G], o2[:, d * G:(d + 1) * G]
                hi = e - o
                ycv = jnp.concatenate(
                    [e + o] + [jnp.take_along_axis(hi[8 * (7 - v):8 * (8 - v)], rev, axis=0) for v in range(8)], axis=0)
                uu = _bc(u_s[pl.ds(r0 // 2, B // 2), :]).astype(f32)
                y = ycv + uu * dvec
                qq = _bc(qs[g, pl.ds(r0 // 2, B // 2), :]).astype(f32)
                oa_s[g, pl.ds(r0, B), :] = (qq * y).astype(bf16)

        def emit(mm, state, ga, t_fill_end, order, pstep):
            pieces = []
            TI = P['TI']
            if ga is not None:
                dvec = load_d(ga)
                GS = max(2, TI)
                pairs = list(range(0, NB, GS))
                if order == 'desc':
                    pairs = pairs[::-1]
                elif order == 'mix':
                    lo, hi = pairs[:len(pairs) // 2], pairs[len(pairs) // 2:][::-1]
                    pairs = [b for pair in zip(hi, lo) for b in pair]
                for i0 in pairs:
                    pp = [(i, r) for r in range(NR) for i in range(i0, i0 + GS, TI)]
                    pieces += [(i, r, list(range(i0, i0 + GS, 2)) if n == len(pp) - 1 else None) for n, (i, r) in enumerate(pp)]
            pcost = lambda i: sum(ii + 1 for ii in range(i, i + TI))
            tot_p = sum(pcost(p[0]) for p in pieces)
            T = 0
            done_cost = 0
            pi = 0
            pend_inv = []
            for (cost, fn, tag) in mm:
                if tag == 'fwd':
                    assert pi == len(pieces) and not pend_inv, "fwd for next tile would overwrite live U/G/u"
                fn()
                T += cost
                for i0 in pend_inv:
                    a_inv(ga, dvec, i0)
                    T += 64
                pend_inv = []
                target = tot_p * min(1.0, T / t_fill_end)
                kk = 0
                while pi < len(pieces) and done_cost < target:
                    i, r, fin = pieces[pi]
                    dep = None
                    if P['PACE'] and 'pace' in state:
                        pace = state['pace']
                        idx = min(pace.shape[0] // RP - 1, kk * pstep * 8 // RP)
                        pv = pltpu.bitcast(pace[idx * RP:(idx + 1) * RP, :], u32)
                        dep = pltpu.bitcast(lax.shift_right_logical(lax.shift_right_logical(pv, u32(16)), u32(16)), f32)
                        kk += 1
                    a_piece(i, r, dep)
                    done_cost += pcost(i)
                    pi += 1
                    if fin is not None:
                        pend_inv.extend(fin)
            assert pi == len(pieces) and not pend_inv
            if ga is not None:
                cp_oa(ga).start()

        def group_step(g, ga, first):
            KS = D // KSPLIT
            state = {}

            hooks = {}

            def proj_part(name, p, c, ks_):
                x = _bc(xs[pl.ds(c * CH // 2, CH // 2), pl.ds(ks_ * KS, KS)])
                if first:
                    w = _bc(ws[g, p, pl.ds(ks_ * KS // 2, KS // 2), :])
                else:
                    w = _bc(wcur[p, pl.ds(ks_ * KS // 2, KS // 2), :])
                part = _dot(x, w)
                state[name] = part if ks_ == 0 else state[name] + part
                state['pace'] = part
                if ks_ == KSPLIT - 1:
                    for h in hooks.get((name, c), []):
                        h()

            def fin_k(c):
                pk = _phi(state.pop('k'))
                pk_s[pl.ds(c * CH, CH), :] = pk.astype(bf16)
                zp = jnp.sum(pk.reshape(CH // 8, 8, G), axis=0)
                state['z'] = zp if c == 0 else state['z'] + zp

            def fin_v(c):
                v_s[pl.ds(c * CH, CH), :] = state.pop('v').astype(bf16)
                if c == NCH - 1:
                    next_w(1)
                    next_w(2)

            def next_w(p):
                if not first:
                    wcur[p] = ws[g + 1, p]

            def fin_q(c):
                pq_s[g, pl.ds(c * CH, CH), :] = _phi(state.pop('q')).astype(bf16)
                if c == NCH - 1:
                    next_w(0)

            def kv_part(n):
                if 'kv' in P['SKIP']:
                    if n == P['KVPARTS'] - 1:
                        kv_s[g] = jnp.zeros((G, G), f32) + state['pace'][0:G, :]
                        z_s[g] = state.pop('z')
                    return
                rows = S // P['KVPARTS']
                a = _ld(pk_s, (n * rows, rows))
                b = _ld(v_s, (n * rows, rows))
                part = lax.dot_general(a, b, (((0,), (0,)), ((), ())), preferred_element_type=f32)
                state['kv'] = part if n == 0 else state['kv'] + part
                if n == P['KVPARTS'] - 1:
                    kv_s[g] = state.pop('kv')
                    z_s[g] = state.pop('z')

            def fwd_task(j):
                if 'fwd' in P['SKIP']:
                    return
                if j == 0:
                    state['sk'] = load_sk(g)
                a_fwd(g, state['sk'], j)

            def wait_all(cps, nm="w"):
                if True:
                    for c in cps:
                        c.wait()

            fwd_start = P['FWD_START0'] if first else P['FWD_START']
            c_fw0 = int(fwd_start * NCH / 16)
            def wait_late():
                cps = cp_a(g)
                if first:
                    cps = cp_consts() + cps
                if not first:
                    cps = cps + [cp_w(g + 1, p) for p in (1, 2, 0)]
                wait_all(cps, 'a')

            if c_fw0 < NCH:
                hooks.setdefault(('k', c_fw0), []).append(wait_late)
            else:
                hooks.setdefault(('q', NCH - 1), []).append(wait_late)
            if first:
                if not P['W0FIRST']:
                    hooks.setdefault(('k', 0), []).append(lambda: wait_all([cp_w(g, 2)], 'wv'))
                    hooks.setdefault(('v', 0), []).append(lambda: wait_all([cp_w(g, 0)], 'wq'))
                for grp, at in X_GROUPS:
                    hooks.setdefault(at, []).append(functools.partial(lambda grp: wait_all([cp_x(c) for c in grp], 'x%d' % grp[0]), grp))

            mm = []
            pc = CH * 8 // KSPLIT // 4
            nfw = NCH - c_fw0
            fwd_sched = {}
            for j in range(0, NB, 2):
                fwd_sched.setdefault(c_fw0 + j * nfw // NB, []).append(j)
            t_fill_end = None
            for c in range(NCH):
                if c == int(P['FILL_END'] * NCH / 16):
                    frac = P['FILL_END'] * NCH / 16 - c
                    t_fill_end = sum(m[0] for m in mm) + frac * 3 * KSPLIT * pc
                fw = list(fwd_sched.get(c, []))
                for name, p, fin in (('k', 1, fin_k), ('v', 2, fin_v)):
                    for ks_ in range(KSPLIT):
                        def t(name=name, p=p, c=c, ks_=ks_, fin=fin):
                            proj_part(name, p, c, ks_)
                            if ks_ == KSPLIT - 1:
                                fin(c)
                        mm.append((pc, t, None))
                    if fw:
                        ntake = (len(fw) + 1) // 2 if name == 'k' else len(fw)
                        for j in fw[:ntake]:
                            mm.append((256, functools.partial(fwd_task, j), 'fwd'))
                        fw = fw[ntake:]
                if c >= 1:
                    for ks_ in range(KSPLIT):
                        def t(c=c - 1, ks_=ks_):
                            proj_part('q', 0, c, ks_)
                            if ks_ == KSPLIT - 1:
                                fin_q(c)
                        mm.append((pc, t, None))
                per = NCH // P['KVPARTS']
                if (c + 1) % per == 0:
                    mm.append((512 // P['KVPARTS'], functools.partial(kv_part, c // per), None))
            for ks_ in range(KSPLIT):
                def t(c=NCH - 1, ks_=ks_):
                    proj_part('q', 0, c, ks_)
                    if ks_ == KSPLIT - 1:
                        fin_q(c)
                mm.append((pc, t, None))
            for j in fwd_sched.get(NCH, []):
                mm.append((256, functools.partial(fwd_task, j), 'fwd'))
            if P['FWD_LAST']:
                fw_idx = [n for n, m in enumerate(mm) if m[2] == 'fwd'][-P['FWD_LAST']:]
                moved = [mm[n] for n in fw_idx]
                mm = [m for n, m in enumerate(mm) if n not in fw_idx] + moved
            emit(mm, state, ga, t_fill_end, P['ORDER'], P['PSTEP'])
            if first:
                wait_all([cp_w(1, p) for p in (1, 2, 0)], 'w1')
                for p in range(3):
                    wcur[p] = ws[1, p]

        def tile_rows(t):
            t0 = t * (RT // 2)
            return pl.ds(t0 if isinstance(t, int) else pl.multiple_of(t0, RT // 2), RT // 2)

        def norm_tasks(t, state):
            pq32 = pq_s.bitcast(u32)

            def norm(gs):
                for g in gs:
                    pq = _bc(pq32[g, tile_rows(t), :])
                    den = _dot(pq, _ld(zb_s, g, (0, G))) + 1e-6
                    pqn_s[g] = (pq.astype(f32) * pl.reciprocal(den, approx=True)).astype(bf16)
                    state['pace'] = den
            return [(RT, functools.partial(norm, range(0, 4)), None), (RT, functools.partial(norm, range(4, 8)), None)]

        def proj_tasks(t, state):
            loc = {}

            def proj(j):
                if 'lhs' not in loc:
                    loc['lhs'] = jnp.concatenate([_ld(pqn_s, g, (0, RT)) for g in range(NG)], axis=1)
                res = _dot(loc['lhs'], _ld(M_s, j, (0, D)))
                ob_s[t, j] = res.astype(bf16)
                state['pace'] = res
                cp_ob(t, j).start()
            return [(2 * RT, functools.partial(proj, j), None) for j in range(NG)]

        def tile_tasks(t, state, norm_next):
            pr = proj_tasks(t, state)
            if not norm_next:
                return pr
            nm = norm_tasks(t + 1, state)
            a, b = P['NPOS'], P['NPOS'] + 2
            return pr[:a] + nm[:1] + pr[a:b] + nm[1:] + pr[b:]

        def m_tasks():
            r = lax.broadcasted_iota(jnp.int32, (G, G), 0) // HEAD
            c = lax.broadcasted_iota(jnp.int32, (G, G), 1) // HEAD
            bd = r == c

            def mt(g):
                z = jnp.sum(z_s[g], axis=0, keepdims=True)
                zc = jnp.broadcast_to(z, (G, G)).T
                zb_s[g] = jnp.where(bd, zc, 0.0).astype(bf16)
                kvb = jnp.where(bd, kv_s[g], 0.0).astype(bf16)
                wo = _bc(wos[pl.ds(g * G // 2, G // 2), :])
                Mg = _dot(kvb, wo)
                for j in range(NG):
                    M_s[j, pl.ds(g * G, G), :] = Mg[:, j * G:(j + 1) * G].astype(bf16)
            return [(256, functools.partial(mt, g), None) for g in range(NG)]

        @pl.when(step == 0)
        def _():
            ks[:, 0:8, :] = jnp.zeros((NG, 8, G), u32)
            cp_w(0, 1).start()
            if P['W0FIRST']:
                cp_w(0, 2).start()
                cp_w(0, 0).start()
                cp_x(0).start()
            else:
                cp_x(0).start()
                cp_w(0, 2).start()
                cp_w(0, 0).start()
            for c in range(1, NCH):
                cp_x(c).start()
            for c in cp_consts():
                c.start()
            for c in cp_a(0):
                c.start()
            for g in range(1, NG + 1):
                for p in (1, 2, 0):
                    cp_w(g, p).start()
                cp_q(g - 1).start()
                if g < NG:
                    for c in cp_a(g):
                        c.start()
            cp_wo().start()
            if True:
                cp_w(0, 1).wait()
                if P['W0FIRST']:
                    cp_w(0, 2).wait()
                    cp_w(0, 0).wait()
                cp_x(0).wait()
            group_step(0, None, True)

        @pl.when(jnp.logical_and(step > 0, step < NG))
        def _():
            cp_q(step - 1).wait()
            group_step(step, step - 1, False)

        @pl.when(step == NG)
        def _():
            cp_wo().wait()
            cp_q(NG - 1).wait()
            state = {}
            mt = m_tasks()
            nm = norm_tasks(0, state)
            mm = mt[:P['NM0']] + nm[:1] + mt[P['NM0']:] + nm[1:] if P['NM0'] < NG else mt + nm
            for t in range(NTA):
                mm += tile_tasks(t, state, True)
            emit(mm, state, NG - 1, sum(m[0] for m in mm) * P['FILL_END_F'], P['ORDER_F'], P['PSTEP_F'])

        @pl.when(jnp.logical_and(step > NG, step < NSTEPS - 1))
        def _():
            state = {}
            for (_, fn, _) in tile_tasks(step - (NG + 1) + NTA, state, True):
                fn()

        @pl.when(step == NSTEPS - 1)
        def _():
            state = {}
            for (_, fn, _) in tile_tasks(NT - 1, state, False):
                fn()
            for g in range(NG):
                cp_oa(g).wait()
            for t in range(NT):
                for j in range(NG):
                    cp_ob(t, j).wait()

    scratch = [
        pltpu.VMEM((NG, S // 2, G), u32), pltpu.VMEM((NG, 8 + S // 2, G), u32), pltpu.VMEM((NG, S // 2, G), u32),
        pltpu.VMEM((4, D), bf16), pltpu.VMEM((NG, G // 2, S), u32), pltpu.VMEM((8, 128), bf16),
        pltpu.VMEM((256, 128), u32), pltpu.VMEM((64, 128), u32),
        pltpu.VMEM((S // 2, D), u32), pltpu.VMEM((NG + 1, 3, D // 2, G), u32), pltpu.VMEM((D // 2, D), u32),
        pltpu.VMEM((3, D // 2, G), u32),
        pltpu.VMEM((S // 2, G), u32),
        pltpu.VMEM((NB, 256, G), f32), pltpu.VMEM((256, G), f32), pltpu.VMEM((NB, 256, G), f32),
        pltpu.VMEM((NB, 2, 128, G), bf16), pltpu.VMEM((NG, S, G), bf16),
        pltpu.VMEM((S, G), bf16), pltpu.VMEM((S, G), bf16), pltpu.VMEM((NG, S, G), bf16),
        pltpu.VMEM((NG, G, G), f32), pltpu.VMEM((NG, 8, G), f32),
        pltpu.VMEM((NG, D, G), bf16), pltpu.VMEM((NG, G, G), bf16), pltpu.VMEM((NT, NG, RT, G), bf16),
        pltpu.VMEM((NG, RT, G), bf16),
        pltpu.SemaphoreType.DMA((4,)), pltpu.SemaphoreType.DMA((NCH,)), pltpu.SemaphoreType.DMA((3 * (NG + 1),)),
        pltpu.SemaphoreType.DMA((NG,)), pltpu.SemaphoreType.DMA((NG,)), pltpu.SemaphoreType.DMA((1,)),
        pltpu.SemaphoreType.DMA((NG,)), pltpu.SemaphoreType.DMA((NT,)),
    ]
    return kernel, scratch, NSTEPS


_KERNEL, _SCRATCH, _NSTEPS = make_kernel(PARAMS)
_FP, _FIP = _dft_mats(PARAMS['RP'])


@jax.jit
def pallas_concat_heads__ssm_conv_h3__linear_attn_block__prompt_kernel(A_q, A_k, A_v, A_shift_k, A_ssm_k, A_ssm_D, B_x, B_wqkv, B_wo):
    out = pl.pallas_call(
        _KERNEL, grid=(_NSTEPS,),
        in_specs=[pl.BlockSpec(memory_space=pl.ANY)] * 11,
        out_specs=pl.BlockSpec(memory_space=pl.ANY),
        out_shape=jax.ShapeDtypeStruct((S, 2 * D), bf16),
        scratch_shapes=_SCRATCH,
        compiler_params=pltpu.CompilerParams(vmem_limit_bytes=110 * 1024 * 1024, dimension_semantics=("arbitrary",)),
    )(A_q.reshape(S, D), A_k.reshape(S, D), A_v.reshape(S, D), A_shift_k.T, A_ssm_k, A_ssm_D.reshape(8, 128),
      jnp.asarray(_FP), jnp.asarray(_FIP), B_x.reshape(S, D), B_wqkv, B_wo)
    return out.reshape(1, S, 2 * D)
```

```python
import functools
import numpy as np
import jax
import jax.numpy as jnp
from jax import lax
from jax.experimental import pallas as pl
from jax.experimental.pallas import tpu as pltpu

f32, bf16, u32 = jnp.float32, jnp.bfloat16, jnp.uint32

S, D = 2048, 1024
G = 128
NG = D // G
B = 128
NB = S // B
HEAD = 32

PARAMS = {'RP': 8, 'KSPLIT': 2, 'CH': 128, 'RT': 256, 'FWD_START': 14.0, 'FWD_START0': 14.0, 'ORDER_F': 'desc', 'PSTEP_F': 8, 'FILL_END': 13.9, 'KVPARTS': 4, 'ORDER': 'asc', 'TI': 4, 'PACE': 1, 'PSTEP': 4, 'NTA': 4, 'NPOS': 2, 'NM0': 6, 'W0FIRST': 1, 'QLAG': 1, 'FWD_END': 16.0, 'ZPAIR': 1, 'FILL_END_F': 0.9, 'SKIP': '', 'XG': '1-2-4-7-11-16'}


def _pack_rows(a):
    b = np.asarray(a, dtype=bf16).view(np.uint16).astype(np.uint32)
    return b[0::2] | (b[1::2] << 16)


def _dft_mats(RP):
    ks = np.concatenate([np.arange(0, 128, 2), np.arange(1, 128, 2)])
    sg = np.where(ks % 2 == 0, 1.0, -1.0)[:, None]
    th = (np.pi * (2 * ks + 1) / 256.0)[:, None]
    t = np.arange(128)[None, :]

    def inter(re, im):
        rows = []
        for r in range(128 // RP):
            rows.append(re[r * RP:(r + 1) * RP])
            rows.append(im[r * RP:(r + 1) * RP])
        return np.concatenate(rows, axis=0)

    hre, him = np.cos(th * t), -np.sin(th * t)
    ure, uim = np.cos(th * (t + 0.5)), -np.sin(th * (t + 0.5))
    FU = inter(ure - sg * uim, uim + sg * ure)
    FH = inter(hre, him)
    phi = th * (np.arange(64)[None, :] + 0.5)
    C1 = ((np.cos(phi) + sg * np.sin(phi)) / 256.0).T
    C2 = ((sg * np.cos(phi) - np.sin(phi)) / 256.0).T
    fwd = np.concatenate([_pack_rows(FU), _pack_rows(FH)], axis=0)
    inv = np.concatenate([_pack_rows(C1), _pack_rows(C2)], axis=0)
    return fwd, inv


def _phi(t):
    return jnp.where(t > 0, t + 1.0, jnp.exp(t)) + 1e-6


def _dot(a, b):
    return jnp.dot(a, b, preferred_element_type=f32)


def _bc(x):
    return pltpu.bitcast(x, bf16)


def _ld(ref, *idx):
    *lead, (r0, n) = idx
    return _bc(ref.bitcast(u32)[(*lead, pl.ds(r0 // 2, n // 2), slice(None))])


def make_kernel(P):
    RP, KSPLIT, CH, RT = P['RP'], P['KSPLIT'], P['CH'], P['RT']
    NR = 128 // RP
    NCH = S // CH
    NT = S // RT
    NTA = P['NTA']
    NSTEPS = NG + 1 + (NT - NTA)
    X_GROUPS = []
    bnds = [int(v) for v in P['XG'].split('-')]
    for lo, hi in zip(bnds[:-1], bnds[1:]):
        X_GROUPS.append((list(range(lo, hi)), lo))

    def kernel(q_hbm, k_hbm, v_hbm, sk_hbm, h_hbm, d_hbm, f_hbm, fi_hbm, x_hbm, w_hbm, wo_hbm, o_hbm,
               qs, ks, vs, sks, hs, ds_, fs, fis, xs, ws, wos, wvs, wcur,
               u_s, U_s, H_s, G_s, Z_s, oa_s, pk_s, gm_s, pq_s, z_s, M_s, zb_s, ob_s, pqn_s,
               sem_c, sem_x, sem_w, sem_a, sem_q, sem_wo, sem_oa, sem_ob):
        step = pl.program_id(0)
        q32, k32, v32, h32 = (r.bitcast(u32) for r in (q_hbm, k_hbm, v_hbm, h_hbm))
        x32, w32, wo32 = (r.bitcast(u32) for r in (x_hbm, w_hbm, wo_hbm))

        def col(g):
            return pl.ds(pl.multiple_of(g * G, G), G)

        def cp_consts():
            return [pltpu.make_async_copy(a, b, sem_c.at[n]) for n, (a, b) in
                    enumerate(((f_hbm, fs), (fi_hbm, fis), (sk_hbm, sks), (d_hbm, ds_)))]

        def cp_x(c):
            rows = pl.ds(c * (CH // 2), CH // 2)
            return pltpu.make_async_copy(x32.at[rows], xs.at[rows], sem_x.at[c])

        def cp_w(g, p):
            gs = min(g, NG - 1) if isinstance(g, int) else jnp.minimum(g, NG - 1)
            off = (D, 0)[p]
            cols = pl.ds(off + gs * G if isinstance(gs, int) else pl.multiple_of(off + gs * G, G), G)
            return pltpu.make_async_copy(w32.at[:, cols], ws.at[g, p], sem_w.at[2 * g + p])

        def cp_a(g):
            return [pltpu.make_async_copy(k32.at[:, col(g)], ks.at[g, pl.ds(8, S // 2)], sem_a.at[g]),
                    pltpu.make_async_copy(v32.at[:, col(g)], vs.at[g], sem_a.at[g]),
                    pltpu.make_async_copy(h32.at[pl.ds(pl.multiple_of(g * (G // 2), G // 2), G // 2)], hs.at[g], sem_a.at[g])]

        def cp_q(g):
            return pltpu.make_async_copy(q32.at[:, col(g)], qs.at[g], sem_q.at[g])

        def cp_wo():
            return [pltpu.make_async_copy(wo32, wos, sem_wo.at[0]),
                    pltpu.make_async_copy(w32.at[:, pl.ds(2 * D, D)], wvs, sem_wo.at[1])]

        def cp_oa(g):
            return pltpu.make_async_copy(oa_s.at[g], o_hbm.at[:, col(g)], sem_oa.at[g])

        def cp_ob(t, j):
            rows = pl.ds(t * RT if isinstance(t, int) else pl.multiple_of(t * RT, RT), RT)
            return pltpu.make_async_copy(ob_s.at[t, j], o_hbm.at[rows, pl.ds(D + j * G, G)], sem_ob.at[t])

        def a_pre(g, sk, j):
            w0 = 8 + j * (B // 2)
            n = B // 2
            lo = lambda x: pltpu.bitcast(lax.shift_left(x, u32(16)), f32)
            hi = lambda x: pltpu.bitcast(x & u32(0xFFFF0000), f32)
            k0, k1, k2 = (ks[g, pl.ds(w0 - d, n), :] for d in range(3))
            e0, o0, e1, o1, o2 = lo(k0), hi(k0), lo(k1), hi(k1), hi(k2)
            s0, s1, s2, s3 = (sk[t:t + 1, :] for t in range(4))
            ye = e0 * s0 + o1 * s1 + e1 * s2 + o2 * s3
            yo = o0 * s0 + e0 * s1 + o1 * s2 + e1 * s3
            vv = vs[g, pl.ds(j * n, n), :]
            u = pltpu.bitcast(pltpu.pack_elementwise([ye * lo(vv), yo * hi(vv)], packed_dtype=bf16), u32)
            u_s[pl.ds(j * n, n), :] = u
            return _bc(u)

        def a_fwd(g, sk, j0):
            u2 = jnp.concatenate([a_pre(g, sk, j0), a_pre(g, sk, j0 + 1)], axis=1)
            U2 = _dot(_bc(fs[0:128, :]), u2)
            h2 = jnp.concatenate([_bc(hs[g, :, pl.ds((j0 + d) * B, B)]) for d in range(2)], axis=0)
            H2 = lax.dot_general(_bc(fs[128:256, :]), h2, (((1,), (1,)), ((), ())), preferred_element_type=f32)
            for d in range(2):
                j = j0 + d
                U_s[j] = U2[:, d * G:(d + 1) * G]
                H = H2[:, d * G:(d + 1) * G]
                if j == 0:
                    G_s[0] = H
                else:
                    for r in range(NR):
                        a, b = 2 * r * RP, (2 * r + 1) * RP
                        hre, him = H[a:a + RP], H[b:b + RP]
                        if d == 0:
                            pre, pim = H_s[pl.ds(a, RP), :], H_s[pl.ds(b, RP), :]
                        else:
                            pre, pim = H2[a:a + RP, 0:G], H2[b:b + RP, 0:G]
                        if r < NR // 2:
                            G_s[j, pl.ds(a, RP), :] = hre - pim
                            G_s[j, pl.ds(b, RP), :] = him + pre
                        else:
                            G_s[j, pl.ds(a, RP), :] = hre + pim
                            G_s[j, pl.ds(b, RP), :] = him - pre
            if j0 + 2 < NB:
                H_s[...] = H2[:, G:2 * G]

        def load_sk(g):
            return sks[:, col(g)].astype(f32)

        def load_d(g):
            dall = ds_[...].astype(f32)
            return jnp.sum(jnp.where(lax.broadcasted_iota(jnp.int32, (8, G), 0) == g, dall, 0.0), axis=0, keepdims=True)

        held = {}

        def a_piece(i0, r, dep=None):
            a, b = 2 * r * RP, (2 * r + 1) * RP
            T = P['TI']
            acc = [(dep, dep)] * T
            gw = {}
            for j in range(i0 + T):
                ure, uim = U_s[j, pl.ds(a, RP), :], U_s[j, pl.ds(b, RP), :]
                for t in range(T):
                    m = i0 + t - j
                    if m < 0:
                        continue
                    if m not in gw:
                        gw[m] = (G_s[m, pl.ds(a, RP), :], G_s[m, pl.ds(b, RP), :])
                    gre, gim = gw[m]
                    tre = gre * ure - gim * uim
                    tim = gre * uim + gim * ure
                    zre, zim = acc[t]
                    acc[t] = (tre if zre is None else zre + tre, tim if zim is None else zim + tim)
            if P['ZPAIR'] and RP == 8:
                if r % 2 == 0:
                    held[(i0, r)] = acc
                else:
                    prev = held.pop((i0, r - 1))
                    for t in range(T):
                        for c in range(2):
                            z = jnp.concatenate([prev[t][c], acc[t][c]], axis=0)
                            Z_s[i0 + t, c, pl.ds((r - 1) * RP, 2 * RP), :] = z.astype(bf16)
            else:
                for t in range(T):
                    Z_s[i0 + t, 0, pl.ds(r * RP, RP), :] = acc[t][0].astype(bf16)
                    Z_s[i0 + t, 1, pl.ds(r * RP, RP), :] = acc[t][1].astype(bf16)

        def a_inv(g, dvec, i0):
            e2 = _dot(_bc(fis[0:32, :]), jnp.concatenate([_ld(Z_s, i0 + d, 0, (0, 128)) for d in range(2)], axis=1))
            o2 = _dot(_bc(fis[32:64, :]), jnp.concatenate([_ld(Z_s, i0 + d, 1, (0, 128)) for d in range(2)], axis=1))
            rev = 7 - lax.broadcasted_iota(jnp.int32, (8, G), 0)
            for d in range(2):
                r0 = (i0 + d) * B
                e, o = e2[:, d * G:(d + 1) * G], o2[:, d * G:(d + 1) * G]
                hi = e - o
                ycv = jnp.concatenate(
                    [e + o] + [jnp.take_along_axis(hi[8 * (7 - v):8 * (8 - v)], rev, axis=0) for v in range(8)], axis=0)
                uu = _bc(u_s[pl.ds(r0 // 2, B // 2), :]).astype(f32)
                y = ycv + uu * dvec
                qq = _bc(qs[g, pl.ds(r0 // 2, B // 2), :]).astype(f32)
                oa_s[g, pl.ds(r0, B), :] = (qq * y).astype(bf16)

        def emit(mm, state, ga, t_fill_end, order, pstep):
            pieces = []
            TI = P['TI']
            if ga is not None:
                dvec = load_d(ga)
                GS = max(2, TI)
                pairs = list(range(0, NB, GS))
                if order == 'desc':
                    pairs = pairs[::-1]
                elif order == 'mix':
                    lo, hi = pairs[:len(pairs) // 2], pairs[len(pairs) // 2:][::-1]
                    pairs = [b for pair in zip(hi, lo) for b in pair]
                for i0 in pairs:
                    pp = [(i, r) for r in range(NR) for i in range(i0, i0 + GS, TI)]
                    pieces += [(i, r, list(range(i0, i0 + GS, 2)) if n == len(pp) - 1 else None) for n, (i, r) in enumerate(pp)]
            pcost = lambda i: sum(ii + 1 for ii in range(i, i + TI))
            tot_p = sum(pcost(p[0]) for p in pieces)
            T = 0
            done_cost = 0
            pi = 0
            pend_inv = []
            for (cost, fn, tag) in mm:
                if tag == 'fwd':
                    assert pi == len(pieces) and not pend_inv, "fwd for next tile would overwrite live U/G/u"
                fn()
                T += cost
                for i0 in pend_inv:
                    a_inv(ga, dvec, i0)
                    T += 64
                pend_inv = []
                target = tot_p * min(1.0, T / t_fill_end)
                kk = 0
                while pi < len(pieces) and done_cost < target:
                    i, r, fin = pieces[pi]
                    dep = None
                    if P['PACE'] and 'pace' in state:
                        pace = state['pace']
                        idx = min(pace.shape[0] // RP - 1, kk * pstep * 8 // RP)
                        pv = pltpu.bitcast(pace[idx * RP:(idx + 1) * RP, :], u32)
                        dep = pltpu.bitcast(lax.shift_right_logical(lax.shift_right_logical(pv, u32(16)), u32(16)), f32)
                        kk += 1
                    a_piece(i, r, dep)
                    done_cost += pcost(i)
                    pi += 1
                    if fin is not None:
                        pend_inv.extend(fin)
            assert pi == len(pieces) and not pend_inv
            if ga is not None:
                cp_oa(ga).start()

        def group_step(g, ga, first):
            KS = D // KSPLIT
            NQ = 4
            QR = S // NQ
            GW = D // 4
            state = {}
            hooks = {}

            def proj_part(name, p, c, ks_):
                x = _bc(xs[pl.ds(c * CH // 2, CH // 2), pl.ds(ks_ * KS, KS)])
                if first:
                    w = _bc(ws[g, p, pl.ds(ks_ * KS // 2, KS // 2), :])
                else:
                    w = _bc(wcur[p, pl.ds(ks_ * KS // 2, KS // 2), :])
                part = _dot(x, w)
                state[name] = part if ks_ == 0 else state[name] + part
                state['pace'] = part
                if ks_ == KSPLIT - 1:
                    for h in hooks.get((name, c), []):
                        h()

            def next_w(p):
                if not first:
                    wcur[p] = ws[g + 1, p]

            def fin_k(c):
                pk = _phi(state.pop('k'))
                pk_s[pl.ds(c * CH, CH), :] = pk.astype(bf16)
                zp = jnp.sum(pk.reshape(CH // 8, 8, G), axis=0)
                state['z'] = zp if c == 0 else state['z'] + zp
                if c == NCH - 1:
                    z_s[g] = state.pop('z')
                    next_w(0)

            def fin_q(c):
                pq_s[g, pl.ds(c * CH, CH), :] = _phi(state.pop('q')).astype(bf16)
                if c == NCH - 1:
                    next_w(1)

            def g_task(n, h):
                a = _ld(pk_s, (n * QR, QR))
                b = _bc(xs[pl.ds(n * QR // 2, QR // 2), pl.ds(h * GW, GW)])
                part = lax.dot_general(a, b, (((0,), (0,)), ((), ())), preferred_element_type=f32)
                state['pace'] = part[:, 0:G]
                acc = part if n == 0 else state[('G', h)] + part
                if n < NQ - 1:
                    state[('G', h)] = acc
                else:
                    for d in range(GW // G):
                        gm_s[g, h * (GW // G) + d] = acc[:, d * G:(d + 1) * G].astype(bf16)

            def fwd_task(j):
                if j == 0:
                    state['sk'] = load_sk(g)
                a_fwd(g, state['sk'], j)

            def wait_all(cps, nm="w"):
                if True:
                    for c in cps:
                        c.wait()

            def wait_late():
                cps = cp_a(g)
                if first:
                    cps = cp_consts() + cps
                else:
                    cps = cps + [cp_w(g + 1, p) for p in range(2)]
                wait_all(cps, 'a')

            pc = CH * 8 // KSPLIT // 4
            units = []

            def add_proj(name, p, c, fin):
                for ks_ in range(KSPLIT):
                    def t(ks_=ks_):
                        proj_part(name, p, c, ks_)
                        if ks_ == KSPLIT - 1:
                            fin(c)
                    units.append((pc, t, (name, c)))

            cq = CH * NQ // S if False else None
            per = NCH // NQ
            gq = [(n, h) for n in range(NQ) for h in range(4)]
            gi = 0
            for c in range(NCH):
                add_proj('k', 0, c, fin_k)
                if c >= per and (c % per) * 4 // per != ((c - 1) % per) * 4 // per or (c >= per and c % per == 0):
                    n, h = gq[gi]
                    assert n < c // per
                    units.append((256, functools.partial(g_task, n, h), ('G', gi)))
                    gi += 1
                if c >= P['QLAG']:
                    add_proj('q', 1, c - P['QLAG'], fin_q)
            rest_q = list(range(NCH - P['QLAG'], NCH))
            while gi < len(gq) or rest_q:
                if rest_q:
                    add_proj('q', 1, rest_q.pop(0), fin_q)
                if gi < len(gq):
                    n, h = gq[gi]
                    units.append((256, functools.partial(g_task, n, h), ('G', gi)))
                    gi += 1

            total = sum(u[0] for u in units)
            fwd_start = (P['FWD_START0'] if first else P['FWD_START']) / 16.0 * total
            t_fill_end = P['FILL_END'] / 16.0 * total
            fwd_end = P['FWD_END'] / 16.0 * total
            pos = [fwd_start + (fwd_end - fwd_start) * n / (NB // 2) for n in range(NB // 2)]
            mm = []
            T = 0
            nf = 0
            last_proj = None
            hooked = False
            for (cost, fn, tag) in units:
                while nf < len(pos) and T >= pos[nf]:
                    if not hooked:
                        hooks.setdefault(last_proj, []).append(wait_late)
                        hooked = True
                    mm.append((256, functools.partial(fwd_task, 2 * nf), 'fwd'))
                    nf += 1
                mm.append((cost, fn, None))
                T += cost
                if tag[0] in ('k', 'q'):
                    last_proj = tag
            if not hooked:
                hooks.setdefault(last_proj, []).append(wait_late)
            while nf < len(pos):
                mm.append((256, functools.partial(fwd_task, 2 * nf), 'fwd'))
                nf += 1
            if first:
                for grp, lo in X_GROUPS:
                    hooks.setdefault(('k', lo - 1), []).append(
                        functools.partial(lambda grp: wait_all([cp_x(c) for c in grp], 'x%d' % grp[0]), grp))
            emit(mm, state, ga, t_fill_end, P['ORDER'], P['PSTEP'])
            if first:
                wait_all([cp_w(1, p) for p in range(2)], 'w1')
                for p in range(2):
                    wcur[p] = ws[1, p]

        def tile_rows(t):
            t0 = t * (RT // 2)
            return pl.ds(t0 if isinstance(t, int) else pl.multiple_of(t0, RT // 2), RT // 2)

        def norm_tasks(t, state):
            pq32 = pq_s.bitcast(u32)

            def norm(gs):
                for g in gs:
                    pq = _bc(pq32[g, tile_rows(t), :])
                    den = _dot(pq, _ld(zb_s, g, (0, G))) + 1e-6
                    pqn_s[g] = (pq.astype(f32) * pl.reciprocal(den, approx=True)).astype(bf16)
                    state['pace'] = den
            return [(RT, functools.partial(norm, range(0, 4)), None), (RT, functools.partial(norm, range(4, 8)), None)]

        def proj_tasks(t, state):
            loc = {}

            def proj(j):
                if 'lhs' not in loc:
                    loc['lhs'] = jnp.concatenate([_ld(pqn_s, g, (0, RT)) for g in range(NG)], axis=1)
                res = _dot(loc['lhs'], _ld(M_s, j, (0, D)))
                ob_s[t, j] = res.astype(bf16)
                state['pace'] = res
                cp_ob(t, j).start()
            return [(2 * RT, functools.partial(proj, j), None) for j in range(NG)]

        def tile_tasks(t, state, norm_next):
            pr = proj_tasks(t, state)
            if not norm_next:
                return pr
            nm = norm_tasks(t + 1, state)
            a, b = P['NPOS'], P['NPOS'] + 2
            return pr[:a] + nm[:1] + pr[a:b] + nm[1:] + pr[b:]

        def m_tasks(state):
            r = lax.broadcasted_iota(jnp.int32, (G, G), 0) // HEAD
            c = lax.broadcasted_iota(jnp.int32, (G, G), 1) // HEAD
            bd = r == c

            def mt(g):
                z = jnp.sum(z_s[g], axis=0, keepdims=True)
                zc = jnp.broadcast_to(z, (G, G)).T
                zb_s[g] = jnp.where(bd, zc, 0.0).astype(bf16)
                gm = jnp.concatenate([_ld(gm_s, g, j, (0, G)) for j in range(NG)], axis=1)
                kv = _dot(gm, _bc(wvs[:, pl.ds(g * G, G)]))
                kvb = jnp.where(bd, kv, 0.0).astype(bf16)
                wo = _bc(wos[pl.ds(g * G // 2, G // 2), :])
                Mg = _dot(kvb, wo)
                state['pace'] = Mg[:, 0:G]
                for j in range(NG):
                    M_s[j, pl.ds(g * G, G), :] = Mg[:, j * G:(j + 1) * G].astype(bf16)
            return [(512, functools.partial(mt, g), None) for g in range(NG)]

        @pl.when(step == 0)
        def _():
            ks[:, 0:8, :] = jnp.zeros((NG, 8, G), u32)
            cp_w(0, 0).start()
            cp_x(0).start()
            cp_w(0, 1).start()
            for c in range(1, NCH):
                cp_x(c).start()
            for c in cp_consts():
                c.start()
            for c in cp_a(0):
                c.start()
            for g in range(1, NG + 1):
                for p in range(2):
                    cp_w(g, p).start()
                cp_q(g - 1).start()
                if g < NG:
                    for c in cp_a(g):
                        c.start()
            for c in cp_wo():
                c.start()
            if True:
                cp_w(0, 0).wait()
                cp_x(0).wait()
                cp_w(0, 1).wait()
            group_step(0, None, True)

        @pl.when(jnp.logical_and(step > 0, step < NG))
        def _():
            cp_q(step - 1).wait()
            group_step(step, step - 1, False)

        @pl.when(step == NG)
        def _():
            for c in cp_wo():
                c.wait()
            cp_q(NG - 1).wait()
            state = {}
            mt = m_tasks(state)
            nm = norm_tasks(0, state)
            mm = mt[:P['NM0']] + nm[:1] + mt[P['NM0']:] + nm[1:] if P['NM0'] < NG else mt + nm
            for t in range(NTA):
                mm += tile_tasks(t, state, True)
            emit(mm, state, NG - 1, sum(m[0] for m in mm) * P['FILL_END_F'], P['ORDER_F'], P['PSTEP_F'])

        @pl.when(jnp.logical_and(step > NG, step < NSTEPS - 1))
        def _():
            state = {}
            for (_, fn, _) in tile_tasks(step - (NG + 1) + NTA, state, True):
                fn()

        @pl.when(step == NSTEPS - 1)
        def _():
            state = {}
            for (_, fn, _) in tile_tasks(NT - 1, state, False):
                fn()
            for g in range(NG):
                cp_oa(g).wait()
            for t in range(NT):
                for j in range(NG):
                    cp_ob(t, j).wait()

    scratch = [
        pltpu.VMEM((NG, S // 2, G), u32), pltpu.VMEM((NG, 8 + S // 2, G), u32), pltpu.VMEM((NG, S // 2, G), u32),
        pltpu.VMEM((4, D), bf16), pltpu.VMEM((NG, G // 2, S), u32), pltpu.VMEM((8, 128), bf16),
        pltpu.VMEM((256, 128), u32), pltpu.VMEM((64, 128), u32),
        pltpu.VMEM((S // 2, D), u32), pltpu.VMEM((NG + 1, 2, D // 2, G), u32), pltpu.VMEM((D // 2, D), u32),
        pltpu.VMEM((D // 2, D), u32), pltpu.VMEM((2, D // 2, G), u32),
        pltpu.VMEM((S // 2, G), u32),
        pltpu.VMEM((NB, 256, G), f32), pltpu.VMEM((256, G), f32), pltpu.VMEM((NB, 256, G), f32),
        pltpu.VMEM((NB, 2, 128, G), bf16), pltpu.VMEM((NG, S, G), bf16),
        pltpu.VMEM((S, G), bf16), pltpu.VMEM((NG, NG, G, G), bf16), pltpu.VMEM((NG, S, G), bf16),
        pltpu.VMEM((NG, 8, G), f32),
        pltpu.VMEM((NG, D, G), bf16), pltpu.VMEM((NG, G, G), bf16), pltpu.VMEM((NT, NG, RT, G), bf16),
        pltpu.VMEM((NG, RT, G), bf16),
        pltpu.SemaphoreType.DMA((4,)), pltpu.SemaphoreType.DMA((NCH,)), pltpu.SemaphoreType.DMA((2 * (NG + 1),)),
        pltpu.SemaphoreType.DMA((NG,)), pltpu.SemaphoreType.DMA((NG,)), pltpu.SemaphoreType.DMA((2,)),
        pltpu.SemaphoreType.DMA((NG,)), pltpu.SemaphoreType.DMA((NT,)),
    ]
    return kernel, scratch, NSTEPS


_KERNEL, _SCRATCH, _NSTEPS = make_kernel(PARAMS)
_FP, _FIP = _dft_mats(PARAMS['RP'])


@jax.jit
def pallas_concat_heads__ssm_conv_h3__linear_attn_block__prompt_kernel(A_q, A_k, A_v, A_shift_k, A_ssm_k, A_ssm_D, B_x, B_wqkv, B_wo):
    out = pl.pallas_call(
        _KERNEL, grid=(_NSTEPS,),
        in_specs=[pl.BlockSpec(memory_space=pl.ANY)] * 11,
        out_specs=pl.BlockSpec(memory_space=pl.ANY),
        out_shape=jax.ShapeDtypeStruct((S, 2 * D), bf16),
        scratch_shapes=_SCRATCH,
        compiler_params=pltpu.CompilerParams(vmem_limit_bytes=110 * 1024 * 1024, dimension_semantics=("arbitrary",)),
    )(A_q.reshape(S, D), A_k.reshape(S, D), A_v.reshape(S, D), A_shift_k.T, A_ssm_k, A_ssm_D.reshape(8, 128),
      jnp.asarray(_FP), jnp.asarray(_FIP), B_x.reshape(S, D), B_wqkv, B_wo)
    return out.reshape(1, S, 2 * D)
```

```python
import functools
import numpy as np
import jax
import jax.numpy as jnp
from jax import lax
from jax.experimental import pallas as pl
from jax.experimental.pallas import tpu as pltpu

f32, bf16, u32 = jnp.float32, jnp.bfloat16, jnp.uint32

S, D = 2048, 1024
G = 128
NG = D // G
B = 128
NB = S // B
HEAD = 32

PARAMS = {'RP': 8, 'KSPLIT': 2, 'CH': 128, 'RT': 256, 'FWD_START': 14.0, 'FWD_START0': 14.0, 'ORDER_F': 'desc', 'PSTEP_F': 8, 'FILL_END': 13.9, 'KVPARTS': 4, 'ORDER': 'desc', 'TI': 4, 'PACE': 1, 'PSTEP': 4, 'NTA': 4, 'NPOS': 2, 'NM0': 6, 'W0FIRST': 1, 'QLAG': 1, 'FWD_END': 16.0, 'ZPAIR': 1, 'FILL_END_F': 0.9, 'SKIP': '', 'XG': '1-2-4-7-11-16'}


def _pack_rows(a):
    b = np.asarray(a, dtype=bf16).view(np.uint16).astype(np.uint32)
    return b[0::2] | (b[1::2] << 16)


def _dft_mats(RP):
    ks = np.concatenate([np.arange(0, 128, 2), np.arange(1, 128, 2)])
    sg = np.where(ks % 2 == 0, 1.0, -1.0)[:, None]
    th = (np.pi * (2 * ks + 1) / 256.0)[:, None]
    t = np.arange(128)[None, :]

    def inter(re, im):
        rows = []
        for r in range(128 // RP):
            rows.append(re[r * RP:(r + 1) * RP])
            rows.append(im[r * RP:(r + 1) * RP])
        return np.concatenate(rows, axis=0)

    hre, him = np.cos(th * t), -np.sin(th * t)
    ure, uim = np.cos(th * (t + 0.5)), -np.sin(th * (t + 0.5))
    FU = inter(ure - sg * uim, uim + sg * ure)
    FH = inter(hre, him)
    phi = th * (np.arange(64)[None, :] + 0.5)
    C1 = ((np.cos(phi) + sg * np.sin(phi)) / 256.0).T
    C2 = ((sg * np.cos(phi) - np.sin(phi)) / 256.0).T
    fwd = np.concatenate([_pack_rows(FU), _pack_rows(FH)], axis=0)
    inv = np.concatenate([_pack_rows(C1), _pack_rows(C2)], axis=0)
    return fwd, inv


def _phi(t):
    return jnp.where(t > 0, t + 1.0, jnp.exp(t)) + 1e-6


def _dot(a, b):
    return jnp.dot(a, b, preferred_element_type=f32)


def _bc(x):
    return pltpu.bitcast(x, bf16)


def _ld(ref, *idx):
    *lead, (r0, n) = idx
    return _bc(ref.bitcast(u32)[(*lead, pl.ds(r0 // 2, n // 2), slice(None))])


def make_kernel(P):
    RP, KSPLIT, CH, RT = P['RP'], P['KSPLIT'], P['CH'], P['RT']
    NR = 128 // RP
    NCH = S // CH
    NT = S // RT
    NTA = P['NTA']
    NSTEPS = NG + 1 + (NT - NTA)
    X_GROUPS = []
    bnds = [int(v) for v in P['XG'].split('-')]
    for lo, hi in zip(bnds[:-1], bnds[1:]):
        X_GROUPS.append((list(range(lo, hi)), lo))

    def kernel(q_hbm, k_hbm, v_hbm, sk_hbm, h_hbm, d_hbm, f_hbm, fi_hbm, x_hbm, w_hbm, wo_hbm, o_hbm,
               qs, ks, vs, sks, hs, ds_, fs, fis, xs, ws, wos, wvs, wcur,
               u_s, U_s, H_s, G_s, Z_s, oa_s, pk_s, gm_s, pq_s, z_s, M_s, zb_s, ob_s, pqn_s,
               sem_c, sem_x, sem_w, sem_a, sem_q, sem_wo, sem_oa, sem_ob):
        step = pl.program_id(0)
        q32, k32, v32, h32 = (r.bitcast(u32) for r in (q_hbm, k_hbm, v_hbm, h_hbm))
        x32, w32, wo32 = (r.bitcast(u32) for r in (x_hbm, w_hbm, wo_hbm))

        def col(g):
            return pl.ds(pl.multiple_of(g * G, G), G)

        def cp_consts():
            return [pltpu.make_async_copy(a, b, sem_c.at[n]) for n, (a, b) in
                    enumerate(((f_hbm, fs), (fi_hbm, fis), (sk_hbm, sks), (d_hbm, ds_)))]

        def cp_x(c):
            rows = pl.ds(c * (CH // 2), CH // 2)
            return pltpu.make_async_copy(x32.at[rows], xs.at[rows], sem_x.at[c])

        def cp_w(g, p):
            gs = min(g, NG - 1) if isinstance(g, int) else jnp.minimum(g, NG - 1)
            off = (D, 0)[p]
            cols = pl.ds(off + gs * G if isinstance(gs, int) else pl.multiple_of(off + gs * G, G), G)
            return pltpu.make_async_copy(w32.at[:, cols], ws.at[g, p], sem_w.at[2 * g + p])

        def cp_a(g):
            return [pltpu.make_async_copy(k32.at[:, col(g)], ks.at[g, pl.ds(8, S // 2)], sem_a.at[g]),
                    pltpu.make_async_copy(v32.at[:, col(g)], vs.at[g], sem_a.at[g]),
                    pltpu.make_async_copy(h32.at[pl.ds(pl.multiple_of(g * (G // 2), G // 2), G // 2)], hs.at[g], sem_a.at[g])]

        def cp_q(g):
            return pltpu.make_async_copy(q32.at[:, col(g)], qs.at[g], sem_q.at[g])

        def cp_wo():
            return [pltpu.make_async_copy(wo32, wos, sem_wo.at[0]),
                    pltpu.make_async_copy(w32.at[:, pl.ds(2 * D, D)], wvs, sem_wo.at[1])]

        def cp_oa(g):
            return pltpu.make_async_copy(oa_s.at[g], o_hbm.at[:, col(g)], sem_oa.at[0])

        def cp_ob(t, j):
            rows = pl.ds(t * RT if isinstance(t, int) else pl.multiple_of(t * RT, RT), RT)
            return pltpu.make_async_copy(ob_s.at[t, j], o_hbm.at[rows, pl.ds(D + j * G, G)], sem_ob.at[0])

        def a_pre(g, sk, j):
            w0 = 8 + j * (B // 2)
            n = B // 2
            lo = lambda x: pltpu.bitcast(lax.shift_left(x, u32(16)), f32)
            hi = lambda x: pltpu.bitcast(x & u32(0xFFFF0000), f32)
            k0, k1, k2 = (ks[g, pl.ds(w0 - d, n), :] for d in range(3))
            e0, o0, e1, o1, o2 = lo(k0), hi(k0), lo(k1), hi(k1), hi(k2)
            s0, s1, s2, s3 = (sk[t:t + 1, :] for t in range(4))
            ye = e0 * s0 + o1 * s1 + e1 * s2 + o2 * s3
            yo = o0 * s0 + e0 * s1 + o1 * s2 + e1 * s3
            vv = vs[g, pl.ds(j * n, n), :]
            u = pltpu.bitcast(pltpu.pack_elementwise([ye * lo(vv), yo * hi(vv)], packed_dtype=bf16), u32)
            u_s[pl.ds(j * n, n), :] = u
            return _bc(u)

        def a_fwd(g, sk, j0):
            u2 = jnp.concatenate([a_pre(g, sk, j0), a_pre(g, sk, j0 + 1)], axis=1)
            U2 = _dot(_bc(fs[0:128, :]), u2)
            h2 = jnp.concatenate([_bc(hs[g, :, pl.ds((j0 + d) * B, B)]) for d in range(2)], axis=0)
            H2 = lax.dot_general(_bc(fs[128:256, :]), h2, (((1,), (1,)), ((), ())), preferred_element_type=f32)
            for d in range(2):
                j = j0 + d
                U_s[j] = U2[:, d * G:(d + 1) * G]
                H = H2[:, d * G:(d + 1) * G]
                if j == 0:
                    G_s[0] = H
                else:
                    for r in range(NR):
                        a, b = 2 * r * RP, (2 * r + 1) * RP
                        hre, him = H[a:a + RP], H[b:b + RP]
                        if d == 0:
                            pre, pim = H_s[pl.ds(a, RP), :], H_s[pl.ds(b, RP), :]
                        else:
                            pre, pim = H2[a:a + RP, 0:G], H2[b:b + RP, 0:G]
                        if r < NR // 2:
                            G_s[j, pl.ds(a, RP), :] = hre - pim
                            G_s[j, pl.ds(b, RP), :] = him + pre
                        else:
                            G_s[j, pl.ds(a, RP), :] = hre + pim
                            G_s[j, pl.ds(b, RP), :] = him - pre
            if j0 + 2 < NB:
                H_s[...] = H2[:, G:2 * G]

        def load_sk(g):
            return sks[:, col(g)].astype(f32)

        def load_d(g):
            dall = ds_[...].astype(f32)
            return jnp.sum(jnp.where(lax.broadcasted_iota(jnp.int32, (8, G), 0) == g, dall, 0.0), axis=0, keepdims=True)

        held = {}

        def a_piece(i0, r, dep=None):
            a, b = 2 * r * RP, (2 * r + 1) * RP
            T = P['TI']
            acc = [(dep, dep)] * T
            gw = {}
            for j in range(i0 + T):
                ure, uim = U_s[j, pl.ds(a, RP), :], U_s[j, pl.ds(b, RP), :]
                for t in range(T):
                    m = i0 + t - j
                    if m < 0:
                        continue
                    if m not in gw:
                        gw[m] = (G_s[m, pl.ds(a, RP), :], G_s[m, pl.ds(b, RP), :])
                    gre, gim = gw[m]
                    tre = gre * ure - gim * uim
                    tim = gre * uim + gim * ure
                    zre, zim = acc[t]
                    acc[t] = (tre if zre is None else zre + tre, tim if zim is None else zim + tim)
            if P['ZPAIR'] and RP == 8:
                if r % 2 == 0:
                    held[(i0, r)] = acc
                else:
                    prev = held.pop((i0, r - 1))
                    for t in range(T):
                        for c in range(2):
                            z = jnp.concatenate([prev[t][c], acc[t][c]], axis=0)
                            Z_s[i0 + t, c, pl.ds((r - 1) * RP, 2 * RP), :] = z.astype(bf16)
            else:
                for t in range(T):
                    Z_s[i0 + t, 0, pl.ds(r * RP, RP), :] = acc[t][0].astype(bf16)
                    Z_s[i0 + t, 1, pl.ds(r * RP, RP), :] = acc[t][1].astype(bf16)

        def a_inv(g, dvec, i0):
            e2 = _dot(_bc(fis[0:32, :]), jnp.concatenate([_ld(Z_s, i0 + d, 0, (0, 128)) for d in range(2)], axis=1))
            o2 = _dot(_bc(fis[32:64, :]), jnp.concatenate([_ld(Z_s, i0 + d, 1, (0, 128)) for d in range(2)], axis=1))
            rev = 7 - lax.broadcasted_iota(jnp.int32, (8, G), 0)
            for d in range(2):
                r0 = (i0 + d) * B
                e, o = e2[:, d * G:(d + 1) * G], o2[:, d * G:(d + 1) * G]
                hi = e - o
                ycv = jnp.concatenate(
                    [e + o] + [jnp.take_along_axis(hi[8 * (7 - v):8 * (8 - v)], rev, axis=0) for v in range(8)], axis=0)
                uu = _bc(u_s[pl.ds(r0 // 2, B // 2), :]).astype(f32)
                y = ycv + uu * dvec
                qq = _bc(qs[g, pl.ds(r0 // 2, B // 2), :]).astype(f32)
                oa_s[g, pl.ds(r0, B), :] = (qq * y).astype(bf16)

        def emit(mm, state, ga, t_fill_end, order, pstep):
            pieces = []
            TI = P['TI']
            if ga is not None:
                dvec = load_d(ga)
                GS = max(2, TI)
                pairs = list(range(0, NB, GS))
                if order == 'desc':
                    pairs = pairs[::-1]
                elif order == 'mix':
                    lo, hi = pairs[:len(pairs) // 2], pairs[len(pairs) // 2:][::-1]
                    pairs = [b for pair in zip(hi, lo) for b in pair]
                for i0 in pairs:
                    pp = [(i, r) for r in range(NR) for i in range(i0, i0 + GS, TI)]
                    pieces += [(i, r, list(range(i0, i0 + GS, 2)) if n == len(pp) - 1 else None) for n, (i, r) in enumerate(pp)]
            pcost = lambda i: sum(ii + 1 for ii in range(i, i + TI))
            tot_p = sum(pcost(p[0]) for p in pieces)
            T = 0
            done_cost = 0
            pi = 0
            pend_inv = []
            for (cost, fn, tag) in mm:
                if tag == 'fwd':
                    assert pi == len(pieces) and not pend_inv, "fwd for next tile would overwrite live U/G/u"
                fn()
                T += cost
                for i0 in pend_inv:
                    a_inv(ga, dvec, i0)
                    T += 64
                pend_inv = []
                target = tot_p * min(1.0, T / t_fill_end)
                kk = 0
                while pi < len(pieces) and done_cost < target:
                    i, r, fin = pieces[pi]
                    dep = None
                    if P['PACE'] and 'pace' in state:
                        pace = state['pace']
                        idx = min(pace.shape[0] // RP - 1, kk * pstep * 8 // RP)
                        pv = pltpu.bitcast(pace[idx * RP:(idx + 1) * RP, :], u32)
                        dep = pltpu.bitcast(lax.shift_right_logical(lax.shift_right_logical(pv, u32(16)), u32(16)), f32)
                        kk += 1
                    a_piece(i, r, dep)
                    done_cost += pcost(i)
                    pi += 1
                    if fin is not None:
                        pend_inv.extend(fin)
            assert pi == len(pieces) and not pend_inv
            if ga is not None:
                cp_oa(ga).start()

        def group_step(g, ga, first):
            KS = D // KSPLIT
            NQ = 4
            QR = S // NQ
            GW = D // 4
            state = {}
            hooks = {}

            def proj_part(name, p, c, ks_):
                x = _bc(xs[pl.ds(c * CH // 2, CH // 2), pl.ds(ks_ * KS, KS)])
                if first:
                    w = _bc(ws[g, p, pl.ds(ks_ * KS // 2, KS // 2), :])
                else:
                    w = _bc(wcur[p, pl.ds(ks_ * KS // 2, KS // 2), :])
                part = _dot(x, w)
                state[name] = part if ks_ == 0 else state[name] + part
                state['pace'] = part
                if ks_ == KSPLIT - 1:
                    for h in hooks.get((name, c), []):
                        h()

            def next_w(p):
                if not first:
                    assert state.get('late_done'), "W(g+1) copied before its DMA was waited for"
                    wcur[p] = ws[g + 1, p]

            def fin_k(c):
                pk = _phi(state.pop('k'))
                pk_s[pl.ds(c * CH, CH), :] = pk.astype(bf16)
                zp = jnp.sum(pk.reshape(CH // 8, 8, G), axis=0)
                state['z'] = zp if c == 0 else state['z'] + zp
                if c == NCH - 1:
                    z_s[g] = state.pop('z')
                    next_w(0)

            def fin_q(c):
                pq_s[g, pl.ds(c * CH, CH), :] = _phi(state.pop('q')).astype(bf16)
                if c == NCH - 1:
                    next_w(1)

            def g_task(n, h):
                a = _ld(pk_s, (n * QR, QR))
                b = _bc(xs[pl.ds(n * QR // 2, QR // 2), pl.ds(h * GW, GW)])
                part = lax.dot_general(a, b, (((0,), (0,)), ((), ())), preferred_element_type=f32)
                state['pace'] = part[:, 0:G]
                acc = part if n == 0 else state[('G', h)] + part
                if n < NQ - 1:
                    state[('G', h)] = acc
                else:
                    for d in range(GW // G):
                        gm_s[g, h * (GW // G) + d] = acc[:, d * G:(d + 1) * G].astype(bf16)

            def fwd_task(j):
                assert state.get('late_done')
                if j == 0:
                    state['sk'] = load_sk(g)
                a_fwd(g, state['sk'], j)

            def wait_all(cps, nm="w"):
                if True:
                    for c in cps:
                        c.wait()

            def wait_late():
                cps = cp_a(g)
                if first:
                    cps = cp_consts() + cps
                else:
                    cps = cps + [cp_w(g + 1, p) for p in range(2)]
                wait_all(cps, 'a')
                state['late_done'] = True

            pc = CH * 8 // KSPLIT // 4
            units = []

            def add_proj(name, p, c, fin):
                for ks_ in range(KSPLIT):
                    def t(ks_=ks_):
                        proj_part(name, p, c, ks_)
                        if ks_ == KSPLIT - 1:
                            fin(c)
                    units.append((pc, t, (name, c)))

            cq = CH * NQ // S if False else None
            per = NCH // NQ
            gq = [(n, h) for n in range(NQ) for h in range(4)]
            gi = 0
            for c in range(NCH):
                add_proj('k', 0, c, fin_k)
                if c >= per and (c % per) * 4 // per != ((c - 1) % per) * 4 // per or (c >= per and c % per == 0):
                    n, h = gq[gi]
                    assert n < c // per
                    units.append((256, functools.partial(g_task, n, h), ('G', gi)))
                    gi += 1
                if c >= P['QLAG']:
                    add_proj('q', 1, c - P['QLAG'], fin_q)
            rest_q = list(range(NCH - P['QLAG'], NCH))
            while gi < len(gq) or rest_q:
                if rest_q:
                    add_proj('q', 1, rest_q.pop(0), fin_q)
                if gi < len(gq):
                    n, h = gq[gi]
                    units.append((256, functools.partial(g_task, n, h), ('G', gi)))
                    gi += 1

            total = sum(u[0] for u in units)
            fwd_start = (P['FWD_START0'] if first else P['FWD_START']) / 16.0 * total
            t_fill_end = P['FILL_END'] / 16.0 * total
            fwd_end = P['FWD_END'] / 16.0 * total
            pos = [fwd_start + (fwd_end - fwd_start) * n / (NB // 2) for n in range(NB // 2)]
            mm = []
            T = 0
            nf = 0
            last_proj = None
            hooked = False
            for (cost, fn, tag) in units:
                while nf < len(pos) and T >= pos[nf]:
                    if not hooked:
                        hooks.setdefault(last_proj, []).append(wait_late)
                        hooked = True
                    mm.append((256, functools.partial(fwd_task, 2 * nf), 'fwd'))
                    nf += 1
                mm.append((cost, fn, None))
                T += cost
                if tag[0] in ('k', 'q'):
                    last_proj = tag
            if not hooked:
                hooks.setdefault(last_proj, []).append(wait_late)
            while nf < len(pos):
                mm.append((256, functools.partial(fwd_task, 2 * nf), 'fwd'))
                nf += 1
            if first:
                for grp, lo in X_GROUPS:
                    hooks.setdefault(('k', lo - 1), []).append(
                        functools.partial(lambda grp: wait_all([cp_x(c) for c in grp], 'x%d' % grp[0]), grp))
            emit(mm, state, ga, t_fill_end, P['ORDER'], P['PSTEP'])
            if first:
                wait_all([cp_w(1, p) for p in range(2)], 'w1')
                for p in range(2):
                    wcur[p] = ws[1, p]

        def tile_rows(t):
            t0 = t * (RT // 2)
            return pl.ds(t0 if isinstance(t, int) else pl.multiple_of(t0, RT // 2), RT // 2)

        def norm_tasks(t, state):
            pq32 = pq_s.bitcast(u32)

            def norm(gs):
                for g in gs:
                    pq = _bc(pq32[g, tile_rows(t), :])
                    den = _dot(pq, _ld(zb_s, g, (0, G))) + 1e-6
                    pqn_s[g] = (pq.astype(f32) * pl.reciprocal(den, approx=True)).astype(bf16)
                    state['pace'] = den
            return [(RT, functools.partial(norm, range(0, 4)), None), (RT, functools.partial(norm, range(4, 8)), None)]

        def proj_tasks(t, state):
            loc = {}

            def proj(j):
                if 'lhs' not in loc:
                    loc['lhs'] = jnp.concatenate([_ld(pqn_s, g, (0, RT)) for g in range(NG)], axis=1)
                res = _dot(loc['lhs'], _ld(M_s, j, (0, D)))
                ob_s[t, j] = res.astype(bf16)
                state['pace'] = res
                cp_ob(t, j).start()
            return [(2 * RT, functools.partial(proj, j), None) for j in range(NG)]

        def tile_tasks(t, state, norm_next):
            pr = proj_tasks(t, state)
            if not norm_next:
                return pr
            nm = norm_tasks(t + 1, state)
            a, b = P['NPOS'], P['NPOS'] + 2
            return pr[:a] + nm[:1] + pr[a:b] + nm[1:] + pr[b:]

        def m_tasks(state):
            r = lax.broadcasted_iota(jnp.int32, (G, G), 0) // HEAD
            c = lax.broadcasted_iota(jnp.int32, (G, G), 1) // HEAD
            bd = r == c

            def mt(g):
                z = jnp.sum(z_s[g], axis=0, keepdims=True)
                zc = jnp.broadcast_to(z, (G, G)).T
                zb_s[g] = jnp.where(bd, zc, 0.0).astype(bf16)
                gm = jnp.concatenate([_ld(gm_s, g, j, (0, G)) for j in range(NG)], axis=1)
                kv = _dot(gm, _bc(wvs[:, pl.ds(g * G, G)]))
                kvb = jnp.where(bd, kv, 0.0).astype(bf16)
                wo = _bc(wos[pl.ds(g * G // 2, G // 2), :])
                Mg = _dot(kvb, wo)
                state['pace'] = Mg[:, 0:G]
                for j in range(NG):
                    M_s[j, pl.ds(g * G, G), :] = Mg[:, j * G:(j + 1) * G].astype(bf16)
            return [(512, functools.partial(mt, g), None) for g in range(NG)]

        @pl.when(step == 0)
        def _():
            ks[:, 0:8, :] = jnp.zeros((NG, 8, G), u32)
            cp_w(0, 0).start()
            cp_x(0).start()
            cp_w(0, 1).start()
            for c in range(1, NCH):
                cp_x(c).start()
            for c in cp_consts():
                c.start()
            for c in cp_a(0):
                c.start()
            for g in range(1, NG + 1):
                for p in range(2):
                    cp_w(g, p).start()
                cp_q(g - 1).start()
                if g < NG:
                    for c in cp_a(g):
                        c.start()
            for c in cp_wo():
                c.start()
            if True:
                cp_w(0, 0).wait()
                cp_x(0).wait()
                cp_w(0, 1).wait()
            group_step(0, None, True)

        @pl.when(jnp.logical_and(step > 0, step < NG))
        def _():
            cp_q(step - 1).wait()
            group_step(step, step - 1, False)

        @pl.when(step == NG)
        def _():
            for c in cp_wo():
                c.wait()
            cp_q(NG - 1).wait()
            state = {}
            mt = m_tasks(state)
            nm = norm_tasks(0, state)
            mm = mt[:P['NM0']] + nm[:1] + mt[P['NM0']:] + nm[1:] if P['NM0'] < NG else mt + nm
            for t in range(NTA):
                mm += tile_tasks(t, state, True)
            emit(mm, state, NG - 1, sum(m[0] for m in mm) * P['FILL_END_F'], P['ORDER_F'], P['PSTEP_F'])

        @pl.when(jnp.logical_and(step > NG, step < NSTEPS - 1))
        def _():
            state = {}
            for (_, fn, _) in tile_tasks(step - (NG + 1) + NTA, state, True):
                fn()

        @pl.when(step == NSTEPS - 1)
        def _():
            state = {}
            for (_, fn, _) in tile_tasks(NT - 1, state, False):
                fn()
            pltpu.make_async_copy(oa_s, oa_s, sem_oa.at[0]).wait()
            pltpu.make_async_copy(ob_s, ob_s, sem_ob.at[0]).wait()

    scratch = [
        pltpu.VMEM((NG, S // 2, G), u32), pltpu.VMEM((NG, 8 + S // 2, G), u32), pltpu.VMEM((NG, S // 2, G), u32),
        pltpu.VMEM((4, D), bf16), pltpu.VMEM((NG, G // 2, S), u32), pltpu.VMEM((8, 128), bf16),
        pltpu.VMEM((256, 128), u32), pltpu.VMEM((64, 128), u32),
        pltpu.VMEM((S // 2, D), u32), pltpu.VMEM((NG + 1, 2, D // 2, G), u32), pltpu.VMEM((D // 2, D), u32),
        pltpu.VMEM((D // 2, D), u32), pltpu.VMEM((2, D // 2, G), u32),
        pltpu.VMEM((S // 2, G), u32),
        pltpu.VMEM((NB, 256, G), f32), pltpu.VMEM((256, G), f32), pltpu.VMEM((NB, 256, G), f32),
        pltpu.VMEM((NB, 2, 128, G), bf16), pltpu.VMEM((NG, S, G), bf16),
        pltpu.VMEM((S, G), bf16), pltpu.VMEM((NG, NG, G, G), bf16), pltpu.VMEM((NG, S, G), bf16),
        pltpu.VMEM((NG, 8, G), f32),
        pltpu.VMEM((NG, D, G), bf16), pltpu.VMEM((NG, G, G), bf16), pltpu.VMEM((NT, NG, RT, G), bf16),
        pltpu.VMEM((NG, RT, G), bf16),
        pltpu.SemaphoreType.DMA((4,)), pltpu.SemaphoreType.DMA((NCH,)), pltpu.SemaphoreType.DMA((2 * (NG + 1),)),
        pltpu.SemaphoreType.DMA((NG,)), pltpu.SemaphoreType.DMA((NG,)), pltpu.SemaphoreType.DMA((2,)),
        pltpu.SemaphoreType.DMA((1,)), pltpu.SemaphoreType.DMA((1,)),
    ]
    return kernel, scratch, NSTEPS


_KERNEL, _SCRATCH, _NSTEPS = make_kernel(PARAMS)
_FP, _FIP = _dft_mats(PARAMS['RP'])


@jax.jit
def pallas_concat_heads__ssm_conv_h3__linear_attn_block__prompt_kernel(A_q, A_k, A_v, A_shift_k, A_ssm_k, A_ssm_D, B_x, B_wqkv, B_wo):
    out = pl.pallas_call(
        _KERNEL, grid=(_NSTEPS,),
        in_specs=[pl.BlockSpec(memory_space=pl.ANY)] * 11,
        out_specs=pl.BlockSpec(memory_space=pl.ANY),
        out_shape=jax.ShapeDtypeStruct((S, 2 * D), bf16),
        scratch_shapes=_SCRATCH,
        compiler_params=pltpu.CompilerParams(vmem_limit_bytes=110 * 1024 * 1024, dimension_semantics=("arbitrary",)),
    )(A_q.reshape(S, D), A_k.reshape(S, D), A_v.reshape(S, D), A_shift_k.T, A_ssm_k, A_ssm_D.reshape(8, 128),
      jnp.asarray(_FP), jnp.asarray(_FIP), B_x.reshape(S, D), B_wqkv, B_wo)
    return out.reshape(1, S, 2 * D)
```

```python
import functools
import numpy as np
import jax
import jax.numpy as jnp
from jax import lax
from jax.experimental import pallas as pl
from jax.experimental.pallas import tpu as pltpu

f32, bf16, u32 = jnp.float32, jnp.bfloat16, jnp.uint32

S, D = 2048, 1024
G = 128
NG = D // G
B = 128
NB = S // B
HEAD = 32

PARAMS = {'RP': 8, 'KSPLIT': 2, 'CH': 128, 'RT': 256, 'FWD_START': 14.0, 'FWD_START0': 14.0, 'ORDER_F': 'desc', 'PSTEP_F': 8, 'FILL_END': 13.9, 'KVPARTS': 4, 'ORDER': 'desc', 'TI': 4, 'PACE': 1, 'PSTEP': 8, 'NTA': 4, 'NTL': 4, 'NPOS': 2, 'NM0': 6, 'W0FIRST': 1, 'QLAG': 1, 'FWD_END': 16.0, 'ZPAIR': 1, 'FILL_END_F': 0.9, 'SKIP': '', 'XG': '1-2-4-7-11-16'}


def _pack_rows(a):
    b = np.asarray(a, dtype=bf16).view(np.uint16).astype(np.uint32)
    return b[0::2] | (b[1::2] << 16)


def _dft_mats(RP):
    ks = np.concatenate([np.arange(0, 128, 2), np.arange(1, 128, 2)])
    sg = np.where(ks % 2 == 0, 1.0, -1.0)[:, None]
    th = (np.pi * (2 * ks + 1) / 256.0)[:, None]
    t = np.arange(128)[None, :]

    def inter(re, im):
        rows = []
        for r in range(128 // RP):
            rows.append(re[r * RP:(r + 1) * RP])
            rows.append(im[r * RP:(r + 1) * RP])
        return np.concatenate(rows, axis=0)

    hre, him = np.cos(th * t), -np.sin(th * t)
    ure, uim = np.cos(th * (t + 0.5)), -np.sin(th * (t + 0.5))
    FU = inter(ure - sg * uim, uim + sg * ure)
    FU = np.concatenate([FU[:, 0::2], FU[:, 1::2]], axis=1)
    FH = inter(hre, him)
    phi = th * (np.arange(64)[None, :] + 0.5)
    C1 = ((np.cos(phi) + sg * np.sin(phi)) / 256.0).T
    C2 = ((sg * np.cos(phi) - np.sin(phi)) / 256.0).T
    fwd = np.concatenate([_pack_rows(FU), _pack_rows(FH)], axis=0)
    inv = np.concatenate([_pack_rows(C1), _pack_rows(C2)], axis=0)
    return fwd, inv


def _phi(t):
    return jnp.where(t > 0, t + 1.0, jnp.exp(t)) + 1e-6


def _dot(a, b):
    return jnp.dot(a, b, preferred_element_type=f32)


def _bc(x):
    return pltpu.bitcast(x, bf16)


def _ld(ref, *idx):
    *lead, (r0, n) = idx
    return _bc(ref.bitcast(u32)[(*lead, pl.ds(r0 // 2, n // 2), slice(None))])


def make_kernel(P):
    RP, KSPLIT, CH, RT = P['RP'], P['KSPLIT'], P['CH'], P['RT']
    NR = 128 // RP
    NCH = S // CH
    NT = S // RT
    NTA = P['NTA']
    NTL = P['NTL']
    NSTEPS = NG + 1 + (NT - NTA - NTL) + 1
    X_GROUPS = []
    bnds = [int(v) for v in P['XG'].split('-')]
    for lo, hi in zip(bnds[:-1], bnds[1:]):
        X_GROUPS.append((list(range(lo, hi)), lo))

    def kernel(q_hbm, k_hbm, v_hbm, sk_hbm, h_hbm, d_hbm, f_hbm, fi_hbm, x_hbm, w_hbm, wo_hbm, o_hbm,
               qs, ks, vs, sks, hs, ds_, fs, fis, xs, ws, wos, wvs, wcur,
               U_s, H_s, G_s, Z_s, oa_s, pk_s, gm_s, pq_s, z_s, M_s, zb_s, ob_s, pqn_s,
               sem_c, sem_x, sem_w, sem_a, sem_q, sem_wo, sem_oa, sem_ob):
        step = pl.program_id(0)
        q32, k32, v32, h32 = (r.bitcast(u32) for r in (q_hbm, k_hbm, v_hbm, h_hbm))
        x32, w32, wo32 = (r.bitcast(u32) for r in (x_hbm, w_hbm, wo_hbm))

        def col(g):
            return pl.ds(pl.multiple_of(g * G, G), G)

        def cp_consts():
            return [pltpu.make_async_copy(a, b, sem_c.at[n]) for n, (a, b) in
                    enumerate(((f_hbm, fs), (fi_hbm, fis), (sk_hbm, sks), (d_hbm, ds_)))]

        def cp_x(c):
            rows = pl.ds(c * (CH // 2), CH // 2)
            return pltpu.make_async_copy(x32.at[rows], xs.at[rows], sem_x.at[c])

        def cp_w(g, p):
            gs = min(g, NG - 1) if isinstance(g, int) else jnp.minimum(g, NG - 1)
            off = (D, 0)[p]
            cols = pl.ds(off + gs * G if isinstance(gs, int) else pl.multiple_of(off + gs * G, G), G)
            return pltpu.make_async_copy(w32.at[:, cols], ws.at[g, p], sem_w.at[2 * g + p])

        def cp_a(g):
            return [pltpu.make_async_copy(k32.at[:, col(g)], ks.at[g, pl.ds(8, S // 2)], sem_a.at[g]),
                    pltpu.make_async_copy(v32.at[:, col(g)], vs.at[g], sem_a.at[g]),
                    pltpu.make_async_copy(h32.at[pl.ds(pl.multiple_of(g * (G // 2), G // 2), G // 2)], hs.at[g], sem_a.at[g])]

        def cp_q(g):
            return pltpu.make_async_copy(q32.at[:, col(g)], qs.at[g], sem_q.at[g])

        def cp_wo():
            return [pltpu.make_async_copy(wo32, wos, sem_wo.at[0]),
                    pltpu.make_async_copy(w32.at[:, pl.ds(2 * D, D)], wvs, sem_wo.at[1])]

        def cp_oa(g):
            return pltpu.make_async_copy(oa_s.at[g], o_hbm.at[:, col(g)], sem_oa.at[0])

        def cp_ob(t, j):
            rows = pl.ds(t * RT if isinstance(t, int) else pl.multiple_of(t * RT, RT), RT)
            return pltpu.make_async_copy(ob_s.at[t, j], o_hbm.at[rows, pl.ds(D + j * G, G)], sem_ob.at[0])

        def a_pre(g, sk, j):
            w0 = 8 + j * (B // 2)
            n = B // 2
            lo = lambda x: pltpu.bitcast(lax.shift_left(x, u32(16)), f32)
            hi = lambda x: pltpu.bitcast(x & u32(0xFFFF0000), f32)
            k0, k1, k2 = (ks[g, pl.ds(w0 - d, n), :] for d in range(3))
            e0, o0, e1, o1, o2 = lo(k0), hi(k0), lo(k1), hi(k1), hi(k2)
            s0, s1, s2, s3 = (sk[t:t + 1, :] for t in range(4))
            ye = e0 * s0 + o1 * s1 + e1 * s2 + o2 * s3
            yo = o0 * s0 + e0 * s1 + o1 * s2 + e1 * s3
            vv = vs[g, pl.ds(j * n, n), :]
            return jnp.concatenate([ye * lo(vv), yo * hi(vv)], axis=0).astype(bf16)

        def a_fwd(g, sk, dvec, j0):
            u2 = jnp.concatenate([a_pre(g, sk, j0), a_pre(g, sk, j0 + 1)], axis=1)
            U2 = _dot(_bc(fs[0:128, :]), u2)
            h2 = jnp.concatenate([_bc(hs[g, :, pl.ds((j0 + d) * B, B)]) for d in range(2)], axis=0)
            H2 = lax.dot_general(_bc(fs[128:256, :]), h2, (((1,), (1,)), ((), ())), preferred_element_type=f32)
            if j0 == 0:
                h0 = jnp.concatenate(
                    [H2[r * RP:(r + 1) * RP, 0:G] + dvec if r % 2 == 0 else H2[r * RP:(r + 1) * RP, 0:G]
                     for r in range(2 * NR)], axis=0)
            for d in range(2):
                j = j0 + d
                U_s[j] = U2[:, d * G:(d + 1) * G]
                H = H2[:, d * G:(d + 1) * G]
                if j == 0:
                    H = h0
                    G_s[0] = H
                else:
                    for r in range(NR):
                        a, b = 2 * r * RP, (2 * r + 1) * RP
                        hre, him = H[a:a + RP], H[b:b + RP]
                        if d == 0:
                            pre, pim = H_s[pl.ds(a, RP), :], H_s[pl.ds(b, RP), :]
                        else:
                            hp = h0 if j0 == 0 else H2[:, 0:G]
                            pre, pim = hp[a:a + RP], hp[b:b + RP]
                        if r < NR // 2:
                            G_s[j, pl.ds(a, RP), :] = hre - pim
                            G_s[j, pl.ds(b, RP), :] = him + pre
                        else:
                            G_s[j, pl.ds(a, RP), :] = hre + pim
                            G_s[j, pl.ds(b, RP), :] = him - pre
            if j0 + 2 < NB:
                H_s[...] = H2[:, G:2 * G]

        def load_sk(g):
            return sks[:, col(g)].astype(f32)

        def load_d(g):
            dall = ds_[...].astype(f32)
            return jnp.sum(jnp.where(lax.broadcasted_iota(jnp.int32, (8, G), 0) == g, dall, 0.0), axis=0, keepdims=True)

        held = {}

        def a_piece(i0, r, dep=None):
            a, b = 2 * r * RP, (2 * r + 1) * RP
            T = P['TI']
            acc = [(dep, dep)] * T
            gw = {}
            for j in range(i0 + T):
                ure, uim = U_s[j, pl.ds(a, RP), :], U_s[j, pl.ds(b, RP), :]
                for t in range(T):
                    m = i0 + t - j
                    if m < 0:
                        continue
                    if m not in gw:
                        gw[m] = (G_s[m, pl.ds(a, RP), :], G_s[m, pl.ds(b, RP), :])
                    gre, gim = gw[m]
                    tre = gre * ure - gim * uim
                    tim = gre * uim + gim * ure
                    zre, zim = acc[t]
                    acc[t] = (tre if zre is None else zre + tre, tim if zim is None else zim + tim)
            if P['ZPAIR'] and RP == 8:
                if r % 2 == 0:
                    held[(i0, r)] = acc
                else:
                    prev = held.pop((i0, r - 1))
                    for t in range(T):
                        for c in range(2):
                            z = jnp.concatenate([prev[t][c], acc[t][c]], axis=0)
                            Z_s[i0 + t, c, pl.ds((r - 1) * RP, 2 * RP), :] = z.astype(bf16)
            else:
                for t in range(T):
                    Z_s[i0 + t, 0, pl.ds(r * RP, RP), :] = acc[t][0].astype(bf16)
                    Z_s[i0 + t, 1, pl.ds(r * RP, RP), :] = acc[t][1].astype(bf16)

        def a_inv(g, i0):
            e2 = _dot(_bc(fis[0:32, :]), jnp.concatenate([_ld(Z_s, i0 + d, 0, (0, 128)) for d in range(2)], axis=1))
            o2 = _dot(_bc(fis[32:64, :]), jnp.concatenate([_ld(Z_s, i0 + d, 1, (0, 128)) for d in range(2)], axis=1))
            rev = 7 - lax.broadcasted_iota(jnp.int32, (8, G), 0)
            for d in range(2):
                r0 = (i0 + d) * B
                e, o = e2[:, d * G:(d + 1) * G], o2[:, d * G:(d + 1) * G]
                hi = e - o
                ycv = jnp.concatenate(
                    [e + o] + [jnp.take_along_axis(hi[8 * (7 - v):8 * (8 - v)], rev, axis=0) for v in range(8)], axis=0)
                y = ycv
                qq = _bc(qs[g, pl.ds(r0 // 2, B // 2), :]).astype(f32)
                oa_s[g, pl.ds(r0, B), :] = (qq * y).astype(bf16)

        def emit(mm, state, ga, t_fill_end, order, pstep):
            pieces = []
            TI = P['TI']
            if ga is not None:
                GS = max(2, TI)
                pairs = list(range(0, NB, GS))
                if order == 'desc':
                    pairs = pairs[::-1]
                elif order == 'mix':
                    lo, hi = pairs[:len(pairs) // 2], pairs[len(pairs) // 2:][::-1]
                    pairs = [b for pair in zip(hi, lo) for b in pair]
                for i0 in pairs:
                    pp = [(i, r) for r in range(NR) for i in range(i0, i0 + GS, TI)]
                    pieces += [(i, r, list(range(i0, i0 + GS, 2)) if n == len(pp) - 1 else None) for n, (i, r) in enumerate(pp)]
            pcost = lambda i: sum(ii + 1 for ii in range(i, i + TI))
            tot_p = sum(pcost(p[0]) for p in pieces)
            T = 0
            done_cost = 0
            pi = 0
            pend_inv = []
            for (cost, fn, tag) in mm:
                if tag == 'fwd':
                    assert pi == len(pieces) and not pend_inv, "fwd for next tile would overwrite live U/G/u"
                fn()
                T += cost
                for i0 in pend_inv:
                    a_inv(ga, i0)
                    T += 64
                pend_inv = []
                target = tot_p * min(1.0, T / t_fill_end)
                kk = 0
                while pi < len(pieces) and done_cost < target:
                    i, r, fin = pieces[pi]
                    dep = None
                    if P['PACE'] and 'pace' in state:
                        pace = state['pace']
                        idx = min(pace.shape[0] // RP - 1, kk * pstep * 8 // RP)
                        pv = pltpu.bitcast(pace[idx * RP:(idx + 1) * RP, :], u32)
                        dep = pltpu.bitcast(lax.shift_right_logical(lax.shift_right_logical(pv, u32(16)), u32(16)), f32)
                        kk += 1
                    a_piece(i, r, dep)
                    done_cost += pcost(i)
                    pi += 1
                    if fin is not None:
                        pend_inv.extend(fin)
            assert pi == len(pieces) and not pend_inv
            if ga is not None:
                cp_oa(ga).start()

        def group_step(g, ga, first):
            KS = D // KSPLIT
            NQ = 4
            QR = S // NQ
            GW = D // 4
            state = {}
            hooks = {}

            def proj_part(name, p, c, ks_):
                x = _bc(xs[pl.ds(c * CH // 2, CH // 2), pl.ds(ks_ * KS, KS)])
                if first:
                    w = _bc(ws[g, p, pl.ds(ks_ * KS // 2, KS // 2), :])
                else:
                    w = _bc(wcur[p, pl.ds(ks_ * KS // 2, KS // 2), :])
                part = _dot(x, w)
                state[name] = part if ks_ == 0 else state[name] + part
                state['pace'] = part
                if ks_ == KSPLIT - 1:
                    for h in hooks.get((name, c), []):
                        h()

            def next_w(p):
                if not first:
                    assert state.get('late_done'), "W(g+1) copied before its DMA was waited for"
                    wcur[p] = ws[g + 1, p]

            def fin_k(c):
                pk = _phi(state.pop('k'))
                pk_s[pl.ds(c * CH, CH), :] = pk.astype(bf16)
                zp = jnp.sum(pk.reshape(CH // 8, 8, G), axis=0)
                state['z'] = zp if c == 0 else state['z'] + zp
                if c == NCH - 1:
                    z_s[g] = state.pop('z')
                    next_w(0)

            def fin_q(c):
                pq_s[g, pl.ds(c * CH, CH), :] = _phi(state.pop('q')).astype(bf16)
                if c == NCH - 1:
                    next_w(1)

            def g_task(n, h):
                a = _ld(pk_s, (n * QR, QR))
                b = _bc(xs[pl.ds(n * QR // 2, QR // 2), pl.ds(h * GW, GW)])
                part = lax.dot_general(a, b, (((0,), (0,)), ((), ())), preferred_element_type=f32)
                state['pace'] = part[:, 0:G]
                acc = part if n == 0 else state[('G', h)] + part
                if n < NQ - 1:
                    state[('G', h)] = acc
                else:
                    for d in range(GW // G):
                        gm_s[g, h * (GW // G) + d] = acc[:, d * G:(d + 1) * G].astype(bf16)

            def fwd_task(j):
                assert state.get('late_done')
                if j == 0:
                    state['sk'] = load_sk(g)
                    state['dvec'] = load_d(g)
                a_fwd(g, state['sk'], state['dvec'], j)

            def wait_all(cps, nm="w"):
                if True:
                    for c in cps:
                        c.wait()

            def wait_late():
                cps = cp_a(g)
                if first:
                    cps = cp_consts() + cps
                else:
                    cps = cps + [cp_w(g + 1, p) for p in range(2)]
                wait_all(cps, 'a')
                state['late_done'] = True

            pc = CH * 8 // KSPLIT // 4
            units = []

            def add_proj(name, p, c, fin):
                for ks_ in range(KSPLIT):
                    def t(ks_=ks_):
                        proj_part(name, p, c, ks_)
                        if ks_ == KSPLIT - 1:
                            fin(c)
                    units.append((pc, t, (name, c)))

            cq = CH * NQ // S if False else None
            per = NCH // NQ
            gq = [(n, h) for n in range(NQ) for h in range(4)]
            gi = 0
            for c in range(NCH):
                add_proj('k', 0, c, fin_k)
                if c >= per and (c % per) * 4 // per != ((c - 1) % per) * 4 // per or (c >= per and c % per == 0):
                    n, h = gq[gi]
                    assert n < c // per
                    units.append((256, functools.partial(g_task, n, h), ('G', gi)))
                    gi += 1
                if c >= P['QLAG']:
                    add_proj('q', 1, c - P['QLAG'], fin_q)
            rest_q = list(range(NCH - P['QLAG'], NCH))
            while gi < len(gq) or rest_q:
                if rest_q:
                    add_proj('q', 1, rest_q.pop(0), fin_q)
                if gi < len(gq):
                    n, h = gq[gi]
                    units.append((256, functools.partial(g_task, n, h), ('G', gi)))
                    gi += 1

            total = sum(u[0] for u in units)
            fwd_start = (P['FWD_START0'] if first else P['FWD_START']) / 16.0 * total
            t_fill_end = P['FILL_END'] / 16.0 * total
            fwd_end = P['FWD_END'] / 16.0 * total
            pos = [fwd_start + (fwd_end - fwd_start) * n / (NB // 2) for n in range(NB // 2)]
            mm = []
            T = 0
            nf = 0
            last_proj = None
            hooked = False
            for (cost, fn, tag) in units:
                while nf < len(pos) and T >= pos[nf]:
                    if not hooked:
                        hooks.setdefault(last_proj, []).append(wait_late)
                        hooked = True
                    mm.append((256, functools.partial(fwd_task, 2 * nf), 'fwd'))
                    nf += 1
                mm.append((cost, fn, None))
                T += cost
                if tag[0] in ('k', 'q'):
                    last_proj = tag
            if not hooked:
                hooks.setdefault(last_proj, []).append(wait_late)
            while nf < len(pos):
                mm.append((256, functools.partial(fwd_task, 2 * nf), 'fwd'))
                nf += 1
            if first:
                for grp, lo in X_GROUPS:
                    hooks.setdefault(('k', lo - 1), []).append(
                        functools.partial(lambda grp: wait_all([cp_x(c) for c in grp], 'x%d' % grp[0]), grp))
            emit(mm, state, ga, t_fill_end, P['ORDER'], P['PSTEP'])
            if first:
                wait_all([cp_w(1, p) for p in range(2)], 'w1')
                for p in range(2):
                    wcur[p] = ws[1, p]

        def tile_rows(t):
            t0 = t * (RT // 2)
            return pl.ds(t0 if isinstance(t, int) else pl.multiple_of(t0, RT // 2), RT // 2)

        def norm_tasks(t, state):
            pq32 = pq_s.bitcast(u32)

            def norm(gs):
                for g in gs:
                    pq = _bc(pq32[g, tile_rows(t), :])
                    den = _dot(pq, _ld(zb_s, g, (0, G))) + 1e-6
                    pqn_s[g] = (pq.astype(f32) * pl.reciprocal(den, approx=True)).astype(bf16)
                    state['pace'] = den
            return [(RT, functools.partial(norm, range(0, 4)), None), (RT, functools.partial(norm, range(4, 8)), None)]

        def proj_tasks(t, state):
            loc = {}

            def proj(j):
                if 'lhs' not in loc:
                    loc['lhs'] = jnp.concatenate([_ld(pqn_s, g, (0, RT)) for g in range(NG)], axis=1)
                res = _dot(loc['lhs'], _ld(M_s, j, (0, D)))
                ob_s[t, j] = res.astype(bf16)
                state['pace'] = res
                cp_ob(t, j).start()
            return [(2 * RT, functools.partial(proj, j), None) for j in range(NG)]

        def tile_tasks(t, state, norm_next):
            pr = proj_tasks(t, state)
            if not norm_next:
                return pr
            nm = norm_tasks(t + 1, state)
            a, b = P['NPOS'], P['NPOS'] + 2
            return pr[:a] + nm[:1] + pr[a:b] + nm[1:] + pr[b:]

        def m_tasks(state):
            r = lax.broadcasted_iota(jnp.int32, (G, G), 0) // HEAD
            c = lax.broadcasted_iota(jnp.int32, (G, G), 1) // HEAD
            bd = r == c

            def mt(g):
                z = jnp.sum(z_s[g], axis=0, keepdims=True)
                zc = jnp.broadcast_to(z, (G, G)).T
                zb_s[g] = jnp.where(bd, zc, 0.0).astype(bf16)
                gm = jnp.concatenate([_ld(gm_s, g, j, (0, G)) for j in range(NG)], axis=1)
                kv = _dot(gm, _bc(wvs[:, pl.ds(g * G, G)]))
                kvb = jnp.where(bd, kv, 0.0).astype(bf16)
                wo = _bc(wos[pl.ds(g * G // 2, G // 2), :])
                Mg = _dot(kvb, wo)
                state['pace'] = Mg[:, 0:G]
                for j in range(NG):
                    M_s[j, pl.ds(g * G, G), :] = Mg[:, j * G:(j + 1) * G].astype(bf16)
            return [(512, functools.partial(mt, g), None) for g in range(NG)]

        @pl.when(step == 0)
        def _():
            ks[:, 0:8, :] = jnp.zeros((NG, 8, G), u32)
            cp_w(0, 0).start()
            cp_x(0).start()
            cp_w(0, 1).start()
            for c in range(1, NCH):
                cp_x(c).start()
            for c in cp_consts():
                c.start()
            for c in cp_a(0):
                c.start()
            for g in range(1, NG + 1):
                for p in range(2):
                    cp_w(g, p).start()
                cp_q(g - 1).start()
                if g < NG:
                    for c in cp_a(g):
                        c.start()
            for c in cp_wo():
                c.start()
            if True:
                cp_w(0, 0).wait()
                cp_x(0).wait()
                cp_w(0, 1).wait()
            group_step(0, None, True)

        @pl.when(jnp.logical_and(step > 0, step < NG))
        def _():
            cp_q(step - 1).wait()
            group_step(step, step - 1, False)

        @pl.when(step == NG)
        def _():
            for c in cp_wo():
                c.wait()
            cp_q(NG - 1).wait()
            state = {}
            mt = m_tasks(state)
            nm = norm_tasks(0, state)
            mm = mt[:P['NM0']] + nm[:1] + mt[P['NM0']:] + nm[1:] if P['NM0'] < NG else mt + nm
            for t in range(NTA):
                mm += tile_tasks(t, state, True)
            emit(mm, state, NG - 1, sum(m[0] for m in mm) * P['FILL_END_F'], P['ORDER_F'], P['PSTEP_F'])

        if NSTEPS - 1 - NG > 1:
            @pl.when(jnp.logical_and(step > NG, step < NSTEPS - 1))
            def _():
                state = {}
                for (_, fn, _) in tile_tasks(step - (NG + 1) + NTA, state, True):
                    fn()

        @pl.when(step == NSTEPS - 1)
        def _():
            state = {}
            for t in range(NT - NTL, NT):
                for (_, fn, _) in tile_tasks(t, state, t < NT - 1):
                    fn()
            pltpu.make_async_copy(oa_s, oa_s, sem_oa.at[0]).wait()
            pltpu.make_async_copy(ob_s, ob_s, sem_ob.at[0]).wait()

    scratch = [
        pltpu.VMEM((NG, S // 2, G), u32), pltpu.VMEM((NG, 8 + S // 2, G), u32), pltpu.VMEM((NG, S // 2, G), u32),
        pltpu.VMEM((4, D), bf16), pltpu.VMEM((NG, G // 2, S), u32), pltpu.VMEM((8, 128), bf16),
        pltpu.VMEM((256, 128), u32), pltpu.VMEM((64, 128), u32),
        pltpu.VMEM((S // 2, D), u32), pltpu.VMEM((NG + 1, 2, D // 2, G), u32), pltpu.VMEM((D // 2, D), u32),
        pltpu.VMEM((D // 2, D), u32), pltpu.VMEM((2, D // 2, G), u32),
        pltpu.VMEM((NB, 256, G), f32), pltpu.VMEM((256, G), f32), pltpu.VMEM((NB, 256, G), f32),
        pltpu.VMEM((NB, 2, 128, G), bf16), pltpu.VMEM((NG, S, G), bf16),
        pltpu.VMEM((S, G), bf16), pltpu.VMEM((NG, NG, G, G), bf16), pltpu.VMEM((NG, S, G), bf16),
        pltpu.VMEM((NG, 8, G), f32),
        pltpu.VMEM((NG, D, G), bf16), pltpu.VMEM((NG, G, G), bf16), pltpu.VMEM((NT, NG, RT, G), bf16),
        pltpu.VMEM((NG, RT, G), bf16),
        pltpu.SemaphoreType.DMA((4,)), pltpu.SemaphoreType.DMA((NCH,)), pltpu.SemaphoreType.DMA((2 * (NG + 1),)),
        pltpu.SemaphoreType.DMA((NG,)), pltpu.SemaphoreType.DMA((NG,)), pltpu.SemaphoreType.DMA((2,)),
        pltpu.SemaphoreType.DMA((1,)), pltpu.SemaphoreType.DMA((1,)),
    ]
    return kernel, scratch, NSTEPS


_KERNEL, _SCRATCH, _NSTEPS = make_kernel(PARAMS)
_FP, _FIP = _dft_mats(PARAMS['RP'])


@jax.jit
def pallas_concat_heads__ssm_conv_h3__linear_attn_block__prompt_kernel(A_q, A_k, A_v, A_shift_k, A_ssm_k, A_ssm_D, B_x, B_wqkv, B_wo):
    out = pl.pallas_call(
        _KERNEL, grid=(_NSTEPS,),
        in_specs=[pl.BlockSpec(memory_space=pl.ANY)] * 11,
        out_specs=pl.BlockSpec(memory_space=pl.ANY),
        out_shape=jax.ShapeDtypeStruct((S, 2 * D), bf16),
        scratch_shapes=_SCRATCH,
        compiler_params=pltpu.CompilerParams(vmem_limit_bytes=110 * 1024 * 1024, dimension_semantics=("arbitrary",)),
    )(A_q.reshape(S, D), A_k.reshape(S, D), A_v.reshape(S, D), A_shift_k.T, A_ssm_k, A_ssm_D.reshape(8, 128),
      jnp.asarray(_FP), jnp.asarray(_FIP), B_x.reshape(S, D), B_wqkv, B_wo)
    return out.reshape(1, S, 2 * D)
```

```python
import functools

import jax
import jax.numpy as jnp
import numpy as np
from jax import lax
from jax.experimental import pallas as pl
from jax.experimental.pallas import tpu as pltpu

f32, bf16, u32 = jnp.float32, jnp.bfloat16, jnp.uint32

S, D = 2048, 1024
G = 128
NG = D // G
HEAD = 32
B = 128
NB = S // B
RP = 8
NR = 128 // RP
TI = 4
CH = 128
NCH = S // CH
KSPLIT = 2
KS = D // KSPLIT
NQ = 4
QR = S // NQ
GW = D // 4
RT = 256
NT = S // RT
NTA = 4
NSTEPS = NG + 2

FWD_START, FWD_END, FILL_END = 14.0 / 16, 1.0, 13.9 / 16
FILL_END_LAST = 0.9
PACE_STRIDE = 8
X_GROUPS = ((1, 2), (2, 4), (4, 7), (7, 11), (11, 16))


def _pack_rows(a):
    b = np.asarray(a, dtype=bf16).view(np.uint16).astype(np.uint32)
    return b[0::2] | (b[1::2] << 16)


def _dft_mats():
    ks = np.concatenate([np.arange(0, 128, 2), np.arange(1, 128, 2)])
    sg = np.where(ks % 2 == 0, 1.0, -1.0)[:, None]
    th = (np.pi * (2 * ks + 1) / 256.0)[:, None]
    t = np.arange(128)[None, :]

    def inter(re, im):
        rows = []
        for r in range(NR):
            rows.append(re[r * RP:(r + 1) * RP])
            rows.append(im[r * RP:(r + 1) * RP])
        return np.concatenate(rows, axis=0)

    hre, him = np.cos(th * t), -np.sin(th * t)
    ure, uim = np.cos(th * (t + 0.5)), -np.sin(th * (t + 0.5))
    fu = inter(ure - sg * uim, uim + sg * ure)
    fu = np.concatenate([fu[:, 0::2], fu[:, 1::2]], axis=1)
    fh = inter(hre, him)
    phi = th * (np.arange(64)[None, :] + 0.5)
    c1 = ((np.cos(phi) + sg * np.sin(phi)) / 256.0).T
    c2 = ((sg * np.cos(phi) - np.sin(phi)) / 256.0).T
    fwd = np.concatenate([_pack_rows(fu), _pack_rows(fh)], axis=0)
    inv = np.concatenate([_pack_rows(c1), _pack_rows(c2)], axis=0)
    return fwd, inv


def _phi(t):
    return jnp.where(t > 0, t + 1.0, jnp.exp(t)) + 1e-6


def _dot(a, b):
    return jnp.dot(a, b, preferred_element_type=f32)


def _bc(x):
    return pltpu.bitcast(x, bf16)


def _ld(ref, *idx):
    *lead, (r0, n) = idx
    return _bc(ref.bitcast(u32)[(*lead, pl.ds(r0 // 2, n // 2), slice(None))])


def _kernel(q_hbm, k_hbm, v_hbm, sk_hbm, h_hbm, d_hbm, f_hbm, fi_hbm, x_hbm, w_hbm, wo_hbm, o_hbm,
            qs, ks, vs, sks, hs, ds_, fs, fis, xs, ws, wos, wvs, wcur,
            U_s, H_s, G_s, Z_s, oa_s, pk_s, gm_s, pq_s, z_s, M_s, zb_s, ob_s, pqn_s,
            sem_c, sem_x, sem_w, sem_a, sem_q, sem_wo, sem_oa, sem_ob):
    step = pl.program_id(0)
    q32, k32, v32, h32 = (r.bitcast(u32) for r in (q_hbm, k_hbm, v_hbm, h_hbm))
    x32, w32, wo32 = (r.bitcast(u32) for r in (x_hbm, w_hbm, wo_hbm))

    def col(g):
        return pl.ds(pl.multiple_of(g * G, G), G)

    def cp_consts():
        return [pltpu.make_async_copy(a, b, sem_c.at[n]) for n, (a, b) in
                enumerate(((f_hbm, fs), (fi_hbm, fis), (sk_hbm, sks), (d_hbm, ds_)))]

    def cp_x(c):
        rows = pl.ds(c * (CH // 2), CH // 2)
        return pltpu.make_async_copy(x32.at[rows], xs.at[rows], sem_x.at[c])

    def cp_w(g, p):
        gs = min(g, NG - 1) if isinstance(g, int) else jnp.minimum(g, NG - 1)
        off = (D, 0)[p]
        cols = pl.ds(off + gs * G if isinstance(gs, int) else pl.multiple_of(off + gs * G, G), G)
        return pltpu.make_async_copy(w32.at[:, cols], ws.at[g, p], sem_w.at[2 * g + p])

    def cp_a(g):
        return [pltpu.make_async_copy(k32.at[:, col(g)], ks.at[g, pl.ds(8, S // 2)], sem_a.at[g]),
                pltpu.make_async_copy(v32.at[:, col(g)], vs.at[g], sem_a.at[g]),
                pltpu.make_async_copy(h32.at[pl.ds(pl.multiple_of(g * (G // 2), G // 2), G // 2)], hs.at[g], sem_a.at[g])]

    def cp_q(g):
        return pltpu.make_async_copy(q32.at[:, col(g)], qs.at[g], sem_q.at[g])

    def cp_wo():
        return [pltpu.make_async_copy(wo32, wos, sem_wo.at[0]),
                pltpu.make_async_copy(w32.at[:, pl.ds(2 * D, D)], wvs, sem_wo.at[1])]

    def cp_oa(g):
        return pltpu.make_async_copy(oa_s.at[g], o_hbm.at[:, col(g)], sem_oa.at[0])

    def cp_ob(t, j):
        return pltpu.make_async_copy(ob_s.at[t, j], o_hbm.at[pl.ds(t * RT, RT), pl.ds(D + j * G, G)], sem_ob.at[0])

    def wait_all(cps):
        for c in cps:
            c.wait()

    def a_pre(g, sk, j):
        n = B // 2
        w0 = 8 + j * n
        lo = lambda x: pltpu.bitcast(lax.shift_left(x, u32(16)), f32)
        hi = lambda x: pltpu.bitcast(x & u32(0xFFFF0000), f32)
        k0, k1, k2 = (ks[g, pl.ds(w0 - d, n), :] for d in range(3))
        e0, o0, e1, o1, o2 = lo(k0), hi(k0), lo(k1), hi(k1), hi(k2)
        s0, s1, s2, s3 = (sk[t:t + 1, :] for t in range(4))
        ye = e0 * s0 + o1 * s1 + e1 * s2 + o2 * s3
        yo = o0 * s0 + e0 * s1 + o1 * s2 + e1 * s3
        vv = vs[g, pl.ds(j * n, n), :]
        return jnp.concatenate([ye * lo(vv), yo * hi(vv)], axis=0).astype(bf16)

    def a_fwd(g, sk, dvec, j0):
        u2 = jnp.concatenate([a_pre(g, sk, j0), a_pre(g, sk, j0 + 1)], axis=1)
        U2 = _dot(_bc(fs[0:128, :]), u2)
        h2 = jnp.concatenate([_bc(hs[g, :, pl.ds((j0 + d) * B, B)]) for d in range(2)], axis=0)
        H2 = lax.dot_general(_bc(fs[128:256, :]), h2, (((1,), (1,)), ((), ())), preferred_element_type=f32)
        if j0 == 0:
            h0 = jnp.concatenate(
                [H2[r * RP:(r + 1) * RP, 0:G] + dvec if r % 2 == 0 else H2[r * RP:(r + 1) * RP, 0:G]
                 for r in range(2 * NR)], axis=0)
        for d in range(2):
            j = j0 + d
            U_s[j] = U2[:, d * G:(d + 1) * G]
            H = H2[:, d * G:(d + 1) * G]
            if j == 0:
                G_s[0] = h0
            else:
                for r in range(NR):
                    a, b = 2 * r * RP, (2 * r + 1) * RP
                    hre, him = H[a:a + RP], H[b:b + RP]
                    if d == 0:
                        pre, pim = H_s[pl.ds(a, RP), :], H_s[pl.ds(b, RP), :]
                    else:
                        hp = h0 if j0 == 0 else H2[:, 0:G]
                        pre, pim = hp[a:a + RP], hp[b:b + RP]
                    if r < NR // 2:
                        G_s[j, pl.ds(a, RP), :] = hre - pim
                        G_s[j, pl.ds(b, RP), :] = him + pre
                    else:
                        G_s[j, pl.ds(a, RP), :] = hre + pim
                        G_s[j, pl.ds(b, RP), :] = him - pre
        if j0 + 2 < NB:
            H_s[...] = H2[:, G:2 * G]

    def load_sk(g):
        return sks[:, col(g)].astype(f32)

    def load_d(g):
        dall = ds_[...].astype(f32)
        rows = lax.broadcasted_iota(jnp.int32, (8, G), 0)
        return jnp.sum(jnp.where(rows == g, dall, 0.0), axis=0, keepdims=True)

    held = {}

    def a_piece(i0, r, dep):
        a, b = 2 * r * RP, (2 * r + 1) * RP
        acc = [(dep, dep)] * TI
        gw = {}
        for j in range(i0 + TI):
            ure, uim = U_s[j, pl.ds(a, RP), :], U_s[j, pl.ds(b, RP), :]
            for t in range(TI):
                m = i0 + t - j
                if m < 0:
                    continue
                if m not in gw:
                    gw[m] = (G_s[m, pl.ds(a, RP), :], G_s[m, pl.ds(b, RP), :])
                gre, gim = gw[m]
                tre = gre * ure - gim * uim
                tim = gre * uim + gim * ure
                zre, zim = acc[t]
                acc[t] = (tre if zre is None else zre + tre, tim if zim is None else zim + tim)
        if r % 2 == 0:
            held[(i0, r)] = acc
        else:
            prev = held.pop((i0, r - 1))
            for t in range(TI):
                for c in range(2):
                    z = jnp.concatenate([prev[t][c], acc[t][c]], axis=0)
                    Z_s[i0 + t, c, pl.ds((r - 1) * RP, 2 * RP), :] = z.astype(bf16)

    def a_inv(g, i0):
        e2 = _dot(_bc(fis[0:32, :]), jnp.concatenate([_ld(Z_s, i0 + d, 0, (0, 128)) for d in range(2)], axis=1))
        o2 = _dot(_bc(fis[32:64, :]), jnp.concatenate([_ld(Z_s, i0 + d, 1, (0, 128)) for d in range(2)], axis=1))
        rev = 7 - lax.broadcasted_iota(jnp.int32, (8, G), 0)
        for d in range(2):
            r0 = (i0 + d) * B
            e, o = e2[:, d * G:(d + 1) * G], o2[:, d * G:(d + 1) * G]
            hi = e - o
            y = jnp.concatenate(
                [e + o] + [jnp.take_along_axis(hi[8 * (7 - v):8 * (8 - v)], rev, axis=0) for v in range(8)], axis=0)
            qq = _bc(qs[g, pl.ds(r0 // 2, B // 2), :]).astype(f32)
            oa_s[g, pl.ds(r0, B), :] = (qq * y).astype(bf16)

    def emit(mm, state, ga, t_fill_end):
        pieces = []
        if ga is not None:
            for i0 in range(NB - TI, -1, -TI):
                pieces += [(i0, r) for r in range(NR)]
        cost_of = lambda i0: sum(i + 1 for i in range(i0, i0 + TI))
        total = sum(cost_of(i0) for i0, _ in pieces)
        t_now, done, nxt, pend_inv = 0, 0, 0, []
        for (cost, fn, is_fwd) in mm:
            if is_fwd:
                assert nxt == len(pieces) and not pend_inv, "the next tile's transforms overwrite U / G"
            fn()
            t_now += cost
            for i0 in pend_inv:
                a_inv(ga, i0)
                t_now += 64
            pend_inv = []
            target = total * min(1.0, t_now / t_fill_end)
            kk = 0
            while nxt < len(pieces) and done < target:
                i0, r = pieces[nxt]
                dep = None
                if 'pace' in state:
                    pace = state['pace']
                    idx = min(pace.shape[0] // RP - 1, kk * PACE_STRIDE)
                    pv = pltpu.bitcast(pace[idx * RP:(idx + 1) * RP, :], u32)
                    dep = pltpu.bitcast(lax.shift_right_logical(lax.shift_right_logical(pv, u32(16)), u32(16)), f32)
                    kk += 1
                a_piece(i0, r, dep)
                done += cost_of(i0)
                nxt += 1
                if r == NR - 1:
                    pend_inv.extend(range(i0, i0 + TI, 2))
        assert nxt == len(pieces) and not pend_inv
        if ga is not None:
            cp_oa(ga).start()

    def group_step(g, ga, first):
        state = {}
        hooks = {}

        def proj_part(name, p, c, ks_):
            x = _bc(xs[pl.ds(c * CH // 2, CH // 2), pl.ds(ks_ * KS, KS)])
            wref = ws.at[g, p] if first else wcur.at[p]
            part = _dot(x, _bc(wref[pl.ds(ks_ * KS // 2, KS // 2), :]))
            state[name] = part if ks_ == 0 else state[name] + part
            state['pace'] = part
            if ks_ == KSPLIT - 1:
                for h in hooks.get((name, c), []):
                    h()

        def next_w(p):
            if not first:
                assert state.get('late_done')
                wcur[p] = ws[g + 1, p]

        def fin_k(c):
            pk = _phi(state.pop('k'))
            pk_s[pl.ds(c * CH, CH), :] = pk.astype(bf16)
            zp = jnp.sum(pk.reshape(CH // 8, 8, G), axis=0)
            state['z'] = zp if c == 0 else state['z'] + zp
            if c == NCH - 1:
                z_s[g] = state.pop('z')
                next_w(0)

        def fin_q(c):
            pq_s[g, pl.ds(c * CH, CH), :] = _phi(state.pop('q')).astype(bf16)
            if c == NCH - 1:
                next_w(1)

        def g_task(n, h):
            a = _ld(pk_s, (n * QR, QR))
            b = _bc(xs[pl.ds(n * QR // 2, QR // 2), pl.ds(h * GW, GW)])
            part = lax.dot_general(a, b, (((0,), (0,)), ((), ())), preferred_element_type=f32)
            state['pace'] = part[:, 0:G]
            acc = part if n == 0 else state[('G', h)] + part
            if n < NQ - 1:
                state[('G', h)] = acc
            else:
                for d in range(GW // G):
                    gm_s[g, h * (GW // G) + d] = acc[:, d * G:(d + 1) * G].astype(bf16)

        def fwd_task(j):
            assert state.get('late_done')
            if j == 0:
                state['sk'] = load_sk(g)
                state['dvec'] = load_d(g)
            a_fwd(g, state['sk'], state['dvec'], j)

        def wait_late():
            wait_all((cp_consts() if first else []) + cp_a(g) + ([] if first else [cp_w(g + 1, p) for p in range(2)]))
            state['late_done'] = True

        pc = CH * 8 // KSPLIT // 4
        units = []

        def add_proj(name, p, c, fin):
            for ks_ in range(KSPLIT):
                def t(ks_=ks_):
                    proj_part(name, p, c, ks_)
                    if ks_ == KSPLIT - 1:
                        fin(c)
                units.append((pc, t, (name, c)))

        per = NCH // NQ
        for c in range(NCH):
            add_proj('k', 0, c, fin_k)
            if c >= per:
                units.append((256, functools.partial(g_task, c // per - 1, c % per), ('G', c)))
            if c >= 1:
                add_proj('q', 1, c - 1, fin_q)
        add_proj('q', 1, NCH - 1, fin_q)
        for h in range(per):
            units.append((256, functools.partial(g_task, NQ - 1, h), ('G', NCH + h)))

        total = sum(u[0] for u in units)
        fwd_start, fwd_end = FWD_START * total, FWD_END * total
        pos = [fwd_start + (fwd_end - fwd_start) * n / (NB // 2) for n in range(NB // 2)]
        mm, t_now, nf, last_proj = [], 0, 0, None
        for (cost, fn, tag) in units:
            while nf < len(pos) and t_now >= pos[nf]:
                if nf == 0:
                    hooks.setdefault(last_proj, []).append(wait_late)
                mm.append((256, functools.partial(fwd_task, 2 * nf), True))
                nf += 1
            mm.append((cost, fn, False))
            t_now += cost
            if tag[0] in ('k', 'q'):
                last_proj = tag
        while nf < len(pos):
            mm.append((256, functools.partial(fwd_task, 2 * nf), True))
            nf += 1
        if first:
            for lo, hi in X_GROUPS:
                hooks.setdefault(('k', lo - 1), []).append(
                    functools.partial(lambda lo, hi: wait_all([cp_x(c) for c in range(lo, hi)]), lo, hi))
        emit(mm, state, ga, FILL_END * total)
        if first:
            wait_all([cp_w(1, p) for p in range(2)])
            for p in range(2):
                wcur[p] = ws[1, p]

    def m_tasks(state):
        r = lax.broadcasted_iota(jnp.int32, (G, G), 0) // HEAD
        c = lax.broadcasted_iota(jnp.int32, (G, G), 1) // HEAD
        bd = r == c

        def mt(g):
            z = jnp.sum(z_s[g], axis=0, keepdims=True)
            zc = jnp.broadcast_to(z, (G, G)).T
            zb_s[g] = jnp.where(bd, zc, 0.0).astype(bf16)
            gm = jnp.concatenate([_ld(gm_s, g, j, (0, G)) for j in range(NG)], axis=1)
            kv = _dot(gm, _bc(wvs[:, pl.ds(g * G, G)]))
            kvb = jnp.where(bd, kv, 0.0).astype(bf16)
            Mg = _dot(kvb, _bc(wos[pl.ds(g * G // 2, G // 2), :]))
            state['pace'] = Mg[:, 0:G]
            for j in range(NG):
                M_s[j, pl.ds(g * G, G), :] = Mg[:, j * G:(j + 1) * G].astype(bf16)
        return [(512, functools.partial(mt, g), False) for g in range(NG)]

    def norm_tasks(t, state):
        def norm(gs):
            for g in gs:
                pq = _ld(pq_s, g, (t * RT, RT))
                den = _dot(pq, _ld(zb_s, g, (0, G))) + 1e-6
                pqn_s[g] = (pq.astype(f32) * pl.reciprocal(den, approx=True)).astype(bf16)
                state['pace'] = den
        return [(RT, functools.partial(norm, range(0, 4)), False), (RT, functools.partial(norm, range(4, 8)), False)]

    def tile_tasks(t, state):
        loc = {}

        def proj(j):
            if 'lhs' not in loc:
                loc['lhs'] = jnp.concatenate([_ld(pqn_s, g, (0, RT)) for g in range(NG)], axis=1)
            res = _dot(loc['lhs'], _ld(M_s, j, (0, D)))
            ob_s[t, j] = res.astype(bf16)
            state['pace'] = res
            cp_ob(t, j).start()

        pr = [(2 * RT, functools.partial(proj, j), False) for j in range(NG)]
        if t == NT - 1:
            return pr
        nm = norm_tasks(t + 1, state)
        return pr[:2] + nm[:1] + pr[2:4] + nm[1:] + pr[4:]

    @pl.when(step == 0)
    def _():
        ks[:, 0:8, :] = jnp.zeros((NG, 8, G), u32)
        cp_w(0, 0).start()
        cp_x(0).start()
        cp_w(0, 1).start()
        for c in range(1, NCH):
            cp_x(c).start()
        for c in cp_consts() + cp_a(0):
            c.start()
        for g in range(1, NG + 1):
            for p in range(2):
                cp_w(g, p).start()
            cp_q(g - 1).start()
            if g < NG:
                for c in cp_a(g):
                    c.start()
        for c in cp_wo():
            c.start()
        wait_all([cp_w(0, 0), cp_x(0), cp_w(0, 1)])
        group_step(0, None, True)

    @pl.when(jnp.logical_and(step > 0, step < NG))
    def _():
        cp_q(step - 1).wait()
        group_step(step, step - 1, False)

    @pl.when(step == NG)
    def _():
        wait_all(cp_wo() + [cp_q(NG - 1)])
        state = {}
        mt = m_tasks(state)
        nm = norm_tasks(0, state)
        mm = mt[:6] + nm[:1] + mt[6:] + nm[1:]
        for t in range(NTA):
            mm += tile_tasks(t, state)
        emit(mm, state, NG - 1, sum(m[0] for m in mm) * FILL_END_LAST)

    @pl.when(step == NG + 1)
    def _():
        state = {}
        for t in range(NTA, NT):
            for (_, fn, _) in tile_tasks(t, state):
                fn()
        pltpu.make_async_copy(oa_s, oa_s, sem_oa.at[0]).wait()
        pltpu.make_async_copy(ob_s, ob_s, sem_ob.at[0]).wait()


_SCRATCH = [
    pltpu.VMEM((NG, S // 2, G), u32), pltpu.VMEM((NG, 8 + S // 2, G), u32), pltpu.VMEM((NG, S // 2, G), u32),
    pltpu.VMEM((4, D), bf16), pltpu.VMEM((NG, G // 2, S), u32), pltpu.VMEM((8, 128), bf16),
    pltpu.VMEM((256, 128), u32), pltpu.VMEM((64, 128), u32),
    pltpu.VMEM((S // 2, D), u32), pltpu.VMEM((NG + 1, 2, D // 2, G), u32), pltpu.VMEM((D // 2, D), u32),
    pltpu.VMEM((D // 2, D), u32), pltpu.VMEM((2, D // 2, G), u32),
    pltpu.VMEM((NB, 256, G), f32), pltpu.VMEM((256, G), f32), pltpu.VMEM((NB, 256, G), f32),
    pltpu.VMEM((NB, 2, 128, G), bf16), pltpu.VMEM((NG, S, G), bf16),
    pltpu.VMEM((S, G), bf16), pltpu.VMEM((NG, NG, G, G), bf16), pltpu.VMEM((NG, S, G), bf16),
    pltpu.VMEM((NG, 8, G), f32),
    pltpu.VMEM((NG, D, G), bf16), pltpu.VMEM((NG, G, G), bf16), pltpu.VMEM((NT, NG, RT, G), bf16),
    pltpu.VMEM((NG, RT, G), bf16),
    pltpu.SemaphoreType.DMA((4,)), pltpu.SemaphoreType.DMA((NCH,)), pltpu.SemaphoreType.DMA((2 * (NG + 1),)),
    pltpu.SemaphoreType.DMA((NG,)), pltpu.SemaphoreType.DMA((NG,)), pltpu.SemaphoreType.DMA((2,)),
    pltpu.SemaphoreType.DMA((1,)), pltpu.SemaphoreType.DMA((1,)),
]
_FWD, _INV = _dft_mats()


@jax.jit
def pallas_concat_heads__ssm_conv_h3__linear_attn_block__prompt_kernel(
        A_q, A_k, A_v, A_shift_k, A_ssm_k, A_ssm_D, B_x, B_wqkv, B_wo):
    out = pl.pallas_call(
        _kernel,
        grid=(NSTEPS,),
        in_specs=[pl.BlockSpec(memory_space=pl.ANY)] * 11,
        out_specs=pl.BlockSpec(memory_space=pl.ANY),
        out_shape=jax.ShapeDtypeStruct((S, 2 * D), bf16),
        scratch_shapes=_SCRATCH,
        compiler_params=pltpu.CompilerParams(vmem_limit_bytes=110 * 1024 * 1024, dimension_semantics=("arbitrary",)),
    )(A_q.reshape(S, D), A_k.reshape(S, D), A_v.reshape(S, D), A_shift_k.T, A_ssm_k, A_ssm_D.reshape(8, 128),
      jnp.asarray(_FWD), jnp.asarray(_INV), B_x.reshape(S, D), B_wqkv, B_wo)
    return out.reshape(1, S, 2 * D)
```

```python
import functools

import jax
import jax.numpy as jnp
import numpy as np
from jax import lax
from jax.experimental import pallas as pl
from jax.experimental.pallas import tpu as pltpu

f32, bf16, u32 = jnp.float32, jnp.bfloat16, jnp.uint32

S, D = 2048, 1024
G = 128
NG = D // G
HEAD = 32
B = 128
NB = S // B
RP = 8
NR = 128 // RP
TI = 4
CH = 128
NCH = S // CH
KSPLIT = 2
KS = D // KSPLIT
NQ = 4
QR = S // NQ
GW = D // 4
RT = 256
NT = S // RT
NTA = 4
NSTEPS = NG + 1 + (NT - NTA)

FWD_START, FWD_END, FILL_END = 14.0 / 16, 1.0, 13.9 / 16
FILL_END_LAST = 0.9
PACE_STRIDE = 8
X_GROUPS = ((1, 2), (2, 4), (4, 7), (7, 11), (11, 16))


def _pack_rows(a):
    b = np.asarray(a, dtype=bf16).view(np.uint16).astype(np.uint32)
    return b[0::2] | (b[1::2] << 16)


def _dft_mats():
    ks = np.concatenate([np.arange(0, 128, 2), np.arange(1, 128, 2)])
    sg = np.where(ks % 2 == 0, 1.0, -1.0)[:, None]
    th = (np.pi * (2 * ks + 1) / 256.0)[:, None]
    t = np.arange(128)[None, :]

    def inter(re, im):
        rows = []
        for r in range(NR):
            rows.append(re[r * RP:(r + 1) * RP])
            rows.append(im[r * RP:(r + 1) * RP])
        return np.concatenate(rows, axis=0)

    hre, him = np.cos(th * t), -np.sin(th * t)
    ure, uim = np.cos(th * (t + 0.5)), -np.sin(th * (t + 0.5))
    fu = inter(ure - sg * uim, uim + sg * ure)
    fu = np.concatenate([fu[:, 0::2], fu[:, 1::2]], axis=1)
    fh = inter(hre, him)
    phi = th * (np.arange(64)[None, :] + 0.5)
    c1 = ((np.cos(phi) + sg * np.sin(phi)) / 256.0).T
    c2 = ((sg * np.cos(phi) - np.sin(phi)) / 256.0).T
    fwd = np.concatenate([_pack_rows(fu), _pack_rows(fh)], axis=0)
    inv = np.concatenate([_pack_rows(c1), _pack_rows(c2)], axis=0)
    return fwd, inv


def _phi(t):
    return jnp.where(t > 0, t + 1.0, jnp.exp(t)) + 1e-6


def _dot(a, b):
    return jnp.dot(a, b, preferred_element_type=f32)


def _bc(x):
    return pltpu.bitcast(x, bf16)


def _ld(ref, *idx):
    *lead, (r0, n) = idx
    return _bc(ref.bitcast(u32)[(*lead, pl.ds(r0 // 2, n // 2), slice(None))])


def _kernel(q_hbm, k_hbm, v_hbm, sk_hbm, h_hbm, d_hbm, f_hbm, fi_hbm, x_hbm, w_hbm, wo_hbm, o_hbm,
            qs, ks, vs, sks, hs, ds_, fs, fis, xs, ws, wos, wvs, wcur,
            U_s, H_s, G_s, Z_s, oa_s, pk_s, gm_s, pq_s, z_s, M_s, zb_s, ob_s, pqn_s,
            sem_c, sem_x, sem_w, sem_a, sem_q, sem_wo, sem_oa, sem_ob):
    step = pl.program_id(0)
    q32, k32, v32, h32 = (r.bitcast(u32) for r in (q_hbm, k_hbm, v_hbm, h_hbm))
    x32, w32, wo32 = (r.bitcast(u32) for r in (x_hbm, w_hbm, wo_hbm))

    def col(g):
        return pl.ds(pl.multiple_of(g * G, G), G)

    def cp_consts():
        return [pltpu.make_async_copy(a, b, sem_c.at[n]) for n, (a, b) in
                enumerate(((f_hbm, fs), (fi_hbm, fis), (sk_hbm, sks), (d_hbm, ds_)))]

    def cp_x(c):
        rows = pl.ds(c * (CH // 2), CH // 2)
        return pltpu.make_async_copy(x32.at[rows], xs.at[rows], sem_x.at[c])

    def cp_w(g, p):
        gs = min(g, NG - 1) if isinstance(g, int) else jnp.minimum(g, NG - 1)
        off = (D, 0)[p]
        cols = pl.ds(off + gs * G if isinstance(gs, int) else pl.multiple_of(off + gs * G, G), G)
        return pltpu.make_async_copy(w32.at[:, cols], ws.at[g, p], sem_w.at[2 * g + p])

    def cp_a(g):
        return [pltpu.make_async_copy(k32.at[:, col(g)], ks.at[g, pl.ds(8, S // 2)], sem_a.at[g]),
                pltpu.make_async_copy(v32.at[:, col(g)], vs.at[g], sem_a.at[g]),
                pltpu.make_async_copy(h32.at[pl.ds(pl.multiple_of(g * (G // 2), G // 2), G // 2)], hs.at[g], sem_a.at[g])]

    def cp_q(g):
        return pltpu.make_async_copy(q32.at[:, col(g)], qs.at[g], sem_q.at[g])

    def cp_wo():
        return [pltpu.make_async_copy(wo32, wos, sem_wo.at[0]),
                pltpu.make_async_copy(w32.at[:, pl.ds(2 * D, D)], wvs, sem_wo.at[1])]

    def cp_oa(g):
        return pltpu.make_async_copy(oa_s.at[g], o_hbm.at[:, col(g)], sem_oa.at[0])

    def cp_ob(t, j):
        rows = pl.ds(t * RT if isinstance(t, int) else pl.multiple_of(t * RT, RT), RT)
        return pltpu.make_async_copy(ob_s.at[t, j], o_hbm.at[rows, pl.ds(D + j * G, G)], sem_ob.at[0])

    def wait_all(cps):
        for c in cps:
            c.wait()

    def a_pre(g, sk, j):
        n = B // 2
        w0 = 8 + j * n
        lo = lambda x: pltpu.bitcast(lax.shift_left(x, u32(16)), f32)
        hi = lambda x: pltpu.bitcast(x & u32(0xFFFF0000), f32)
        k0, k1, k2 = (ks[g, pl.ds(w0 - d, n), :] for d in range(3))
        e0, o0, e1, o1, o2 = lo(k0), hi(k0), lo(k1), hi(k1), hi(k2)
        s0, s1, s2, s3 = (sk[t:t + 1, :] for t in range(4))
        ye = e0 * s0 + o1 * s1 + e1 * s2 + o2 * s3
        yo = o0 * s0 + e0 * s1 + o1 * s2 + e1 * s3
        vv = vs[g, pl.ds(j * n, n), :]
        return jnp.concatenate([ye * lo(vv), yo * hi(vv)], axis=0).astype(bf16)

    def a_fwd(g, sk, dvec, j0):
        u2 = jnp.concatenate([a_pre(g, sk, j0), a_pre(g, sk, j0 + 1)], axis=1)
        U2 = _dot(_bc(fs[0:128, :]), u2)
        h2 = jnp.concatenate([_bc(hs[g, :, pl.ds((j0 + d) * B, B)]) for d in range(2)], axis=0)
        H2 = lax.dot_general(_bc(fs[128:256, :]), h2, (((1,), (1,)), ((), ())), preferred_element_type=f32)
        if j0 == 0:
            h0 = jnp.concatenate(
                [H2[r * RP:(r + 1) * RP, 0:G] + dvec if r % 2 == 0 else H2[r * RP:(r + 1) * RP, 0:G]
                 for r in range(2 * NR)], axis=0)
        for d in range(2):
            j = j0 + d
            U_s[j] = U2[:, d * G:(d + 1) * G]
            H = H2[:, d * G:(d + 1) * G]
            if j == 0:
                G_s[0] = h0
            else:
                for r in range(NR):
                    a, b = 2 * r * RP, (2 * r + 1) * RP
                    hre, him = H[a:a + RP], H[b:b + RP]
                    if d == 0:
                        pre, pim = H_s[pl.ds(a, RP), :], H_s[pl.ds(b, RP), :]
                    else:
                        hp = h0 if j0 == 0 else H2[:, 0:G]
                        pre, pim = hp[a:a + RP], hp[b:b + RP]
                    if r < NR // 2:
                        G_s[j, pl.ds(a, RP), :] = hre - pim
                        G_s[j, pl.ds(b, RP), :] = him + pre
                    else:
                        G_s[j, pl.ds(a, RP), :] = hre + pim
                        G_s[j, pl.ds(b, RP), :] = him - pre
        if j0 + 2 < NB:
            H_s[...] = H2[:, G:2 * G]

    def load_sk(g):
        return sks[:, col(g)].astype(f32)

    def load_d(g):
        dall = ds_[...].astype(f32)
        rows = lax.broadcasted_iota(jnp.int32, (8, G), 0)
        return jnp.sum(jnp.where(rows == g, dall, 0.0), axis=0, keepdims=True)

    held = {}

    def a_piece(i0, r, dep):
        a, b = 2 * r * RP, (2 * r + 1) * RP
        acc = [(dep, dep)] * TI
        gw = {}
        for j in range(i0 + TI):
            ure, uim = U_s[j, pl.ds(a, RP), :], U_s[j, pl.ds(b, RP), :]
            for t in range(TI):
                m = i0 + t - j
                if m < 0:
                    continue
                if m not in gw:
                    gw[m] = (G_s[m, pl.ds(a, RP), :], G_s[m, pl.ds(b, RP), :])
                gre, gim = gw[m]
                tre = gre * ure - gim * uim
                tim = gre * uim + gim * ure
                zre, zim = acc[t]
                acc[t] = (tre if zre is None else zre + tre, tim if zim is None else zim + tim)
        if r % 2 == 0:
            held[(i0, r)] = acc
        else:
            prev = held.pop((i0, r - 1))
            for t in range(TI):
                for c in range(2):
                    z = jnp.concatenate([prev[t][c], acc[t][c]], axis=0)
                    Z_s[i0 + t, c, pl.ds((r - 1) * RP, 2 * RP), :] = z.astype(bf16)

    def a_inv(g, i0):
        e2 = _dot(_bc(fis[0:32, :]), jnp.concatenate([_ld(Z_s, i0 + d, 0, (0, 128)) for d in range(2)], axis=1))
        o2 = _dot(_bc(fis[32:64, :]), jnp.concatenate([_ld(Z_s, i0 + d, 1, (0, 128)) for d in range(2)], axis=1))
        rev = 7 - lax.broadcasted_iota(jnp.int32, (8, G), 0)
        for d in range(2):
            r0 = (i0 + d) * B
            e, o = e2[:, d * G:(d + 1) * G], o2[:, d * G:(d + 1) * G]
            hi = e - o
            y = jnp.concatenate(
                [e + o] + [jnp.take_along_axis(hi[8 * (7 - v):8 * (8 - v)], rev, axis=0) for v in range(8)], axis=0)
            qq = _bc(qs[g, pl.ds(r0 // 2, B // 2), :]).astype(f32)
            oa_s[g, pl.ds(r0, B), :] = (qq * y).astype(bf16)

    def emit(mm, state, ga, t_fill_end):
        pieces = []
        if ga is not None:
            for i0 in range(NB - TI, -1, -TI):
                pieces += [(i0, r) for r in range(NR)]
        cost_of = lambda i0: sum(i + 1 for i in range(i0, i0 + TI))
        total = sum(cost_of(i0) for i0, _ in pieces)
        t_now, done, nxt, pend_inv = 0, 0, 0, []
        for (cost, fn, is_fwd) in mm:
            if is_fwd:
                assert nxt == len(pieces) and not pend_inv, "the next tile's transforms overwrite U / G"
            fn()
            t_now += cost
            for i0 in pend_inv:
                a_inv(ga, i0)
                t_now += 64
            pend_inv = []
            target = total * min(1.0, t_now / t_fill_end)
            kk = 0
            while nxt < len(pieces) and done < target:
                i0, r = pieces[nxt]
                dep = None
                if 'pace' in state:
                    pace = state['pace']
                    idx = min(pace.shape[0] // RP - 1, kk * PACE_STRIDE)
                    pv = pltpu.bitcast(pace[idx * RP:(idx + 1) * RP, :], u32)
                    dep = pltpu.bitcast(lax.shift_right_logical(lax.shift_right_logical(pv, u32(16)), u32(16)), f32)
                    kk += 1
                a_piece(i0, r, dep)
                done += cost_of(i0)
                nxt += 1
                if r == NR - 1:
                    pend_inv.extend(range(i0, i0 + TI, 2))
        assert nxt == len(pieces) and not pend_inv
        if ga is not None:
            cp_oa(ga).start()

    def group_step(g, ga, first):
        state = {}
        hooks = {}

        def proj_part(name, p, c, ks_):
            x = _bc(xs[pl.ds(c * CH // 2, CH // 2), pl.ds(ks_ * KS, KS)])
            wref = ws.at[g, p] if first else wcur.at[p]
            part = _dot(x, _bc(wref[pl.ds(ks_ * KS // 2, KS // 2), :]))
            state[name] = part if ks_ == 0 else state[name] + part
            state['pace'] = part
            if ks_ == KSPLIT - 1:
                for h in hooks.get((name, c), []):
                    h()

        def next_w(p):
            if not first:
                assert state.get('late_done')
                wcur[p] = ws[g + 1, p]

        def fin_k(c):
            pk = _phi(state.pop('k'))
            pk_s[pl.ds(c * CH, CH), :] = pk.astype(bf16)
            zp = jnp.sum(pk.reshape(CH // 8, 8, G), axis=0)
            state['z'] = zp if c == 0 else state['z'] + zp
            if c == NCH - 1:
                z_s[g] = state.pop('z')
                next_w(0)

        def fin_q(c):
            pq_s[g, pl.ds(c * CH, CH), :] = _phi(state.pop('q')).astype(bf16)
            if c == NCH - 1:
                next_w(1)

        def g_task(n, h):
            a = _ld(pk_s, (n * QR, QR))
            b = _bc(xs[pl.ds(n * QR // 2, QR // 2), pl.ds(h * GW, GW)])
            part = lax.dot_general(a, b, (((0,), (0,)), ((), ())), preferred_element_type=f32)
            state['pace'] = part[:, 0:G]
            acc = part if n == 0 else state[('G', h)] + part
            if n < NQ - 1:
                state[('G', h)] = acc
            else:
                for d in range(GW // G):
                    gm_s[g, h * (GW // G) + d] = acc[:, d * G:(d + 1) * G].astype(bf16)

        def fwd_task(j):
            assert state.get('late_done')
            if j == 0:
                state['sk'] = load_sk(g)
                state['dvec'] = load_d(g)
            a_fwd(g, state['sk'], state['dvec'], j)

        def wait_late():
            wait_all((cp_consts() if first else []) + cp_a(g) + ([] if first else [cp_w(g + 1, p) for p in range(2)]))
            state['late_done'] = True

        pc = CH * 8 // KSPLIT // 4
        units = []

        def add_proj(name, p, c, fin):
            for ks_ in range(KSPLIT):
                def t(ks_=ks_):
                    proj_part(name, p, c, ks_)
                    if ks_ == KSPLIT - 1:
                        fin(c)
                units.append((pc, t, (name, c)))

        per = NCH // NQ
        for c in range(NCH):
            add_proj('k', 0, c, fin_k)
            if c >= per:
                units.append((256, functools.partial(g_task, c // per - 1, c % per), ('G', c)))
            if c >= 1:
                add_proj('q', 1, c - 1, fin_q)
        add_proj('q', 1, NCH - 1, fin_q)
        for h in range(per):
            units.append((256, functools.partial(g_task, NQ - 1, h), ('G', NCH + h)))

        total = sum(u[0] for u in units)
        fwd_start, fwd_end = FWD_START * total, FWD_END * total
        pos = [fwd_start + (fwd_end - fwd_start) * n / (NB // 2) for n in range(NB // 2)]
        mm, t_now, nf, last_proj = [], 0, 0, None
        for (cost, fn, tag) in units:
            while nf < len(pos) and t_now >= pos[nf]:
                if nf == 0:
                    hooks.setdefault(last_proj, []).append(wait_late)
                mm.append((256, functools.partial(fwd_task, 2 * nf), True))
                nf += 1
            mm.append((cost, fn, False))
            t_now += cost
            if tag[0] in ('k', 'q'):
                last_proj = tag
        while nf < len(pos):
            mm.append((256, functools.partial(fwd_task, 2 * nf), True))
            nf += 1
        if first:
            for lo, hi in X_GROUPS:
                hooks.setdefault(('k', lo - 1), []).append(
                    functools.partial(lambda lo, hi: wait_all([cp_x(c) for c in range(lo, hi)]), lo, hi))
        emit(mm, state, ga, FILL_END * total)
        if first:
            wait_all([cp_w(1, p) for p in range(2)])
            for p in range(2):
                wcur[p] = ws[1, p]

    def m_tasks(state):
        r = lax.broadcasted_iota(jnp.int32, (G, G), 0) // HEAD
        c = lax.broadcasted_iota(jnp.int32, (G, G), 1) // HEAD
        bd = r == c

        def mt(g):
            z = jnp.sum(z_s[g], axis=0, keepdims=True)
            zc = jnp.broadcast_to(z, (G, G)).T
            zb_s[g] = jnp.where(bd, zc, 0.0).astype(bf16)
            gm = jnp.concatenate([_ld(gm_s, g, j, (0, G)) for j in range(NG)], axis=1)
            kv = _dot(gm, _bc(wvs[:, pl.ds(g * G, G)]))
            kvb = jnp.where(bd, kv, 0.0).astype(bf16)
            Mg = _dot(kvb, _bc(wos[pl.ds(g * G // 2, G // 2), :]))
            state['pace'] = Mg[:, 0:G]
            for j in range(NG):
                M_s[j, pl.ds(g * G, G), :] = Mg[:, j * G:(j + 1) * G].astype(bf16)
        return [(512, functools.partial(mt, g), False) for g in range(NG)]

    def norm_tasks(t, state):
        t0 = t * (RT // 2)
        rows = pl.ds(t0 if isinstance(t, int) else pl.multiple_of(t0, RT // 2), RT // 2)

        def norm(gs):
            for g in gs:
                pq = _bc(pq_s.bitcast(u32)[g, rows, :])
                den = _dot(pq, _ld(zb_s, g, (0, G))) + 1e-6
                pqn_s[g] = (pq.astype(f32) * pl.reciprocal(den, approx=True)).astype(bf16)
                state['pace'] = den
        return [(RT, functools.partial(norm, range(0, 4)), False), (RT, functools.partial(norm, range(4, 8)), False)]

    def tile_tasks(t, state, last=False):
        loc = {}

        def proj(j):
            if 'lhs' not in loc:
                loc['lhs'] = jnp.concatenate([_ld(pqn_s, g, (0, RT)) for g in range(NG)], axis=1)
            res = _dot(loc['lhs'], _ld(M_s, j, (0, D)))
            ob_s[t, j] = res.astype(bf16)
            state['pace'] = res
            cp_ob(t, j).start()

        pr = [(2 * RT, functools.partial(proj, j), False) for j in range(NG)]
        if last:
            return pr
        nm = norm_tasks(t + 1, state)
        return pr[:2] + nm[:1] + pr[2:4] + nm[1:] + pr[4:]

    @pl.when(step == 0)
    def _():
        ks[:, 0:8, :] = jnp.zeros((NG, 8, G), u32)
        cp_w(0, 0).start()
        cp_x(0).start()
        cp_w(0, 1).start()
        for c in range(1, NCH):
            cp_x(c).start()
        for c in cp_consts() + cp_a(0):
            c.start()
        for g in range(1, NG + 1):
            for p in range(2):
                cp_w(g, p).start()
            cp_q(g - 1).start()
            if g < NG:
                for c in cp_a(g):
                    c.start()
        for c in cp_wo():
            c.start()
        wait_all([cp_w(0, 0), cp_x(0), cp_w(0, 1)])
        group_step(0, None, True)

    @pl.when(jnp.logical_and(step > 0, step < NG))
    def _():
        cp_q(step - 1).wait()
        group_step(step, step - 1, False)

    @pl.when(step == NG)
    def _():
        wait_all(cp_wo() + [cp_q(NG - 1)])
        state = {}
        mt = m_tasks(state)
        nm = norm_tasks(0, state)
        mm = mt[:6] + nm[:1] + mt[6:] + nm[1:]
        for t in range(NTA):
            mm += tile_tasks(t, state)
        emit(mm, state, NG - 1, sum(m[0] for m in mm) * FILL_END_LAST)

    @pl.when(jnp.logical_and(step > NG, step < NSTEPS - 1))
    def _():
        for (_, fn, _) in tile_tasks(step - (NG + 1) + NTA, {}):
            fn()

    @pl.when(step == NSTEPS - 1)
    def _():
        for (_, fn, _) in tile_tasks(NT - 1, {}, last=True):
            fn()
        pltpu.make_async_copy(oa_s, oa_s, sem_oa.at[0]).wait()
        pltpu.make_async_copy(ob_s, ob_s, sem_ob.at[0]).wait()


_SCRATCH = [
    pltpu.VMEM((NG, S // 2, G), u32), pltpu.VMEM((NG, 8 + S // 2, G), u32), pltpu.VMEM((NG, S // 2, G), u32),
    pltpu.VMEM((4, D), bf16), pltpu.VMEM((NG, G // 2, S), u32), pltpu.VMEM((8, 128), bf16),
    pltpu.VMEM((256, 128), u32), pltpu.VMEM((64, 128), u32),
    pltpu.VMEM((S // 2, D), u32), pltpu.VMEM((NG + 1, 2, D // 2, G), u32), pltpu.VMEM((D // 2, D), u32),
    pltpu.VMEM((D // 2, D), u32), pltpu.VMEM((2, D // 2, G), u32),
    pltpu.VMEM((NB, 256, G), f32), pltpu.VMEM((256, G), f32), pltpu.VMEM((NB, 256, G), f32),
    pltpu.VMEM((NB, 2, 128, G), bf16), pltpu.VMEM((NG, S, G), bf16),
    pltpu.VMEM((S, G), bf16), pltpu.VMEM((NG, NG, G, G), bf16), pltpu.VMEM((NG, S, G), bf16),
    pltpu.VMEM((NG, 8, G), f32),
    pltpu.VMEM((NG, D, G), bf16), pltpu.VMEM((NG, G, G), bf16), pltpu.VMEM((NT, NG, RT, G), bf16),
    pltpu.VMEM((NG, RT, G), bf16),
    pltpu.SemaphoreType.DMA((4,)), pltpu.SemaphoreType.DMA((NCH,)), pltpu.SemaphoreType.DMA((2 * (NG + 1),)),
    pltpu.SemaphoreType.DMA((NG,)), pltpu.SemaphoreType.DMA((NG,)), pltpu.SemaphoreType.DMA((2,)),
    pltpu.SemaphoreType.DMA((1,)), pltpu.SemaphoreType.DMA((1,)),
]
_FWD, _INV = _dft_mats()


@jax.jit
def pallas_concat_heads__ssm_conv_h3__linear_attn_block__prompt_kernel(
        A_q, A_k, A_v, A_shift_k, A_ssm_k, A_ssm_D, B_x, B_wqkv, B_wo):
    out = pl.pallas_call(
        _kernel,
        grid=(NSTEPS,),
        in_specs=[pl.BlockSpec(memory_space=pl.ANY)] * 11,
        out_specs=pl.BlockSpec(memory_space=pl.ANY),
        out_shape=jax.ShapeDtypeStruct((S, 2 * D), bf16),
        scratch_shapes=_SCRATCH,
        compiler_params=pltpu.CompilerParams(vmem_limit_bytes=110 * 1024 * 1024, dimension_semantics=("arbitrary",)),
    )(A_q.reshape(S, D), A_k.reshape(S, D), A_v.reshape(S, D), A_shift_k.T, A_ssm_k, A_ssm_D.reshape(8, 128),
      jnp.asarray(_FWD), jnp.asarray(_INV), B_x.reshape(S, D), B_wqkv, B_wo)
    return out.reshape(1, S, 2 * D)
```

```python
import functools

import jax
import jax.numpy as jnp
import numpy as np
from jax import lax
from jax.experimental import pallas as pl
from jax.experimental.pallas import tpu as pltpu

f32, bf16, u32 = jnp.float32, jnp.bfloat16, jnp.uint32

S, D = 2048, 1024
G = 128
NG = D // G
HEAD = 32
B = 128
NB = S // B
RP = 8
NR = 128 // RP
TI = 4
CH = 128
NCH = S // CH
KSPLIT = 2
KS = D // KSPLIT
NQ = 4
QR = S // NQ
GW = D // 4
RT = 256
NT = S // RT
NTA = 4
NTL = 2
NSTEPS = NG + 2 + (NT - NTA - NTL)

FWD_START, FWD_END, FILL_END = 14.0 / 16, 1.0, 13.9 / 16
FILL_END_LAST = 0.9
PACE_STRIDE = 8
X_GROUPS = ((1, 2), (2, 4), (4, 7), (7, 11), (11, 16))


def _pack_rows(a):
    b = np.asarray(a, dtype=bf16).view(np.uint16).astype(np.uint32)
    return b[0::2] | (b[1::2] << 16)


def _dft_mats():
    ks = np.concatenate([np.arange(0, 128, 2), np.arange(1, 128, 2)])
    sg = np.where(ks % 2 == 0, 1.0, -1.0)[:, None]
    th = (np.pi * (2 * ks + 1) / 256.0)[:, None]
    t = np.arange(128)[None, :]

    def inter(re, im):
        rows = []
        for r in range(NR):
            rows.append(re[r * RP:(r + 1) * RP])
            rows.append(im[r * RP:(r + 1) * RP])
        return np.concatenate(rows, axis=0)

    hre, him = np.cos(th * t), -np.sin(th * t)
    ure, uim = np.cos(th * (t + 0.5)), -np.sin(th * (t + 0.5))
    fu = inter(ure - sg * uim, uim + sg * ure)
    fu = np.concatenate([fu[:, 0::2], fu[:, 1::2]], axis=1)
    fh = inter(hre, him)
    phi = th * (np.arange(64)[None, :] + 0.5)
    c1 = ((np.cos(phi) + sg * np.sin(phi)) / 256.0).T
    c2 = ((sg * np.cos(phi) - np.sin(phi)) / 256.0).T
    fwd = np.concatenate([_pack_rows(fu), _pack_rows(fh)], axis=0)
    inv = np.concatenate([_pack_rows(c1), _pack_rows(c2)], axis=0)
    return fwd, inv


def _phi(t):
    return jnp.where(t > 0, t + 1.0, jnp.exp(t)) + 1e-6


def _dot(a, b):
    return jnp.dot(a, b, preferred_element_type=f32)


def _bc(x):
    return pltpu.bitcast(x, bf16)


def _ld(ref, *idx):
    *lead, (r0, n) = idx
    return _bc(ref.bitcast(u32)[(*lead, pl.ds(r0 // 2, n // 2), slice(None))])


def _kernel(q_hbm, k_hbm, v_hbm, sk_hbm, h_hbm, d_hbm, f_hbm, fi_hbm, x_hbm, w_hbm, wo_hbm, o_hbm,
            qs, ks, vs, sks, hs, ds_, fs, fis, xs, ws, wos, wvs, wcur,
            U_s, H_s, G_s, Z_s, oa_s, pk_s, gm_s, pq_s, z_s, M_s, zb_s, ob_s, pqn_s,
            sem_c, sem_x, sem_w, sem_a, sem_q, sem_wo, sem_oa, sem_ob):
    step = pl.program_id(0)
    q32, k32, v32, h32 = (r.bitcast(u32) for r in (q_hbm, k_hbm, v_hbm, h_hbm))
    x32, w32, wo32 = (r.bitcast(u32) for r in (x_hbm, w_hbm, wo_hbm))

    def col(g):
        return pl.ds(pl.multiple_of(g * G, G), G)

    def cp_consts():
        return [pltpu.make_async_copy(a, b, sem_c.at[n]) for n, (a, b) in
                enumerate(((f_hbm, fs), (fi_hbm, fis), (sk_hbm, sks), (d_hbm, ds_)))]

    def cp_x(c):
        rows = pl.ds(c * (CH // 2), CH // 2)
        return pltpu.make_async_copy(x32.at[rows], xs.at[rows], sem_x.at[c])

    def cp_w(g, p):
        gs = min(g, NG - 1) if isinstance(g, int) else jnp.minimum(g, NG - 1)
        off = (D, 0)[p]
        cols = pl.ds(off + gs * G if isinstance(gs, int) else pl.multiple_of(off + gs * G, G), G)
        return pltpu.make_async_copy(w32.at[:, cols], ws.at[g, p], sem_w.at[2 * g + p])

    def cp_a(g):
        return [pltpu.make_async_copy(k32.at[:, col(g)], ks.at[g, pl.ds(8, S // 2)], sem_a.at[g]),
                pltpu.make_async_copy(v32.at[:, col(g)], vs.at[g], sem_a.at[g]),
                pltpu.make_async_copy(h32.at[pl.ds(pl.multiple_of(g * (G // 2), G // 2), G // 2)], hs.at[g], sem_a.at[g])]

    def cp_q(g):
        return pltpu.make_async_copy(q32.at[:, col(g)], qs.at[g], sem_q.at[g])

    def cp_wo():
        return [pltpu.make_async_copy(wo32, wos, sem_wo.at[0]),
                pltpu.make_async_copy(w32.at[:, pl.ds(2 * D, D)], wvs, sem_wo.at[1])]

    def cp_oa(g):
        return pltpu.make_async_copy(oa_s.at[g], o_hbm.at[:, col(g)], sem_oa.at[0])

    def cp_ob(t, j):
        rows = pl.ds(t * RT if isinstance(t, int) else pl.multiple_of(t * RT, RT), RT)
        return pltpu.make_async_copy(ob_s.at[t, j], o_hbm.at[rows, pl.ds(D + j * G, G)], sem_ob.at[0])

    def wait_all(cps):
        for c in cps:
            c.wait()

    def a_pre(g, sk, j):
        n = B // 2
        w0 = 8 + j * n
        lo = lambda x: pltpu.bitcast(lax.shift_left(x, u32(16)), f32)
        hi = lambda x: pltpu.bitcast(x & u32(0xFFFF0000), f32)
        k0, k1, k2 = (ks[g, pl.ds(w0 - d, n), :] for d in range(3))
        e0, o0, e1, o1, o2 = lo(k0), hi(k0), lo(k1), hi(k1), hi(k2)
        s0, s1, s2, s3 = (sk[t:t + 1, :] for t in range(4))
        ye = e0 * s0 + o1 * s1 + e1 * s2 + o2 * s3
        yo = o0 * s0 + e0 * s1 + o1 * s2 + e1 * s3
        vv = vs[g, pl.ds(j * n, n), :]
        return jnp.concatenate([ye * lo(vv), yo * hi(vv)], axis=0).astype(bf16)

    def a_fwd(g, sk, dvec, j0):
        u2 = jnp.concatenate([a_pre(g, sk, j0), a_pre(g, sk, j0 + 1)], axis=1)
        U2 = _dot(_bc(fs[0:128, :]), u2)
        h2 = jnp.concatenate([_bc(hs[g, :, pl.ds((j0 + d) * B, B)]) for d in range(2)], axis=0)
        H2 = lax.dot_general(_bc(fs[128:256, :]), h2, (((1,), (1,)), ((), ())), preferred_element_type=f32)
        if j0 == 0:
            h0 = jnp.concatenate(
                [H2[r * RP:(r + 1) * RP, 0:G] + dvec if r % 2 == 0 else H2[r * RP:(r + 1) * RP, 0:G]
                 for r in range(2 * NR)], axis=0)
        for d in range(2):
            j = j0 + d
            U_s[j] = U2[:, d * G:(d + 1) * G]
            H = H2[:, d * G:(d + 1) * G]
            if j == 0:
                G_s[0] = h0
            else:
                for r in range(NR):
                    a, b = 2 * r * RP, (2 * r + 1) * RP
                    hre, him = H[a:a + RP], H[b:b + RP]
                    if d == 0:
                        pre, pim = H_s[pl.ds(a, RP), :], H_s[pl.ds(b, RP), :]
                    else:
                        hp = h0 if j0 == 0 else H2[:, 0:G]
                        pre, pim = hp[a:a + RP], hp[b:b + RP]
                    if r < NR // 2:
                        G_s[j, pl.ds(a, RP), :] = hre - pim
                        G_s[j, pl.ds(b, RP), :] = him + pre
                    else:
                        G_s[j, pl.ds(a, RP), :] = hre + pim
                        G_s[j, pl.ds(b, RP), :] = him - pre
        if j0 + 2 < NB:
            H_s[...] = H2[:, G:2 * G]

    def load_sk(g):
        return sks[:, col(g)].astype(f32)

    def load_d(g):
        dall = ds_[...].astype(f32)
        rows = lax.broadcasted_iota(jnp.int32, (8, G), 0)
        return jnp.sum(jnp.where(rows == g, dall, 0.0), axis=0, keepdims=True)

    held = {}

    def a_piece(i0, r, dep):
        a, b = 2 * r * RP, (2 * r + 1) * RP
        acc = [(dep, dep)] * TI
        gw = {}
        for j in range(i0 + TI):
            ure, uim = U_s[j, pl.ds(a, RP), :], U_s[j, pl.ds(b, RP), :]
            for t in range(TI):
                m = i0 + t - j
                if m < 0:
                    continue
                if m not in gw:
                    gw[m] = (G_s[m, pl.ds(a, RP), :], G_s[m, pl.ds(b, RP), :])
                gre, gim = gw[m]
                tre = gre * ure - gim * uim
                tim = gre * uim + gim * ure
                zre, zim = acc[t]
                acc[t] = (tre if zre is None else zre + tre, tim if zim is None else zim + tim)
        if r % 2 == 0:
            held[(i0, r)] = acc
        else:
            prev = held.pop((i0, r - 1))
            for t in range(TI):
                for c in range(2):
                    z = jnp.concatenate([prev[t][c], acc[t][c]], axis=0)
                    Z_s[i0 + t, c, pl.ds((r - 1) * RP, 2 * RP), :] = z.astype(bf16)

    def a_inv(g, i0):
        e2 = _dot(_bc(fis[0:32, :]), jnp.concatenate([_ld(Z_s, i0 + d, 0, (0, 128)) for d in range(2)], axis=1))
        o2 = _dot(_bc(fis[32:64, :]), jnp.concatenate([_ld(Z_s, i0 + d, 1, (0, 128)) for d in range(2)], axis=1))
        rev = 7 - lax.broadcasted_iota(jnp.int32, (8, G), 0)
        for d in range(2):
            r0 = (i0 + d) * B
            e, o = e2[:, d * G:(d + 1) * G], o2[:, d * G:(d + 1) * G]
            hi = e - o
            y = jnp.concatenate(
                [e + o] + [jnp.take_along_axis(hi[8 * (7 - v):8 * (8 - v)], rev, axis=0) for v in range(8)], axis=0)
            qq = _bc(qs[g, pl.ds(r0 // 2, B // 2), :]).astype(f32)
            oa_s[g, pl.ds(r0, B), :] = (qq * y).astype(bf16)

    def emit(mm, state, ga, t_fill_end):
        pieces = []
        if ga is not None:
            for i0 in range(NB - TI, -1, -TI):
                pieces += [(i0, r) for r in range(NR)]
        cost_of = lambda i0: sum(i + 1 for i in range(i0, i0 + TI))
        total = sum(cost_of(i0) for i0, _ in pieces)
        t_now, done, nxt, pend_inv = 0, 0, 0, []
        for (cost, fn, is_fwd) in mm:
            if is_fwd:
                assert nxt == len(pieces) and not pend_inv, "the next tile's transforms overwrite U / G"
            fn()
            t_now += cost
            for i0 in pend_inv:
                a_inv(ga, i0)
                t_now += 64
            pend_inv = []
            target = total * min(1.0, t_now / t_fill_end)
            kk = 0
            while nxt < len(pieces) and done < target:
                i0, r = pieces[nxt]
                dep = None
                if 'pace' in state:
                    pace = state['pace']
                    idx = min(pace.shape[0] // RP - 1, kk * PACE_STRIDE)
                    pv = pltpu.bitcast(pace[idx * RP:(idx + 1) * RP, :], u32)
                    dep = pltpu.bitcast(lax.shift_right_logical(lax.shift_right_logical(pv, u32(16)), u32(16)), f32)
                    kk += 1
                a_piece(i0, r, dep)
                done += cost_of(i0)
                nxt += 1
                if r == NR - 1:
                    pend_inv.extend(range(i0, i0 + TI, 2))
        assert nxt == len(pieces) and not pend_inv
        if ga is not None:
            cp_oa(ga).start()

    def group_step(g, ga, first):
        state = {}
        hooks = {}

        def proj_part(name, p, c, ks_):
            x = _bc(xs[pl.ds(c * CH // 2, CH // 2), pl.ds(ks_ * KS, KS)])
            wref = ws.at[g, p] if first else wcur.at[p]
            part = _dot(x, _bc(wref[pl.ds(ks_ * KS // 2, KS // 2), :]))
            state[name] = part if ks_ == 0 else state[name] + part
            state['pace'] = part
            if ks_ == KSPLIT - 1:
                for h in hooks.get((name, c), []):
                    h()

        def next_w(p):
            if not first:
                assert state.get('late_done')
                wcur[p] = ws[g + 1, p]

        def fin_k(c):
            pk = _phi(state.pop('k'))
            pk_s[pl.ds(c * CH, CH), :] = pk.astype(bf16)
            zp = jnp.sum(pk.reshape(CH // 8, 8, G), axis=0)
            state['z'] = zp if c == 0 else state['z'] + zp
            if c == NCH - 1:
                z_s[g] = state.pop('z')
                next_w(0)

        def fin_q(c):
            pq_s[g, pl.ds(c * CH, CH), :] = _phi(state.pop('q')).astype(bf16)
            if c == NCH - 1:
                next_w(1)

        def g_task(n, h):
            a = _ld(pk_s, (n * QR, QR))
            b = _bc(xs[pl.ds(n * QR // 2, QR // 2), pl.ds(h * GW, GW)])
            part = lax.dot_general(a, b, (((0,), (0,)), ((), ())), preferred_element_type=f32)
            state['pace'] = part[:, 0:G]
            acc = part if n == 0 else state[('G', h)] + part
            if n < NQ - 1:
                state[('G', h)] = acc
            else:
                for d in range(GW // G):
                    gm_s[g, h * (GW // G) + d] = acc[:, d * G:(d + 1) * G].astype(bf16)

        def fwd_task(j):
            assert state.get('late_done')
            if j == 0:
                state['sk'] = load_sk(g)
                state['dvec'] = load_d(g)
            a_fwd(g, state['sk'], state['dvec'], j)

        def wait_late():
            wait_all((cp_consts() if first else []) + cp_a(g) + ([] if first else [cp_w(g + 1, p) for p in range(2)]))
            state['late_done'] = True

        pc = CH * 8 // KSPLIT // 4
        units = []

        def add_proj(name, p, c, fin):
            for ks_ in range(KSPLIT):
                def t(ks_=ks_):
                    proj_part(name, p, c, ks_)
                    if ks_ == KSPLIT - 1:
                        fin(c)
                units.append((pc, t, (name, c)))

        per = NCH // NQ
        for c in range(NCH):
            add_proj('k', 0, c, fin_k)
            if c >= per:
                units.append((256, functools.partial(g_task, c // per - 1, c % per), ('G', c)))
            if c >= 1:
                add_proj('q', 1, c - 1, fin_q)
        add_proj('q', 1, NCH - 1, fin_q)
        for h in range(per):
            units.append((256, functools.partial(g_task, NQ - 1, h), ('G', NCH + h)))

        total = sum(u[0] for u in units)
        fwd_start, fwd_end = FWD_START * total, FWD_END * total
        pos = [fwd_start + (fwd_end - fwd_start) * n / (NB // 2) for n in range(NB // 2)]
        mm, t_now, nf, last_proj = [], 0, 0, None
        for (cost, fn, tag) in units:
            while nf < len(pos) and t_now >= pos[nf]:
                if nf == 0:
                    hooks.setdefault(last_proj, []).append(wait_late)
                mm.append((256, functools.partial(fwd_task, 2 * nf), True))
                nf += 1
            mm.append((cost, fn, False))
            t_now += cost
            if tag[0] in ('k', 'q'):
                last_proj = tag
        while nf < len(pos):
            mm.append((256, functools.partial(fwd_task, 2 * nf), True))
            nf += 1
        if first:
            for lo, hi in X_GROUPS:
                hooks.setdefault(('k', lo - 1), []).append(
                    functools.partial(lambda lo, hi: wait_all([cp_x(c) for c in range(lo, hi)]), lo, hi))
        emit(mm, state, ga, FILL_END * total)
        if first:
            wait_all([cp_w(1, p) for p in range(2)])
            for p in range(2):
                wcur[p] = ws[1, p]

    def m_tasks(state):
        r = lax.broadcasted_iota(jnp.int32, (G, G), 0) // HEAD
        c = lax.broadcasted_iota(jnp.int32, (G, G), 1) // HEAD
        bd = r == c

        def mt(g):
            z = jnp.sum(z_s[g], axis=0, keepdims=True)
            zc = jnp.broadcast_to(z, (G, G)).T
            zb_s[g] = jnp.where(bd, zc, 0.0).astype(bf16)
            gm = jnp.concatenate([_ld(gm_s, g, j, (0, G)) for j in range(NG)], axis=1)
            kv = _dot(gm, _bc(wvs[:, pl.ds(g * G, G)]))
            kvb = jnp.where(bd, kv, 0.0).astype(bf16)
            Mg = _dot(kvb, _bc(wos[pl.ds(g * G // 2, G // 2), :]))
            state['pace'] = Mg[:, 0:G]
            for j in range(NG):
                M_s[j, pl.ds(g * G, G), :] = Mg[:, j * G:(j + 1) * G].astype(bf16)
        return [(512, functools.partial(mt, g), False) for g in range(NG)]

    def norm_tasks(t, state):
        t0 = t * (RT // 2)
        rows = pl.ds(t0 if isinstance(t, int) else pl.multiple_of(t0, RT // 2), RT // 2)

        def norm(gs):
            for g in gs:
                pq = _bc(pq_s.bitcast(u32)[g, rows, :])
                den = _dot(pq, _ld(zb_s, g, (0, G))) + 1e-6
                pqn_s[g] = (pq.astype(f32) * pl.reciprocal(den, approx=True)).astype(bf16)
                state['pace'] = den
        return [(RT, functools.partial(norm, range(0, 4)), False), (RT, functools.partial(norm, range(4, 8)), False)]

    def tile_tasks(t, state, last=False):
        loc = {}

        def proj(j):
            if 'lhs' not in loc:
                loc['lhs'] = jnp.concatenate([_ld(pqn_s, g, (0, RT)) for g in range(NG)], axis=1)
            res = _dot(loc['lhs'], _ld(M_s, j, (0, D)))
            ob_s[t, j] = res.astype(bf16)
            state['pace'] = res
            cp_ob(t, j).start()

        pr = [(2 * RT, functools.partial(proj, j), False) for j in range(NG)]
        if last:
            return pr
        nm = norm_tasks(t + 1, state)
        return pr[:2] + nm[:1] + pr[2:4] + nm[1:] + pr[4:]

    @pl.when(step == 0)
    def _():
        ks[:, 0:8, :] = jnp.zeros((NG, 8, G), u32)
        cp_w(0, 0).start()
        cp_x(0).start()
        cp_w(0, 1).start()
        for c in range(1, NCH):
            cp_x(c).start()
        for c in cp_consts() + cp_a(0):
            c.start()
        for g in range(1, NG + 1):
            for p in range(2):
                cp_w(g, p).start()
            cp_q(g - 1).start()
            if g < NG:
                for c in cp_a(g):
                    c.start()
        for c in cp_wo():
            c.start()
        wait_all([cp_w(0, 0), cp_x(0), cp_w(0, 1)])
        group_step(0, None, True)

    @pl.when(jnp.logical_and(step > 0, step < NG))
    def _():
        cp_q(step - 1).wait()
        group_step(step, step - 1, False)

    @pl.when(step == NG)
    def _():
        wait_all(cp_wo() + [cp_q(NG - 1)])
        state = {}
        mt = m_tasks(state)
        nm = norm_tasks(0, state)
        mm = mt[:6] + nm[:1] + mt[6:] + nm[1:]
        for t in range(NTA):
            mm += tile_tasks(t, state)
        emit(mm, state, NG - 1, sum(m[0] for m in mm) * FILL_END_LAST)

    @pl.when(jnp.logical_and(step > NG, step < NSTEPS - 1))
    def _():
        for (_, fn, _) in tile_tasks(step - (NG + 1) + NTA, {}):
            fn()

    @pl.when(step == NSTEPS - 1)
    def _():
        for t in range(NT - NTL, NT):
            for (_, fn, _) in tile_tasks(t, {}, last=t == NT - 1):
                fn()
        pltpu.make_async_copy(oa_s, oa_s, sem_oa.at[0]).wait()
        pltpu.make_async_copy(ob_s, ob_s, sem_ob.at[0]).wait()


_SCRATCH = [
    pltpu.VMEM((NG, S // 2, G), u32), pltpu.VMEM((NG, 8 + S // 2, G), u32), pltpu.VMEM((NG, S // 2, G), u32),
    pltpu.VMEM((4, D), bf16), pltpu.VMEM((NG, G // 2, S), u32), pltpu.VMEM((8, 128), bf16),
    pltpu.VMEM((256, 128), u32), pltpu.VMEM((64, 128), u32),
    pltpu.VMEM((S // 2, D), u32), pltpu.VMEM((NG + 1, 2, D // 2, G), u32), pltpu.VMEM((D // 2, D), u32),
    pltpu.VMEM((D // 2, D), u32), pltpu.VMEM((2, D // 2, G), u32),
    pltpu.VMEM((NB, 256, G), f32), pltpu.VMEM((256, G), f32), pltpu.VMEM((NB, 256, G), f32),
    pltpu.VMEM((NB, 2, 128, G), bf16), pltpu.VMEM((NG, S, G), bf16),
    pltpu.VMEM((S, G), bf16), pltpu.VMEM((NG, NG, G, G), bf16), pltpu.VMEM((NG, S, G), bf16),
    pltpu.VMEM((NG, 8, G), f32),
    pltpu.VMEM((NG, D, G), bf16), pltpu.VMEM((NG, G, G), bf16), pltpu.VMEM((NT, NG, RT, G), bf16),
    pltpu.VMEM((NG, RT, G), bf16),
    pltpu.SemaphoreType.DMA((4,)), pltpu.SemaphoreType.DMA((NCH,)), pltpu.SemaphoreType.DMA((2 * (NG + 1),)),
    pltpu.SemaphoreType.DMA((NG,)), pltpu.SemaphoreType.DMA((NG,)), pltpu.SemaphoreType.DMA((2,)),
    pltpu.SemaphoreType.DMA((1,)), pltpu.SemaphoreType.DMA((1,)),
]
_FWD, _INV = _dft_mats()


@jax.jit
def pallas_concat_heads__ssm_conv_h3__linear_attn_block__prompt_kernel(
        A_q, A_k, A_v, A_shift_k, A_ssm_k, A_ssm_D, B_x, B_wqkv, B_wo):
    out = pl.pallas_call(
        _kernel,
        grid=(NSTEPS,),
        in_specs=[pl.BlockSpec(memory_space=pl.ANY)] * 11,
        out_specs=pl.BlockSpec(memory_space=pl.ANY),
        out_shape=jax.ShapeDtypeStruct((S, 2 * D), bf16),
        scratch_shapes=_SCRATCH,
        compiler_params=pltpu.CompilerParams(vmem_limit_bytes=110 * 1024 * 1024, dimension_semantics=("arbitrary",)),
    )(A_q.reshape(S, D), A_k.reshape(S, D), A_v.reshape(S, D), A_shift_k.T, A_ssm_k, A_ssm_D.reshape(8, 128),
      jnp.asarray(_FWD), jnp.asarray(_INV), B_x.reshape(S, D), B_wqkv, B_wo)
    return out.reshape(1, S, 2 * D)
```

```python
import functools

import jax
import jax.numpy as jnp
import numpy as np
from jax import lax
from jax.experimental import pallas as pl
from jax.experimental.pallas import tpu as pltpu

f32, bf16, u32 = jnp.float32, jnp.bfloat16, jnp.uint32

S, D = 2048, 1024
G = 128
NG = D // G
HEAD = 32
B = 128
NB = S // B
RP = 8
NR = 128 // RP
TI = 4
CH = 128
NCH = S // CH
KSPLIT = 2
KS = D // KSPLIT
RT = 256
NT = S // RT
NTA = 4
NTL = 2
NSTEPS = NG + 2 + (NT - NTA - NTL)

FWD_START, FWD_END, FILL_END = 14.0 / 16, 1.0, 13.9 / 16
FILL_END_LAST = 0.9
PACE_STRIDE = 8
X_GROUPS = ((1, 2), (2, 3), (3, 5), (5, 8), (8, 12), (12, 16))


def _pack_rows(a):
    b = np.asarray(a, dtype=bf16).view(np.uint16).astype(np.uint32)
    return b[0::2] | (b[1::2] << 16)


def _dft_mats():
    ks = np.concatenate([np.arange(0, 128, 2), np.arange(1, 128, 2)])
    sg = np.where(ks % 2 == 0, 1.0, -1.0)[:, None]
    th = (np.pi * (2 * ks + 1) / 256.0)[:, None]
    t = np.arange(128)[None, :]

    def inter(re, im):
        rows = []
        for r in range(NR):
            rows.append(re[r * RP:(r + 1) * RP])
            rows.append(im[r * RP:(r + 1) * RP])
        return np.concatenate(rows, axis=0)

    hre, him = np.cos(th * t), -np.sin(th * t)
    ure, uim = np.cos(th * (t + 0.5)), -np.sin(th * (t + 0.5))
    fu = inter(ure - sg * uim, uim + sg * ure)
    fu = np.concatenate([fu[:, 0::2], fu[:, 1::2]], axis=1)
    fh = inter(hre, him)
    phi = th * (np.arange(64)[None, :] + 0.5)
    c1 = ((np.cos(phi) + sg * np.sin(phi)) / 256.0).T
    c2 = ((sg * np.cos(phi) - np.sin(phi)) / 256.0).T
    fwd = np.concatenate([_pack_rows(fu), _pack_rows(fh)], axis=0)
    inv = np.concatenate([_pack_rows(c1), _pack_rows(c2)], axis=0)
    return fwd, inv


def _phi(t):
    return jnp.where(t > 0, t + 1.0, jnp.exp(t)) + 1e-6


def _dot(a, b):
    return jnp.dot(a, b, preferred_element_type=f32)


def _bc(x):
    return pltpu.bitcast(x, bf16)


def _ld(ref, *idx):
    *lead, (r0, n) = idx
    return _bc(ref.bitcast(u32)[(*lead, pl.ds(r0 // 2, n // 2), slice(None))])


def _kernel(q_hbm, k_hbm, v_hbm, sk_hbm, h_hbm, d_hbm, f_hbm, fi_hbm, x_hbm, w_hbm, wo_hbm, o_hbm,
            qs, ks, vs, sks, hs, ds_, fs, fis, xs, ws, wos, wvs, wcur,
            U_s, H_s, G_s, Z_s, oa_s, pk_s, gm_s, pq_s, z_s, M_s, zb_s, ob_s, pqn_s,
            sem_c, sem_x, sem_w, sem_a, sem_q, sem_wo, sem_oa, sem_ob):
    step = pl.program_id(0)
    q32, k32, v32, h32 = (r.bitcast(u32) for r in (q_hbm, k_hbm, v_hbm, h_hbm))
    x32, w32, wo32 = (r.bitcast(u32) for r in (x_hbm, w_hbm, wo_hbm))

    def col(g):
        return pl.ds(pl.multiple_of(g * G, G), G)

    def cp_consts():
        return [pltpu.make_async_copy(a, b, sem_c.at[n]) for n, (a, b) in
                enumerate(((f_hbm, fs), (fi_hbm, fis), (sk_hbm, sks), (d_hbm, ds_)))]

    def cp_x(c):
        rows = pl.ds(c * (CH // 2), CH // 2)
        return pltpu.make_async_copy(x32.at[rows], xs.at[rows], sem_x.at[c])

    def cp_w(g, p):
        gs = min(g, NG - 1) if isinstance(g, int) else jnp.minimum(g, NG - 1)
        off = (D, 0)[p]
        cols = pl.ds(off + gs * G if isinstance(gs, int) else pl.multiple_of(off + gs * G, G), G)
        return pltpu.make_async_copy(w32.at[:, cols], ws.at[g, p], sem_w.at[2 * g + p])

    def cp_a(g):
        return [pltpu.make_async_copy(k32.at[:, col(g)], ks.at[g, pl.ds(8, S // 2)], sem_a.at[g]),
                pltpu.make_async_copy(v32.at[:, col(g)], vs.at[g], sem_a.at[g]),
                pltpu.make_async_copy(h32.at[pl.ds(pl.multiple_of(g * (G // 2), G // 2), G // 2)], hs.at[g], sem_a.at[g])]

    def cp_q(g):
        return pltpu.make_async_copy(q32.at[:, col(g)], qs.at[g], sem_q.at[g])

    def cp_wo():
        return [pltpu.make_async_copy(wo32, wos, sem_wo.at[0]),
                pltpu.make_async_copy(w32.at[:, pl.ds(2 * D, D)], wvs, sem_wo.at[1])]

    def cp_oa(g):
        return pltpu.make_async_copy(oa_s.at[g], o_hbm.at[:, col(g)], sem_oa.at[0])

    def cp_ob(t, j):
        rows = pl.ds(t * RT if isinstance(t, int) else pl.multiple_of(t * RT, RT), RT)
        return pltpu.make_async_copy(ob_s.at[t, j], o_hbm.at[rows, pl.ds(D + j * G, G)], sem_ob.at[0])

    def wait_all(cps):
        for c in cps:
            c.wait()

    def a_pre(g, sk, j):
        n = B // 2
        w0 = 8 + j * n
        lo = lambda x: pltpu.bitcast(lax.shift_left(x, u32(16)), f32)
        hi = lambda x: pltpu.bitcast(x & u32(0xFFFF0000), f32)
        k0, k1, k2 = (ks[g, pl.ds(w0 - d, n), :] for d in range(3))
        e0, o0, e1, o1, o2 = lo(k0), hi(k0), lo(k1), hi(k1), hi(k2)
        s0, s1, s2, s3 = (sk[t:t + 1, :] for t in range(4))
        ye = e0 * s0 + o1 * s1 + e1 * s2 + o2 * s3
        yo = o0 * s0 + e0 * s1 + o1 * s2 + e1 * s3
        vv = vs[g, pl.ds(j * n, n), :]
        return jnp.concatenate([ye * lo(vv), yo * hi(vv)], axis=0).astype(bf16)

    def a_fwd(g, sk, dvec, j0):
        u2 = jnp.concatenate([a_pre(g, sk, j0), a_pre(g, sk, j0 + 1)], axis=1)
        U2 = _dot(_bc(fs[0:128, :]), u2)
        h2 = jnp.concatenate([_bc(hs[g, :, pl.ds((j0 + d) * B, B)]) for d in range(2)], axis=0)
        H2 = lax.dot_general(_bc(fs[128:256, :]), h2, (((1,), (1,)), ((), ())), preferred_element_type=f32)
        if j0 == 0:
            h0 = jnp.concatenate(
                [H2[r * RP:(r + 1) * RP, 0:G] + dvec if r % 2 == 0 else H2[r * RP:(r + 1) * RP, 0:G]
                 for r in range(2 * NR)], axis=0)
        for d in range(2):
            j = j0 + d
            U_s[j] = U2[:, d * G:(d + 1) * G]
            H = H2[:, d * G:(d + 1) * G]
            if j == 0:
                G_s[0] = h0
            else:
                for r in range(NR):
                    a, b = 2 * r * RP, (2 * r + 1) * RP
                    hre, him = H[a:a + RP], H[b:b + RP]
                    if d == 0:
                        pre, pim = H_s[pl.ds(a, RP), :], H_s[pl.ds(b, RP), :]
                    else:
                        hp = h0 if j0 == 0 else H2[:, 0:G]
                        pre, pim = hp[a:a + RP], hp[b:b + RP]
                    if r < NR // 2:
                        G_s[j, pl.ds(a, RP), :] = hre - pim
                        G_s[j, pl.ds(b, RP), :] = him + pre
                    else:
                        G_s[j, pl.ds(a, RP), :] = hre + pim
                        G_s[j, pl.ds(b, RP), :] = him - pre
        if j0 + 2 < NB:
            H_s[...] = H2[:, G:2 * G]

    def load_sk(g):
        return sks[:, col(g)].astype(f32)

    def load_d(g):
        dall = ds_[...].astype(f32)
        rows = lax.broadcasted_iota(jnp.int32, (8, G), 0)
        return jnp.sum(jnp.where(rows == g, dall, 0.0), axis=0, keepdims=True)

    held = {}

    def a_piece(i0, r, dep):
        a, b = 2 * r * RP, (2 * r + 1) * RP
        acc = [(dep, dep)] * TI
        gw = {}
        for j in range(i0 + TI):
            ure, uim = U_s[j, pl.ds(a, RP), :], U_s[j, pl.ds(b, RP), :]
            for t in range(TI):
                m = i0 + t - j
                if m < 0:
                    continue
                if m not in gw:
                    gw[m] = (G_s[m, pl.ds(a, RP), :], G_s[m, pl.ds(b, RP), :])
                gre, gim = gw[m]
                tre = gre * ure - gim * uim
                tim = gre * uim + gim * ure
                zre, zim = acc[t]
                acc[t] = (tre if zre is None else zre + tre, tim if zim is None else zim + tim)
        if r % 2 == 0:
            held[(i0, r)] = acc
        else:
            prev = held.pop((i0, r - 1))
            for t in range(TI):
                for c in range(2):
                    z = jnp.concatenate([prev[t][c], acc[t][c]], axis=0)
                    Z_s[i0 + t, c, pl.ds((r - 1) * RP, 2 * RP), :] = z.astype(bf16)

    def a_inv(g, i0):
        e2 = _dot(_bc(fis[0:32, :]), jnp.concatenate([_ld(Z_s, i0 + d, 0, (0, 128)) for d in range(2)], axis=1))
        o2 = _dot(_bc(fis[32:64, :]), jnp.concatenate([_ld(Z_s, i0 + d, 1, (0, 128)) for d in range(2)], axis=1))
        rev = 7 - lax.broadcasted_iota(jnp.int32, (8, G), 0)
        for d in range(2):
            r0 = (i0 + d) * B
            e, o = e2[:, d * G:(d + 1) * G], o2[:, d * G:(d + 1) * G]
            hi = e - o
            y = jnp.concatenate(
                [e + o] + [jnp.take_along_axis(hi[8 * (7 - v):8 * (8 - v)], rev, axis=0) for v in range(8)], axis=0)
            qq = _bc(qs[g, pl.ds(r0 // 2, B // 2), :]).astype(f32)
            oa_s[g, pl.ds(r0, B), :] = (qq * y).astype(bf16)

    def emit(mm, state, ga, t_fill_end):
        pieces = []
        if ga is not None:
            for i0 in range(NB - TI, -1, -TI):
                pieces += [(i0, r) for r in range(NR)]
        cost_of = lambda i0: sum(i + 1 for i in range(i0, i0 + TI))
        total = sum(cost_of(i0) for i0, _ in pieces)
        t_now, done, nxt, pend_inv = 0, 0, 0, []
        for (cost, fn, is_fwd) in mm:
            if is_fwd:
                assert nxt == len(pieces) and not pend_inv, "the next tile's transforms overwrite U / G"
            fn()
            t_now += cost
            for i0 in pend_inv:
                a_inv(ga, i0)
                t_now += 64
            pend_inv = []
            target = total * min(1.0, t_now / t_fill_end)
            kk = 0
            while nxt < len(pieces) and done < target:
                i0, r = pieces[nxt]
                dep = None
                if 'pace' in state:
                    pace = state['pace']
                    idx = min(pace.shape[0] // RP - 1, kk * PACE_STRIDE)
                    pv = pltpu.bitcast(pace[idx * RP:(idx + 1) * RP, :], u32)
                    dep = pltpu.bitcast(lax.shift_right_logical(lax.shift_right_logical(pv, u32(16)), u32(16)), f32)
                    kk += 1
                a_piece(i0, r, dep)
                done += cost_of(i0)
                nxt += 1
                if r == NR - 1:
                    pend_inv.extend(range(i0, i0 + TI, 2))
        assert nxt == len(pieces) and not pend_inv
        if ga is not None:
            cp_oa(ga).start()

    def group_step(g, ga, first):
        nq = NCH if first else 4
        per = NCH // nq
        qr, gw = S // nq, D // per
        state = {}
        hooks = {}

        def proj_part(name, p, c, ks_):
            x = _bc(xs[pl.ds(c * CH // 2, CH // 2), pl.ds(ks_ * KS, KS)])
            wref = ws.at[g, p] if first else wcur.at[p]
            part = _dot(x, _bc(wref[pl.ds(ks_ * KS // 2, KS // 2), :]))
            state[name] = part if ks_ == 0 else state[name] + part
            state['pace'] = part
            if ks_ == KSPLIT - 1:
                for h in hooks.get((name, c), []):
                    h()

        def next_w(p):
            if not first:
                assert state.get('late_done')
                wcur[p] = ws[g + 1, p]

        def fin_k(c):
            pk = _phi(state.pop('k'))
            pk_s[pl.ds(c * CH, CH), :] = pk.astype(bf16)
            zp = jnp.sum(pk.reshape(CH // 8, 8, G), axis=0)
            state['z'] = zp if c == 0 else state['z'] + zp
            if c == NCH - 1:
                z_s[g] = state.pop('z')
                next_w(0)

        def fin_q(c):
            pq_s[g, pl.ds(c * CH, CH), :] = _phi(state.pop('q')).astype(bf16)
            if c == NCH - 1:
                next_w(1)

        def g_task(n, h):
            a = _ld(pk_s, (n * qr, qr))
            b = _bc(xs[pl.ds(n * qr // 2, qr // 2), pl.ds(h * gw, gw)])
            part = lax.dot_general(a, b, (((0,), (0,)), ((), ())), preferred_element_type=f32)
            state['pace'] = part[:, 0:G]
            acc = part if n == 0 else state[('G', h)] + part
            if n < nq - 1:
                state[('G', h)] = acc
            else:
                for d in range(gw // G):
                    gm_s[g, h * (gw // G) + d] = acc[:, d * G:(d + 1) * G].astype(bf16)

        def fwd_task(j):
            assert state.get('late_done')
            if j == 0:
                state['sk'] = load_sk(g)
                state['dvec'] = load_d(g)
            a_fwd(g, state['sk'], state['dvec'], j)

        def wait_late():
            wait_all((cp_consts() if first else []) + cp_a(g) + ([] if first else [cp_w(g + 1, p) for p in range(2)]))
            state['late_done'] = True

        pc = CH * 8 // KSPLIT // 4
        units = []

        def add_proj(name, p, c, fin):
            for ks_ in range(KSPLIT):
                def t(ks_=ks_):
                    proj_part(name, p, c, ks_)
                    if ks_ == KSPLIT - 1:
                        fin(c)
                units.append((pc, t, (name, c)))

        for c in range(NCH):
            add_proj('k', 0, c, fin_k)
            if c >= per:
                units.append((256, functools.partial(g_task, c // per - 1, c % per), ('G', c)))
            if c >= 1:
                add_proj('q', 1, c - 1, fin_q)
        add_proj('q', 1, NCH - 1, fin_q)
        for h in range(per):
            units.append((256, functools.partial(g_task, nq - 1, h), ('G', NCH + h)))

        total = sum(u[0] for u in units)
        fwd_start, fwd_end = FWD_START * total, FWD_END * total
        pos = [fwd_start + (fwd_end - fwd_start) * n / (NB // 2) for n in range(NB // 2)]
        mm, t_now, nf, last_proj = [], 0, 0, None
        for (cost, fn, tag) in units:
            while nf < len(pos) and t_now >= pos[nf]:
                if nf == 0:
                    hooks.setdefault(last_proj, []).append(wait_late)
                mm.append((256, functools.partial(fwd_task, 2 * nf), True))
                nf += 1
            mm.append((cost, fn, False))
            t_now += cost
            if tag[0] in ('k', 'q'):
                last_proj = tag
        while nf < len(pos):
            mm.append((256, functools.partial(fwd_task, 2 * nf), True))
            nf += 1
        if first:
            for lo, hi in X_GROUPS:
                hooks.setdefault(('q', lo - 2) if lo >= 2 else ('k', 0), []).append(
                    functools.partial(lambda lo, hi: wait_all([cp_x(c) for c in range(lo, hi)]), lo, hi))
        emit(mm, state, ga, FILL_END * total)
        if first:
            wait_all([cp_w(1, p) for p in range(2)])
            for p in range(2):
                wcur[p] = ws[1, p]

    def m_tasks(state):
        r = lax.broadcasted_iota(jnp.int32, (G, G), 0) // HEAD
        c = lax.broadcasted_iota(jnp.int32, (G, G), 1) // HEAD
        bd = r == c

        def mt(g):
            z = jnp.sum(z_s[g], axis=0, keepdims=True)
            zc = jnp.broadcast_to(z, (G, G)).T
            zb_s[g] = jnp.where(bd, zc, 0.0).astype(bf16)
            gm = jnp.concatenate([_ld(gm_s, g, j, (0, G)) for j in range(NG)], axis=1)
            kv = _dot(gm, _bc(wvs[:, pl.ds(g * G, G)]))
            kvb = jnp.where(bd, kv, 0.0).astype(bf16)
            Mg = _dot(kvb, _bc(wos[pl.ds(g * G // 2, G // 2), :]))
            state['pace'] = Mg[:, 0:G]
            for j in range(NG):
                M_s[j, pl.ds(g * G, G), :] = Mg[:, j * G:(j + 1) * G].astype(bf16)
        return [(512, functools.partial(mt, g), False) for g in range(NG)]

    def norm_tasks(t, state):
        t0 = t * (RT // 2)
        rows = pl.ds(t0 if isinstance(t, int) else pl.multiple_of(t0, RT // 2), RT // 2)

        def norm(gs):
            for g in gs:
                pq = _bc(pq_s.bitcast(u32)[g, rows, :])
                den = _dot(pq, _ld(zb_s, g, (0, G))) + 1e-6
                pqn_s[g] = (pq.astype(f32) * pl.reciprocal(den, approx=True)).astype(bf16)
                state['pace'] = den
        return [(RT, functools.partial(norm, range(0, 4)), False), (RT, functools.partial(norm, range(4, 8)), False)]

    def tile_tasks(t, state, last=False):
        loc = {}

        def proj(j):
            if 'lhs' not in loc:
                loc['lhs'] = jnp.concatenate([_ld(pqn_s, g, (0, RT)) for g in range(NG)], axis=1)
            res = _dot(loc['lhs'], _ld(M_s, j, (0, D)))
            ob_s[t, j] = res.astype(bf16)
            state['pace'] = res
            cp_ob(t, j).start()

        pr = [(2 * RT, functools.partial(proj, j), False) for j in range(NG)]
        if last:
            return pr
        nm = norm_tasks(t + 1, state)
        return pr[:2] + nm[:1] + pr[2:4] + nm[1:] + pr[4:]

    @pl.when(step == 0)
    def _():
        ks[:, 0:8, :] = jnp.zeros((NG, 8, G), u32)
        cp_w(0, 0).start()
        cp_x(0).start()
        cp_w(0, 1).start()
        for c in range(1, NCH):
            cp_x(c).start()
        for c in cp_consts() + cp_a(0):
            c.start()
        for g in range(1, NG + 1):
            for p in range(2):
                cp_w(g, p).start()
            cp_q(g - 1).start()
            if g < NG:
                for c in cp_a(g):
                    c.start()
        for c in cp_wo():
            c.start()
        wait_all([cp_w(0, 0), cp_x(0), cp_w(0, 1)])
        group_step(0, None, True)

    @pl.when(jnp.logical_and(step > 0, step < NG))
    def _():
        cp_q(step - 1).wait()
        group_step(step, step - 1, False)

    @pl.when(step == NG)
    def _():
        wait_all(cp_wo() + [cp_q(NG - 1)])
        state = {}
        mt = m_tasks(state)
        nm = norm_tasks(0, state)
        mm = mt[:6] + nm[:1] + mt[6:] + nm[1:]
        for t in range(NTA):
            mm += tile_tasks(t, state)
        emit(mm, state, NG - 1, sum(m[0] for m in mm) * FILL_END_LAST)

    @pl.when(jnp.logical_and(step > NG, step < NSTEPS - 1))
    def _():
        for (_, fn, _) in tile_tasks(step - (NG + 1) + NTA, {}):
            fn()

    @pl.when(step == NSTEPS - 1)
    def _():
        for t in range(NT - NTL, NT):
            for (_, fn, _) in tile_tasks(t, {}, last=t == NT - 1):
                fn()
        pltpu.make_async_copy(oa_s, oa_s, sem_oa.at[0]).wait()
        pltpu.make_async_copy(ob_s, ob_s, sem_ob.at[0]).wait()


_SCRATCH = [
    pltpu.VMEM((NG, S // 2, G), u32), pltpu.VMEM((NG, 8 + S // 2, G), u32), pltpu.VMEM((NG, S // 2, G), u32),
    pltpu.VMEM((4, D), bf16), pltpu.VMEM((NG, G // 2, S), u32), pltpu.VMEM((8, 128), bf16),
    pltpu.VMEM((256, 128), u32), pltpu.VMEM((64, 128), u32),
    pltpu.VMEM((S // 2, D), u32), pltpu.VMEM((NG + 1, 2, D // 2, G), u32), pltpu.VMEM((D // 2, D), u32),
    pltpu.VMEM((D // 2, D), u32), pltpu.VMEM((2, D // 2, G), u32),
    pltpu.VMEM((NB, 256, G), f32), pltpu.VMEM((256, G), f32), pltpu.VMEM((NB, 256, G), f32),
    pltpu.VMEM((NB, 2, 128, G), bf16), pltpu.VMEM((NG, S, G), bf16),
    pltpu.VMEM((S, G), bf16), pltpu.VMEM((NG, NG, G, G), bf16), pltpu.VMEM((NG, S, G), bf16),
    pltpu.VMEM((NG, 8, G), f32),
    pltpu.VMEM((NG, D, G), bf16), pltpu.VMEM((NG, G, G), bf16), pltpu.VMEM((NT, NG, RT, G), bf16),
    pltpu.VMEM((NG, RT, G), bf16),
    pltpu.SemaphoreType.DMA((4,)), pltpu.SemaphoreType.DMA((NCH,)), pltpu.SemaphoreType.DMA((2 * (NG + 1),)),
    pltpu.SemaphoreType.DMA((NG,)), pltpu.SemaphoreType.DMA((NG,)), pltpu.SemaphoreType.DMA((2,)),
    pltpu.SemaphoreType.DMA((1,)), pltpu.SemaphoreType.DMA((1,)),
]
_FWD, _INV = _dft_mats()


@jax.jit
def pallas_concat_heads__ssm_conv_h3__linear_attn_block__prompt_kernel(
        A_q, A_k, A_v, A_shift_k, A_ssm_k, A_ssm_D, B_x, B_wqkv, B_wo):
    out = pl.pallas_call(
        _kernel,
        grid=(NSTEPS,),
        in_specs=[pl.BlockSpec(memory_space=pl.ANY)] * 11,
        out_specs=pl.BlockSpec(memory_space=pl.ANY),
        out_shape=jax.ShapeDtypeStruct((S, 2 * D), bf16),
        scratch_shapes=_SCRATCH,
        compiler_params=pltpu.CompilerParams(vmem_limit_bytes=110 * 1024 * 1024, dimension_semantics=("arbitrary",)),
    )(A_q.reshape(S, D), A_k.reshape(S, D), A_v.reshape(S, D), A_shift_k.T, A_ssm_k, A_ssm_D.reshape(8, 128),
      jnp.asarray(_FWD), jnp.asarray(_INV), B_x.reshape(S, D), B_wqkv, B_wo)
    return out.reshape(1, S, 2 * D)
```
